```python
import jax
import jax.numpy as jnp

def _softmax(x, axis=-1):
    return jax.nn.softmax(x, axis=axis)
def _gelu(x):
    return jax.nn.gelu(x, approximate=True)
def _silu(x):
    return jax.nn.silu(x)
def _sigmoid(x):
    return jax.nn.sigmoid(x)
def _layernorm(x, axis=-1, eps=1e-5):
    m = jnp.mean(x, axis=axis, keepdims=True)
    v = jnp.var(x, axis=axis, keepdims=True)
    return (x - m) / jnp.sqrt(v + eps)
def _scatter_add(tgt, idx, src, axis=0):
    return tgt.at[idx].add(src)
def _segment_sum(src, seg, n):
    return jax.ops.segment_sum(src, seg, n)
class _Rng:
    def __init__(self, key):
        self._k = key
    def _next(self):
        self._k, sub = jax.random.split(self._k)
        return sub
    def normal(self, shape):
        return jax.random.normal(self._next(), shape, dtype=jnp.bfloat16)
    def randint(self, lo, hi, shape):
        return jax.random.randint(self._next(), shape, lo, hi, dtype=jnp.int32)
    def uniform(self, shape, lo=0.0, hi=1.0):
        return jax.random.uniform(self._next(), shape, jnp.bfloat16, lo, hi)
    def permutation(self, n):
        return jax.random.permutation(self._next(), n)


kernel_name = 'gated_mix__linear_kernel_hedgehog__moe_arch_mod__prompt'

def setup_inputs():
    _rng = _Rng(jax.random.key(int.from_bytes(__import__("os").urandom(4), "little")))
    _w = (lambda a: (lambda t: t.astype(jnp.bfloat16) if jnp.issubdtype(t.dtype, jnp.floating) else t)(jnp.asarray(a)))
    def _A_setup():
        B, S, D, H = 1, 2048, 1024, 32
        Dh = D // H
        return {
            "x": _w((lambda *s: _rng.normal(s) * 0.05)(B, S, D)),
            "wqkv": _w((lambda *s: _rng.normal(s) * 0.05)(D, 3 * D)),
            "w_phi": _w((lambda *s: _rng.normal(s) * 0.05)(H, Dh, Dh) * (Dh ** -0.5)),
            "wo": _w((lambda *s: _rng.normal(s) * 0.05)(D, D)),
        }
    _A_in = _A_setup()

    def _B_setup():
        B, S, D, F, C = 1, 2048, 1024, 3584, 1
        return {
            "x": _w((lambda *s: _rng.normal(s) * 0.05)(B, S, D)),
            "w_r": _w((lambda *s: _rng.normal(s) * 0.05)(D)),
            "w_gate": _w((lambda *s: _rng.normal(s) * 0.05)(D, F)),
            "w_up": _w((lambda *s: _rng.normal(s) * 0.05)(D, F)),
            "w_down": _w((lambda *s: _rng.normal(s) * 0.05)(F, D)),
        }
    _B_in = _B_setup()

    return {
        "A_x": _A_in["x"],
        "A_wqkv": _A_in["wqkv"],
        "A_w_phi": _A_in["w_phi"],
        "A_wo": _A_in["wo"],
        "B_x": _B_in["x"],
        "B_w_r": _B_in["w_r"],
        "B_w_gate": _B_in["w_gate"],
        "B_w_up": _B_in["w_up"],
        "B_w_down": _B_in["w_down"],
        "gate_w": _w((lambda *s: _rng.normal(s) * 0.05)(1024)),
    }

def reference(A_x, A_wqkv, A_w_phi, A_wo, B_x, B_w_r, B_w_gate, B_w_up, B_w_down, gate_w):
    def _A_ref(x, wqkv, w_phi, wo):
        B, S, D = x.shape
        H = 32; Dh = D // H
        qkv = (lambda x, *d: x.transpose(*d))((x @ wqkv).reshape(B, S, 3, H, Dh), 2, 0, 3, 1, 4)
        q, k, v = qkv[0], qkv[1], qkv[2]
        pq = jnp.einsum("bhsd,hdf->bhsf", q, w_phi)
        pk = jnp.einsum("bhsd,hdf->bhsf", k, w_phi)
        phi_q = jnp.concatenate([_softmax(pq, axis=-1), _softmax(-pq, axis=-1)], axis=-1)
        phi_k = jnp.concatenate([_softmax(pk, axis=-1), _softmax(-pk, axis=-1)], axis=-1)
        kv = jnp.einsum("bhsf,bhsd->bhfd", phi_k, v)
        z  = jnp.einsum("bhsf->bhf", phi_k)
        num = jnp.einsum("bhqf,bhfd->bhqd", phi_q, kv)
        den = jnp.einsum("bhqf,bhf->bhq", phi_q, z)[..., None] + 1e-6
        o = num / den
        return (lambda x, *d: x.transpose(*d))(o, 0, 2, 1, 3).reshape(B, S, D) @ wo

    def _B_ref(x, w_r, w_gate, w_up, w_down):
        B, S, D = x.shape
        C = 1
        r = x @ w_r
        idx = jnp.argsort(-r, axis=-1)[:, :C]
        idx_e = jnp.repeat(idx.reshape(B, C, 1), D, axis=2)
        x_sel = jnp.take_along_axis(x, idx_e, axis=1)
        g = _silu(x_sel @ w_gate)
        u = x_sel @ w_up
        y = (g * u) @ w_down
        r_sel = _sigmoid(jnp.take_along_axis(r, idx, axis=1))
        y = y * r_sel.reshape(B, C, 1)
        b_off = (jnp.arange(B) * S).reshape(B, 1)
        flat_idx = (idx + b_off).reshape(B * C)
        zero = (x * 0.0).reshape(B * S, D)
        upd = _scatter_add(zero, flat_idx, y.reshape(B * C, D), axis=0)
        return x + upd.reshape(B, S, D)

    x = A_x
    g = _sigmoid((x * gate_w).sum(-1, keepdims=True))
    a = _A_ref(x, A_wqkv, A_w_phi, A_wo)
    b = _B_ref(x, B_w_r, B_w_gate, B_w_up, B_w_down)
    return g * a + (1 - g) * b
```

```python
import functools
import jax
import jax.numpy as jnp
import numpy as np
from jax import lax
from jax.experimental import pallas as pl
from jax.experimental.pallas import tpu as pltpu

S, D, H, DH, F = 2048, 1024, 32, 32, 3584
TM = 512
NT = S // TM
LOG2E = 1.4426950408889634
BF = jnp.bfloat16
F32 = jnp.float32


def _nt(a, b):
    return lax.dot_general(a, b, (((1,), (1,)), ((), ())), preferred_element_type=F32)


def _nn(a, b):
    return jnp.dot(a, b, preferred_element_type=F32)


def _red(x4, op):
    r = x4[:, 0]
    for k in range(1, 8):
        r = op(r, x4[:, k])
    r = op(r, pltpu.roll(r, 4, 1))
    r = op(r, pltpu.roll(r, 2, 1))
    return r


def kernel(xa_h, wqkv_h, wphi_h, wo_h, wr_h, wg_h, wu_h, wd_h, gw_h, out_h,
           xa, wq, wk, wv, wkf, wvt, wqf, wo, wg, wu, wd, wphi, wr, gw,
           ob, kvacc, zacc, kvt, zb, xsb, hb, yv, sem, osem):
    def cp(src, dst, k):
        return pltpu.make_async_copy(src, dst, sem.at[k])

    c_wphi = cp(wphi_h, wphi, 0)
    c_wk = cp(wqkv_h.at[:, pl.ds(D, D)], wk, 1)
    c_wv = cp(wqkv_h.at[:, pl.ds(2 * D, D)], wv, 2)
    c_xa = cp(xa_h, xa, 3)
    c_wq = cp(wqkv_h.at[:, pl.ds(0, D)], wq, 4)
    c_wr = cp(wr_h, wr, 6)
    c_gw = cp(gw_h, gw, 7)
    c_wo = cp(wo_h, wo, 8)
    c_wg = cp(wg_h, wg, 9)
    c_wu = cp(wu_h, wu, 10)
    c_wd = cp(wd_h, wd, 11)
    for c in (c_wphi, c_wk, c_wv, c_xa, c_wq, c_wr, c_gw, c_wo, c_wg, c_wu, c_wd):
        c.start()

    c_wphi.wait()
    jj = lax.broadcasted_iota(jnp.int32, (128, DH), 0)
    ff = lax.broadcasted_iota(jnp.int32, (128, DH), 1)
    et = jnp.where(((jj % 64) // 2) == ff, 1.0, 0.0).astype(BF)
    bd = _nt(et, wphi[...])
    j2 = lax.broadcasted_iota(jnp.int32, (128, D), 0)
    c2 = lax.broadcasted_iota(jnp.int32, (128, D), 1)
    keep = ((c2 % 128) // DH) == ((j2 // 64) * 2 + (j2 % 2))
    bd = jnp.where(keep, bd, 0.0).astype(BF)

    def fold(w_ref, dst):
        for g in range(8):
            t = _nt(bd[:, g * 128:(g + 1) * 128], w_ref[:, g * 128:(g + 1) * 128])
            dst[g * 128:(g + 1) * 128, :] = (t * LOG2E).astype(BF)

    c_wk.wait()
    fold(wk, wkf)
    c_wv.wait()
    wvt[...] = wv[...].T
    kvacc[...] = jnp.zeros_like(kvacc)
    zacc[...] = jnp.zeros_like(zacc)
    c_xa.wait()

    def p1(i, carry):
        xt = xa[pl.ds(pl.multiple_of(i * TM, TM), TM), :]
        pT = _nt(wkf[...], xt)
        vT = _nt(wvt[...], xt).astype(BF)
        p4 = pT.reshape(16, 8, 8, TM)
        mx = _red(p4, jnp.maximum)
        mn = _red(p4, jnp.minimum)
        ep = jnp.exp2(p4 - mx[:, None])
        en = jnp.exp2(mn[:, None] - p4)
        rp = 1.0 / _red(ep, jnp.add)
        rn = 1.0 / _red(en, jnp.add)
        php = (ep * rp[:, None]).reshape(16, 64, TM)
        phn = (en * rn[:, None]).reshape(16, 64, TM)
        ph = jnp.concatenate([php, phn], axis=1)
        zz = ph[:, :, 0:128]
        for c in range(1, TM // 128):
            zz = zz + ph[:, :, c * 128:(c + 1) * 128]
        zacc[...] += zz
        phb = ph.astype(BF)
        for j in range(16):
            kvacc[j] += _nt(vT[j * 64:(j + 1) * 64], phb[j])
        return carry

    lax.fori_loop(0, NT, p1, 0)

    r3 = lax.broadcasted_iota(jnp.int32, (16, 64, 128), 1)
    c3 = lax.broadcasted_iota(jnp.int32, (16, 64, 128), 2)
    kvt[...] = jnp.where((r3 // DH) == (c3 % 2), kvacc[...], 0.0).astype(BF)
    zb[...] = jnp.broadcast_to(jnp.sum(zacc[...], axis=2, keepdims=True), zb.shape)
    c_wq.wait()
    fold(wq, wqf)

    c_wr.wait()
    c_gw.wait()
    wrf = wr[...].astype(F32)

    def rt(i, carry):
        bv, bi = carry
        xt = xa[pl.ds(pl.multiple_of(i * 128, 128), 128), :].astype(F32)
        acc = xt[:, 0:128] * wrf[0:1]
        for k in range(1, 8):
            acc = acc + xt[:, k * 128:(k + 1) * 128] * wrf[k:k + 1]
        r = jnp.sum(acc, axis=1, keepdims=True).astype(BF).astype(F32)
        r = jnp.where(r != r, -jnp.inf, r)
        r = jnp.broadcast_to(r, (128, 128))
        idx = lax.broadcasted_iota(jnp.int32, (128, 128), 0) + i * 128
        better = r > bv
        return jnp.where(better, r, bv), jnp.where(better, idx, bi)

    bv0 = jnp.full((128, 128), -jnp.inf, F32)
    bi0 = lax.broadcasted_iota(jnp.int32, (128, 128), 0)
    bv, bi = lax.fori_loop(0, S // 128, rt, (bv0, bi0))
    rmax = jnp.max(bv, axis=0, keepdims=True)
    idx = jnp.min(jnp.where(bv == rmax, bi, S))
    rsel = jax.nn.sigmoid(rmax)

    base = pl.multiple_of((idx // 16) * 16, 16)
    blk = xa[pl.ds(base, 16), :].astype(F32)
    rows = lax.broadcasted_iota(jnp.int32, (16, D), 0)
    xs = jnp.sum(jnp.where(rows == idx - base, blk, 0.0), axis=0, keepdims=True)
    xsb[...] = jnp.broadcast_to(xs, (128, D)).T

    c_wg.wait()
    c_wu.wait()

    def gu(c, carry):
        cs = pl.ds(pl.multiple_of(c * 512, 512), 512)
        ag = jnp.zeros((16, 512), F32)
        au = jnp.zeros((16, 512), F32)
        for k in range(D // 16):
            xk = xsb[k * 16:(k + 1) * 16, :]
            xk = jnp.concatenate([xk] * 4, axis=1)
            ag = ag + wg[k * 16:(k + 1) * 16, cs].astype(F32) * xk
            au = au + wu[k * 16:(k + 1) * 16, cs].astype(F32) * xk
        g = jnp.sum(ag, axis=0, keepdims=True)
        u = jnp.sum(au, axis=0, keepdims=True)
        h = g * jax.nn.sigmoid(g) * u
        hb[cs, :] = jnp.broadcast_to(h, (128, 512)).T
        return carry

    lax.fori_loop(0, F // 512, gu, 0)
    c_wd.wait()

    def dn(c, acc):
        for k in range(512 // 16):
            rs = pl.ds(pl.multiple_of(c * 512 + k * 16, 16), 16)
            hk = hb[rs, :]
            hk = jnp.concatenate([hk] * 8, axis=1)
            acc = acc + wd[rs, :].astype(F32) * hk
        return acc

    ay = lax.fori_loop(0, F // 512, dn, jnp.zeros((16, D), F32))
    y = jnp.sum(ay, axis=0, keepdims=True) * jnp.concatenate([rsel] * 8, axis=1)
    yv[...] = jnp.broadcast_to(y, (8, D))

    c_wo.wait()
    gwf = gw[...].astype(F32)

    def p2(i, carry):
        r0 = pl.multiple_of(i * TM, TM)
        xt = xa[pl.ds(r0, TM), :]
        pT = _nt(wqf[...], xt)
        p4 = pT.reshape(16, 8, 8, TM)
        mx = _red(p4, jnp.maximum)
        mn = _red(p4, jnp.minimum)
        ep = jnp.exp2(p4 - mx[:, None])
        en = jnp.exp2(mn[:, None] - p4)
        rp = 1.0 / _red(ep, jnp.add)
        rn = 1.0 / _red(en, jnp.add)
        z4 = zb[...].reshape(16, 2, 8, 8, 128)
        zp = jnp.concatenate([z4[:, 0]] * (TM // 128), axis=-1)
        zn = jnp.concatenate([z4[:, 1]] * (TM // 128), axis=-1)
        den = _red(ep * zp, jnp.add) * rp + _red(en * zn, jnp.add) * rn + 1e-6
        rd = 1.0 / den
        php = (ep * (rp * rd)[:, None]).reshape(16, 64, TM)
        phn = (en * (rn * rd)[:, None]).reshape(16, 64, TM)
        phb = jnp.concatenate([php, phn], axis=1).astype(BF)
        oT = jnp.concatenate([_nn(kvt[j], phb[j]) for j in range(16)], axis=0)
        o = oT.astype(BF).T
        a = _nn(o, wo[...])
        xf = xt.astype(F32)
        acc = xf[:, 0:128] * gwf[0:1]
        for k in range(1, 8):
            acc = acc + xf[:, k * 128:(k + 1) * 128] * gwf[k:k + 1]
        g = jax.nn.sigmoid(jnp.sum(acc, axis=1, keepdims=True))
        xbt = xf
        rr = lax.broadcasted_iota(jnp.int32, (TM, D), 0) + i * TM
        upd = xbt * 0.0 + jnp.where(rr == idx, yv[0:1, :], 0.0)
        b = xbt + upd
        ob[pl.ds(r0, TM), :] = (g * a + (1.0 - g) * b).astype(BF)
        pltpu.make_async_copy(ob.at[pl.ds(r0, TM), :], out_h.at[pl.ds(r0, TM), :], osem.at[i]).start()
        return carry

    lax.fori_loop(0, NT, p2, 0)
    for i in range(NT):
        pltpu.make_async_copy(ob.at[pl.ds(i * TM, TM), :], out_h.at[pl.ds(i * TM, TM), :], osem.at[i]).wait()


@jax.jit
def pallas_gated_mix__linear_kernel_hedgehog__moe_arch_mod__prompt_kernel(
        A_x, A_wqkv, A_w_phi, A_wo, B_x, B_w_r, B_w_gate, B_w_up, B_w_down, gate_w):
    anyspec = pl.BlockSpec(memory_space=pl.ANY)
    V = pltpu.VMEM
    out = pl.pallas_call(
        kernel,
        out_shape=jax.ShapeDtypeStruct((S, D), BF),
        in_specs=[anyspec] * 9,
        out_specs=anyspec,
        scratch_shapes=[
            V((S, D), BF), V((D, D), BF), V((D, D), BF), V((D, D), BF),
            V((D, D), BF), V((D, D), BF), V((D, D), BF), V((D, D), BF),
            V((D, F), BF), V((D, F), BF), V((F, D), BF),
            V((D, DH), BF), V((8, 128), BF), V((8, 128), BF),
            V((S, D), BF), V((16, 64, 128), F32), V((16, 128, 128), F32),
            V((16, 64, 128), BF), V((16, 128, 128), F32),
            V((D, 128), F32), V((F, 128), F32), V((8, D), F32),
            pltpu.SemaphoreType.DMA((12,)), pltpu.SemaphoreType.DMA((NT,)),
        ],
        compiler_params=pltpu.CompilerParams(vmem_limit_bytes=110 * 2**20),
    )(A_x.reshape(S, D), A_wqkv, A_w_phi.reshape(D, DH), A_wo,
      B_w_r.reshape(8, 128), B_w_gate, B_w_up, B_w_down, gate_w.reshape(8, 128))
    return out.reshape(1, S, D)
```

```python
import functools
import jax
import jax.numpy as jnp
import numpy as np
from jax import lax
from jax.experimental import pallas as pl
from jax.experimental.pallas import tpu as pltpu

S, D, H, DH, F = 2048, 1024, 32, 32, 3584
TM = 512
NT = S // TM
FG = F // 2
FC = F // NT
LOG2E = 1.4426950408889634
BF = jnp.bfloat16
F32 = jnp.float32


def _nt(a, b):
    return lax.dot_general(a, b, (((1,), (1,)), ((), ())), preferred_element_type=F32)


def _nn(a, b):
    return jnp.dot(a, b, preferred_element_type=F32)


def _red8(x4, op):
    r = x4[:, 0]
    for k in range(1, 8):
        r = op(r, x4[:, k])
    return r


def _rot(r, op):
    r = op(r, pltpu.roll(r, 4, 1))
    return op(r, pltpu.roll(r, 2, 1))


def _dual_softmax_parts(pT):
    n = pT.shape[0] // 64
    p4 = pT.reshape(n, 8, 8, pT.shape[1])
    mx = _rot(_red8(p4, jnp.maximum), jnp.maximum)
    mn = _rot(_red8(p4, jnp.minimum), jnp.minimum)
    ep = jnp.exp2(p4 - mx[:, None])
    en = jnp.exp2(mn[:, None] - p4)
    rp = 1.0 / _rot(_red8(ep, jnp.add), jnp.add)
    rn = 1.0 / _rot(_red8(en, jnp.add), jnp.add)
    return ep, en, rp, rn


def _rowdot(xf, w8):
    acc = xf[:, 0:128] * w8[0:1]
    for k in range(1, 8):
        acc = acc + xf[:, k * 128:(k + 1) * 128] * w8[k:k + 1]
    return jnp.sum(acc, axis=1, keepdims=True)


def kernel(xa_h, wqkv_h, wphi_h, wo_h, wr_h, wg_h, wu_h, wd_h, gw_h, out_h,
           xa, wq, wk, wv, wkf, wvt, wqf, wo, wg, wu, wd, wphi, wr, gw,
           ob, kvacc, zacc, kvt, zb, gb, xsb, gu, hb, yacc, pb, sem, xsem, gsem, usem, osem):
    def cp(src, dst, k):
        return pltpu.make_async_copy(src, dst, sem.at[k])

    def xcp(i):
        return pltpu.make_async_copy(xa_h.at[pl.ds(i * TM, TM), :], xa.at[pl.ds(i * TM, TM), :], xsem.at[i])

    def gucp(i):
        cs = pl.ds(pl.multiple_of(i * FG, 128), FG)
        return (pltpu.make_async_copy(wg_h.at[:, cs], wg.at[:, cs], gsem.at[i]),
                pltpu.make_async_copy(wu_h.at[:, cs], wu.at[:, cs], usem.at[i]))

    HD = D // 2
    c_wphi = cp(wphi_h, wphi, 0)
    c_wk = [cp(wqkv_h.at[:, pl.ds(D + j * HD, HD)], wk.at[:, pl.ds(j * HD, HD)], 1 + j) for j in range(2)]
    c_wv = cp(wqkv_h.at[:, pl.ds(2 * D, D)], wv, 3)
    c_wq = cp(wqkv_h.at[:, pl.ds(0, D)], wq, 4)
    c_wr = cp(wr_h, wr, 5)
    c_gw = cp(gw_h, gw, 6)
    c_wo = cp(wo_h, wo, 7)
    c_wd = cp(wd_h, wd, 8)
    for c in (c_wphi, c_wk[0], c_wk[1], xcp(0), c_wr, c_gw):
        c.start()

    jj = lax.broadcasted_iota(jnp.int32, (128, DH), 0)
    ff = lax.broadcasted_iota(jnp.int32, (128, DH), 1)
    et = jnp.where(((jj & 63) >> 1) == ff, 1.0, 0.0).astype(BF)
    j2 = lax.broadcasted_iota(jnp.int32, (128, 128), 0)
    c2 = lax.broadcasted_iota(jnp.int32, (128, 128), 1)
    keep = (c2 >> 5) == ((j2 >> 6) * 2 + (j2 & 1))
    kvacc[...] = jnp.zeros_like(kvacc)
    zacc[...] = jnp.zeros_like(zacc)
    yacc[...] = jnp.zeros_like(yacc)
    c_wphi.wait()
    bd = _nt(et, wphi[...])
    bds = [jnp.where(keep, bd[:, g * 128:(g + 1) * 128], 0.0).astype(BF) for g in range(8)]

    def fold(w_ref, dst, groups):
        for g in groups:
            t = _nt(bds[g], w_ref[:, g * 128:(g + 1) * 128])
            dst[g * 128:(g + 1) * 128, :] = (t * LOG2E).astype(BF)

    c_wk[0].wait()
    c_wv.start()
    fold(wk, wkf, range(0, 4))
    c_wk[1].wait()
    xcp(1).start()
    fold(wk, wkf, range(4, 8))
    xcp(0).wait()
    for c in (xcp(2), xcp(3), *gucp(0), *gucp(1), c_wq, c_wo, c_wd):
        c.start()

    def phi_k(pT, j0):
        n = pT.shape[0] // 64
        ep, en, rp, rn = _dual_softmax_parts(pT)
        php = (ep * rp[:, None]).reshape(n, 64, TM)
        phn = (en * rn[:, None]).reshape(n, 64, TM)
        ph = jnp.concatenate([php, phn], axis=1)
        zz = ph[:, :, 0:128]
        for c in range(1, TM // 128):
            zz = zz + ph[:, :, c * 128:(c + 1) * 128]
        zacc[j0:j0 + n] += zz
        return ph.astype(BF)

    def kv_update(vT, phb, j0):
        for j in range(phb.shape[0]):
            kvacc[j0 + j] += _nt(vT[(j0 + j) * 64:(j0 + j + 1) * 64], phb[j])

    def router(t, bv, bi):
        xf = xa[t * TM:(t + 1) * TM, :].astype(F32)
        gb[t * TM:(t + 1) * TM, :] = jnp.broadcast_to(jax.nn.sigmoid(_rowdot(xf, gw[...].astype(F32))), (TM, 128))
        r = _rowdot(xf, wr[...].astype(F32)).astype(BF).astype(F32)
        r = jnp.broadcast_to(jnp.where(r != r, -jnp.inf, r), (TM, 128))
        row = lax.broadcasted_iota(jnp.int32, (8, 128), 0) + t * TM
        for k in range(TM // 8):
            rk = r[k * 8:(k + 1) * 8]
            better = rk > bv
            bv = jnp.where(better, rk, bv)
            bi = jnp.where(better, row + k * 8, bi)
        return bv, bi

    xt = xa[0:TM, :]
    pa = _nt(wkf[0:512, :], xt)
    pha = phi_k(pa, 0)
    pb_ = _nt(wkf[512:768, :], xt)
    c_wv.wait()
    xcp(1).wait()
    c_wr.wait()
    c_gw.wait()
    wvt[...] = wv[...].T
    pc = _nt(wkf[768:1024, :], xt)
    phb_ = phi_k(jnp.concatenate([pb_, pc], axis=0), 8)
    vT = _nt(wvt[...], xt).astype(BF)
    kv_update(vT, pha, 0)
    kv_update(vT, phb_, 8)
    bv = jnp.full((8, 128), -jnp.inf, F32)
    bi = lax.broadcasted_iota(jnp.int32, (8, 128), 0)
    bv, bi = router(0, bv, bi)
    bv, bi = router(1, bv, bi)

    def p1_tile(xt):
        pT = _nt(wkf[...], xt)
        vT = _nt(wvt[...], xt).astype(BF)
        kv_update(vT, phi_k(pT, 0), 0)

    xcp(2).wait()
    xcp(3).wait()
    p1_tile(xa[TM:2 * TM, :])
    bv, bi = router(2, bv, bi)
    bv, bi = router(3, bv, bi)

    rmax = jnp.max(bv, axis=0, keepdims=True)
    idx = jnp.min(jnp.where(bv == rmax, bi, S))
    rsel = jax.nn.sigmoid(rmax)
    base = pl.multiple_of((idx >> 4) << 4, 16)
    rows = lax.broadcasted_iota(jnp.int32, (16, D), 0)
    blk = xa[pl.ds(base, 16), :].astype(F32)
    xs = jnp.sum(jnp.where(rows == idx - base, blk, 0.0), axis=0, keepdims=True)
    xsb[...] = jnp.broadcast_to(xs, (128, D)).T
    never = idx < 0

    def p1(i, carry):
        for c in gucp(i):
            c.wait()
        acc = jnp.zeros((8, 128), F32)
        for c in range(FG // 128):
            cs = pl.ds(pl.multiple_of(i * FG + c * 128, 128), 128)
            for m, w_ref in enumerate((wg, wu)):
                acc = jnp.where(never, acc, 0.0)
                for k in range(D // 16):
                    t = w_ref[k * 16:(k + 1) * 16, cs].astype(F32) * xsb[k * 16:(k + 1) * 16, :]
                    acc = acc + t[0:8]
                    acc = acc + t[8:16]
                gu[m * 8:(m + 1) * 8, cs] = acc
        p1_tile(xa[pl.ds(pl.multiple_of((i + 2) * TM, TM), TM), :])
        return carry

    lax.fori_loop(0, 2, p1, 0)

    c_wq.wait()
    c_wo.wait()
    c_wd.wait()
    r3 = lax.broadcasted_iota(jnp.int32, (16, 64, 128), 1)
    c3 = lax.broadcasted_iota(jnp.int32, (16, 64, 128), 2)
    kvt[...] = jnp.where((r3 >> 5) == (c3 & 1), kvacc[...], 0.0).astype(BF)
    zb[...] = jnp.broadcast_to(jnp.sum(zacc[...], axis=2, keepdims=True), zb.shape)
    fold(wq, wqf, range(8))
    gg = jnp.sum(gu[0:8, :], axis=0, keepdims=True)
    uu = jnp.sum(gu[8:16, :], axis=0, keepdims=True)
    hb[...] = jnp.broadcast_to(gg * jax.nn.sigmoid(gg) * uu, (128, F)).T
    t0 = idx // TM

    def ocp(t, i):
        r0 = pl.multiple_of(t * TM, TM)
        return pltpu.make_async_copy(ob.at[pl.ds(r0, TM), :], out_h.at[pl.ds(r0, TM), :], osem.at[i])

    def p2(i, carry):
        t = (t0 + i) % NT
        r0 = pl.multiple_of(t * TM, TM)
        fs = pl.ds(pl.multiple_of(i * FC, 128), FC)
        wdc = wd.at[fs, :]
        hbc = hb.at[fs, :]
        acc = jnp.zeros((8, 128), F32)
        for c in range(D // 128):
            acc = jnp.where(never, acc, 0.0)
            for k in range(FC // 16):
                tt = wdc[k * 16:(k + 1) * 16, c * 128:(c + 1) * 128].astype(F32) * hbc[k * 16:(k + 1) * 16, :]
                acc = acc + tt[0:8]
                acc = acc + tt[8:16]
            yacc[:, c * 128:(c + 1) * 128] += acc

        xt = xa[pl.ds(r0, TM), :]
        pT = _nt(wqf[...], xt)
        ep, en, rp, rn = _dual_softmax_parts(pT)
        z4 = zb[...].reshape(16, 2, 8, 8, 128)
        zp = jnp.concatenate([z4[:, 0]] * (TM // 128), axis=-1)
        zn = jnp.concatenate([z4[:, 1]] * (TM // 128), axis=-1)
        den = _rot(_red8(ep * zp, jnp.add) * rp + _red8(en * zn, jnp.add) * rn, jnp.add) + 1e-6
        rd = 1.0 / den
        php = (ep * (rp * rd)[:, None]).reshape(16, 64, TM)
        phn = (en * (rn * rd)[:, None]).reshape(16, 64, TM)
        phb = jnp.concatenate([php, phn], axis=1).astype(BF)
        oT = jnp.concatenate([_nn(kvt[j], phb[j]) for j in range(16)], axis=0)
        o = oT.astype(BF).T
        a = _nn(o, wo[...])
        g = jnp.concatenate([gb[pl.ds(r0, TM), :]] * (D // 128), axis=1)
        ob[pl.ds(r0, TM), :] = (g * a + (1.0 - g) * xt.astype(F32)).astype(BF)
        ocp(t, i).start()
        return carry

    lax.fori_loop(0, NT, p2, 0)
    y = jnp.sum(yacc[...], axis=0, keepdims=True) * jnp.concatenate([rsel] * 8, axis=1)
    gsel = jnp.concatenate([gb[pl.ds(base, 16), :]] * (D // 128), axis=1)
    ocp(t0, 0).wait()
    old = ob[pl.ds(base, 16), :].astype(F32)
    pb[...] = jnp.where(rows == idx - base, old + (1.0 - gsel) * y, old).astype(BF)
    c_patch = cp(pb, out_h.at[pl.ds(base, 16), :], 9)
    c_patch.start()
    for i in range(1, NT):
        ocp((t0 + i) % NT, i).wait()
    c_patch.wait()


@jax.jit
def pallas_gated_mix__linear_kernel_hedgehog__moe_arch_mod__prompt_kernel(
        A_x, A_wqkv, A_w_phi, A_wo, B_x, B_w_r, B_w_gate, B_w_up, B_w_down, gate_w):
    anyspec = pl.BlockSpec(memory_space=pl.ANY)
    V = pltpu.VMEM
    out = pl.pallas_call(
        kernel,
        out_shape=jax.ShapeDtypeStruct((S, D), BF),
        in_specs=[anyspec] * 9,
        out_specs=anyspec,
        scratch_shapes=[
            V((S, D), BF), V((D, D), BF), V((D, D), BF), V((D, D), BF),
            V((D, D), BF), V((D, D), BF), V((D, D), BF), V((D, D), BF),
            V((D, F), BF), V((D, F), BF), V((F, D), BF),
            V((D, DH), BF), V((8, 128), BF), V((8, 128), BF),
            V((S, D), BF), V((16, 64, 128), F32), V((16, 128, 128), F32),
            V((16, 64, 128), BF), V((16, 128, 128), F32), V((S, 128), F32),
            V((D, 128), F32), V((16, F), F32), V((F, 128), F32), V((8, D), F32), V((16, D), BF),
            pltpu.SemaphoreType.DMA((10,)), pltpu.SemaphoreType.DMA((NT,)),
            pltpu.SemaphoreType.DMA((2,)), pltpu.SemaphoreType.DMA((2,)), pltpu.SemaphoreType.DMA((NT,)),
        ],
        compiler_params=pltpu.CompilerParams(vmem_limit_bytes=110 * 2**20, flags={"XLA_TPU_EVENLY_DISTRIBUTE_CRITICAL_NODES": True}),
    )(A_x.reshape(S, D), A_wqkv, A_w_phi.reshape(D, DH), A_wo,
      B_w_r.reshape(8, 128), B_w_gate, B_w_up, B_w_down, gate_w.reshape(8, 128))
    return out.reshape(1, S, D)
```

```python
import functools
import jax
import jax.numpy as jnp
import numpy as np
from jax import lax
from jax.experimental import pallas as pl
from jax.experimental.pallas import tpu as pltpu

S, D, H, DH, F = 2048, 1024, 32, 32, 3584
TM = 512
NT = S // TM
HT = TM // 2
HD = D // 2
FG = F // 2
FC = F // NT
LOG2E = 1.4426950408889634
BF = jnp.bfloat16
F32 = jnp.float32


def _nt(a, b):
    return lax.dot_general(a, b, (((1,), (1,)), ((), ())), preferred_element_type=F32)


def _nn(a, b):
    return jnp.dot(a, b, preferred_element_type=F32)


def _red8(x4, op):
    r = x4[:, 0]
    for k in range(1, 8):
        r = op(r, x4[:, k])
    return r


def _rot(r, op):
    r = op(r, pltpu.roll(r, 4, 1))
    return op(r, pltpu.roll(r, 2, 1))


def _dual_softmax_parts(pT):
    n = pT.shape[0] // 64
    p4 = pT.reshape(n, 8, 8, pT.shape[1])
    mx = _rot(_red8(p4, jnp.maximum), jnp.maximum)
    mn = _rot(_red8(p4, jnp.minimum), jnp.minimum)
    ep = jnp.exp2(p4 - mx[:, None])
    en = jnp.exp2(mn[:, None] - p4)
    rp = 1.0 / _rot(_red8(ep, jnp.add), jnp.add)
    rn = 1.0 / _rot(_red8(en, jnp.add), jnp.add)
    return ep, en, rp, rn


def _rowdot(xf, w8):
    acc = xf[:, 0:128] * w8[0:1]
    for k in range(1, 8):
        acc = acc + xf[:, k * 128:(k + 1) * 128] * w8[k:k + 1]
    return jnp.sum(acc, axis=1, keepdims=True)


def _lhs_combos(a11, a12, a21, a22):
    return (a11 + a22, a21 + a22, a11, a22, a11 + a12, a21 - a11, a12 - a22)


def _rhs_combos(b11, b12, b21, b22):
    return (b11 + b22, b11, b12 - b22, b21 - b11, b22, b11 + b12, b21 + b22)


def _assemble(m):
    c11 = m[0] + m[3] - m[4] + m[6]
    c12 = m[2] + m[4]
    c21 = m[1] + m[3]
    c22 = m[0] - m[1] + m[2] + m[5]
    return jnp.concatenate([jnp.concatenate([c11, c12], axis=1), jnp.concatenate([c21, c22], axis=1)], axis=0)


XSLOT = {0: 0, 2: 1, 3: 2, 5: 3, 6: 4}


def kernel(xa_h, wqkv_h, wphi_h, wo_h, wr_h, wg_h, wu_h, wd_h, gw_h, out_h,
           xa, wq, wk, wv, wo, wg, wu, wd, wphi, wr, gw,
           ob, kvacc, zacc, kvt, zb, gb, xsb, gu, hb, yacc, pb, wk7, wv7, wq7, wo7, xc5,
           sem, ksem, xsem, gsem, usem, osem):
    def cp(src, dst, k):
        return pltpu.make_async_copy(src, dst, sem.at[k])

    def xcp(j, r0, n):
        return pltpu.make_async_copy(xa_h.at[pl.ds(r0, n), :], xa.at[pl.ds(r0, n), :], xsem.at[j])

    def gucp(i):
        cs = pl.ds(pl.multiple_of(i * FG, 128), FG)
        return (pltpu.make_async_copy(wg_h.at[:, cs], wg.at[:, cs], gsem.at[i]),
                pltpu.make_async_copy(wu_h.at[:, cs], wu.at[:, cs], usem.at[i]))

    def kcp(g):
        return [pltpu.make_async_copy(wqkv_h.at[:, pl.ds(D + c * 128, 128)], wk.at[:, pl.ds(c * 128, 128)], ksem.at[c])
                for c in (g, g + 4)]

    c_wphi = cp(wphi_h, wphi, 0)
    c_wv = cp(wqkv_h.at[:, pl.ds(2 * D, D)], wv, 1)
    c_wq = cp(wqkv_h.at[:, pl.ds(0, D)], wq, 2)
    c_wr = cp(wr_h, wr, 3)
    c_gw = cp(gw_h, gw, 4)
    c_wo = cp(wo_h, wo, 5)
    c_wd = cp(wd_h, wd, 6)
    c_x = [xcp(0, 0, HT), xcp(1, HT, HT)] + [xcp(1 + t, t * TM, TM) for t in range(1, NT)]
    for c in (c_wphi, *kcp(0), *kcp(1), c_wr, c_gw):
        c.start()

    jj = lax.broadcasted_iota(jnp.int32, (128, DH), 0)
    ff = lax.broadcasted_iota(jnp.int32, (128, DH), 1)
    et = jnp.where(((jj & 63) >> 1) == ff, 1.0, 0.0).astype(BF)
    j2 = lax.broadcasted_iota(jnp.int32, (128, 128), 0)
    c2 = lax.broadcasted_iota(jnp.int32, (128, 128), 1)
    keep = (c2 >> 5) == ((j2 >> 6) * 2 + (j2 & 1))
    kvacc[...] = jnp.zeros_like(kvacc)
    zacc[...] = jnp.zeros_like(zacc)
    yacc[...] = jnp.zeros_like(yacc)
    c_wphi.wait()
    bd = _nt(et, wphi[...])
    bds = [jnp.where(keep, bd[:, g * 128:(g + 1) * 128], 0.0).astype(BF) for g in range(8)]

    def fold7(w_ref, dst, g):
        ta = _nt(bds[g], w_ref[:, g * 128:(g + 1) * 128]) * LOG2E
        tb = _nt(bds[g + 4], w_ref[:, (g + 4) * 128:(g + 5) * 128]) * LOG2E
        for j, c in enumerate(_lhs_combos(ta[:, :HD], ta[:, HD:], tb[:, :HD], tb[:, HD:])):
            dst[j, g * 128:(g + 1) * 128, :] = c.astype(BF)

    nxt = [kcp(2), kcp(3), [c_x[0]], [c_x[1]]]
    for g in range(4):
        for c in kcp(g):
            c.wait()
        for c in nxt[g]:
            c.start()
        fold7(wk, wk7, g)
    c_x[0].wait()
    c_wv.start()
    c_x[1].wait()
    for c in (c_x[2], c_x[3], c_x[4], *gucp(0), c_wo, *gucp(1), c_wq, c_wd):
        c.start()

    def x_combos(t, xf):
        c = _rhs_combos(xf[:HT, :HD], xf[HT:, :HD], xf[:HT, HD:], xf[HT:, HD:])
        for j, s in XSLOT.items():
            xc5[t, s] = c[j].astype(BF)

    def x_operand(t, j):
        r0 = t * TM if isinstance(t, int) else pl.multiple_of(t * TM, TM)
        if j == 1:
            return xa[pl.ds(r0, HT), 0:HD]
        if j == 4:
            return xa[pl.ds(r0 + HT, HT), HD:D]
        return xc5[t, XSLOT[j]]

    def prods(w7, t, js):
        return {j: _nt(w7[j], x_operand(t, j)) for j in js}

    def proj_t(w7, t):
        return _assemble(prods(w7, t, range(7)))

    def phi_k(pT):
        n = pT.shape[0] // 64
        ep, en, rp, rn = _dual_softmax_parts(pT)
        php = (ep * rp[:, None]).reshape(n, 64, TM)
        phn = (en * rn[:, None]).reshape(n, 64, TM)
        ph = jnp.concatenate([php, phn], axis=1)
        zz = ph[:, :, 0:128]
        for c in range(1, TM // 128):
            zz = zz + ph[:, :, c * 128:(c + 1) * 128]
        zacc[...] += zz
        return ph.astype(BF)

    def kv_update(vT, phb):
        for j in range(phb.shape[0]):
            kvacc[j] += _nt(vT[j * 64:(j + 1) * 64], phb[j])

    def router(t, bv, bi, combos=True):
        xf = xa[t * TM:(t + 1) * TM, :].astype(F32)
        if combos:
            x_combos(t, xf)
        gb[t * TM:(t + 1) * TM, :] = jnp.broadcast_to(jax.nn.sigmoid(_rowdot(xf, gw[...].astype(F32))), (TM, 128))
        r = _rowdot(xf, wr[...].astype(F32)).astype(BF).astype(F32)
        r = jnp.broadcast_to(jnp.where(r != r, -jnp.inf, r), (TM, 128))
        row = lax.broadcasted_iota(jnp.int32, (8, 128), 0) + t * TM
        for k in range(TM // 8):
            rk = r[k * 8:(k + 1) * 8]
            better = rk > bv
            bv = jnp.where(better, rk, bv)
            bi = jnp.where(better, row + k * 8, bi)
        return bv, bi

    x_combos(0, xa[0:TM, :].astype(F32))
    mk = prods(wk7, 0, (1, 4, 2, 3))
    c_wv.wait()
    c_x[2].wait()
    c_wr.wait()
    c_gw.wait()
    for g in range(4):
        ta = wv[:, g * 128:(g + 1) * 128].T.astype(F32)
        tb = wv[:, (g + 4) * 128:(g + 5) * 128].T.astype(F32)
        for j, c in enumerate(_lhs_combos(ta[:, :HD], ta[:, HD:], tb[:, :HD], tb[:, HD:])):
            wv7[j, g * 128:(g + 1) * 128, :] = c.astype(BF)
    mk.update(prods(wk7, 0, (0, 6, 5)))
    kv_update(proj_t(wv7, 0).astype(BF), phi_k(_assemble(mk)))
    bv = jnp.full((8, 128), -jnp.inf, F32)
    bi = lax.broadcasted_iota(jnp.int32, (8, 128), 0)
    bv, bi = router(0, bv, bi, combos=False)
    bv, bi = router(1, bv, bi)

    def p1_tile(t):
        kv_update(proj_t(wv7, t).astype(BF), phi_k(proj_t(wk7, t)))

    c_x[3].wait()
    c_x[4].wait()
    p1_tile(1)
    bv, bi = router(2, bv, bi)
    bv, bi = router(3, bv, bi)

    rmax = jnp.max(bv, axis=0, keepdims=True)
    idx = jnp.min(jnp.where(bv == rmax, bi, S))
    rsel = jax.nn.sigmoid(rmax)
    base = pl.multiple_of((idx >> 4) << 4, 16)
    rows = lax.broadcasted_iota(jnp.int32, (16, D), 0)
    blk = xa[pl.ds(base, 16), :].astype(F32)
    xs = jnp.sum(jnp.where(rows == idx - base, blk, 0.0), axis=0, keepdims=True)
    xsb[...] = jnp.broadcast_to(xs, (128, D)).T
    never = idx < 0
    c_wo.wait()

    def p1(i, carry):
        for c in gucp(i):
            c.wait()
        for c in range(FG // 128):
            cs = pl.ds(pl.multiple_of(i * FG + c * 128, 128), 128)
            ag = jnp.zeros((8, 128), F32) if c == 0 else jnp.where(never, ag, 0.0)
            au = jnp.zeros((8, 128), F32) if c == 0 else jnp.where(never, au, 0.0)
            for k in range(D // 16):
                ks = slice(k * 16, (k + 1) * 16)
                xk = xsb[ks, :]
                tg = wg[ks, cs].astype(F32) * xk
                tu = wu[ks, cs].astype(F32) * xk
                ag = ag + tg[0:8] + tg[8:16]
                au = au + tu[0:8] + tu[8:16]
            gu[0:8, cs] = ag
            gu[8:16, cs] = au
        for q in range(HD // 2 // 16):
            ra = pl.ds(pl.multiple_of(i * (HD // 2) + q * 16, 16), 16)
            rb = pl.ds(pl.multiple_of(HD + i * (HD // 2) + q * 16, 16), 16)
            ta = wo[ra, :].astype(F32)
            tb = wo[rb, :].astype(F32)
            for j, c in enumerate(_rhs_combos(ta[:, :HD], ta[:, HD:], tb[:, :HD], tb[:, HD:])):
                if j not in (1, 4):
                    wo7[XSLOT[j], ra, :] = c.astype(BF)
        p1_tile(i + 2)
        return carry

    lax.fori_loop(0, 2, p1, 0)

    c_wq.wait()
    c_wd.wait()
    r3 = lax.broadcasted_iota(jnp.int32, (16, 64, 128), 1)
    c3 = lax.broadcasted_iota(jnp.int32, (16, 64, 128), 2)
    kvt[...] = jnp.where((r3 >> 5) == (c3 & 1), kvacc[...], 0.0).astype(BF)
    zb[...] = jnp.broadcast_to(jnp.sum(zacc[...], axis=2, keepdims=True), zb.shape)
    for g in range(4):
        fold7(wq, wq7, g)
    gg = jnp.sum(gu[0:8, :], axis=0, keepdims=True)
    uu = jnp.sum(gu[8:16, :], axis=0, keepdims=True)
    hb[...] = jnp.broadcast_to(gg * jax.nn.sigmoid(gg) * uu, (128, F)).T
    t0 = idx // TM

    def ocp(t, i):
        r0 = pl.multiple_of(t * TM, TM)
        return pltpu.make_async_copy(ob.at[pl.ds(r0, TM), :], out_h.at[pl.ds(r0, TM), :], osem.at[i])

    def wo_operand(j):
        if j == 1:
            return wo[0:HD, 0:HD]
        if j == 4:
            return wo[HD:D, HD:D]
        return wo7[XSLOT[j]]

    def p2(i, carry):
        t = (t0 + i) % NT
        r0 = pl.multiple_of(t * TM, TM)
        fs = pl.ds(pl.multiple_of(i * FC, 128), FC)
        wdc = wd.at[fs, :]
        hbc = hb.at[fs, :]
        acc = jnp.zeros((8, 128), F32)
        for c in range(D // 128):
            acc = jnp.where(never, acc, 0.0)
            for k in range(FC // 16):
                tt = wdc[k * 16:(k + 1) * 16, c * 128:(c + 1) * 128].astype(F32) * hbc[k * 16:(k + 1) * 16, :]
                acc = acc + tt[0:8]
                acc = acc + tt[8:16]
            yacc[:, c * 128:(c + 1) * 128] += acc

        pT = proj_t(wq7, t)
        ep, en, rp, rn = _dual_softmax_parts(pT)
        z4 = zb[...].reshape(16, 2, 8, 8, 128)
        zp = jnp.concatenate([z4[:, 0]] * (TM // 128), axis=-1)
        zn = jnp.concatenate([z4[:, 1]] * (TM // 128), axis=-1)
        den = _rot(_red8(ep * zp, jnp.add) * rp + _red8(en * zn, jnp.add) * rn, jnp.add) + 1e-6
        rd = 1.0 / den
        php = (ep * (rp * rd)[:, None]).reshape(16, 64, TM)
        phn = (en * (rn * rd)[:, None]).reshape(16, 64, TM)
        phb = jnp.concatenate([php, phn], axis=1).astype(BF)
        oT = jnp.concatenate([_nn(kvt[j], phb[j]) for j in range(16)], axis=0)
        oc = _lhs_combos(oT[:HD, :HT], oT[HD:, :HT], oT[:HD, HT:], oT[HD:, HT:])
        a = _assemble([_nn(oc[j].astype(BF).T, wo_operand(j)) for j in range(7)])
        g = jnp.concatenate([gb[pl.ds(r0, TM), :]] * (D // 128), axis=1)
        ob[pl.ds(r0, TM), :] = (g * a + (1.0 - g) * xa[pl.ds(r0, TM), :].astype(F32)).astype(BF)
        ocp(t, i).start()
        return carry

    lax.fori_loop(0, NT, p2, 0)
    y = jnp.sum(yacc[...], axis=0, keepdims=True) * jnp.concatenate([rsel] * 8, axis=1)
    gsel = jnp.concatenate([gb[pl.ds(base, 16), :]] * (D // 128), axis=1)
    ocp(t0, 0).wait()
    old = ob[pl.ds(base, 16), :].astype(F32)
    pb[...] = jnp.where(rows == idx - base, old + (1.0 - gsel) * y, old).astype(BF)
    c_patch = cp(pb, out_h.at[pl.ds(base, 16), :], 7)
    c_patch.start()
    for i in range(1, NT):
        ocp((t0 + i) % NT, i).wait()
    c_patch.wait()


@jax.jit
def pallas_gated_mix__linear_kernel_hedgehog__moe_arch_mod__prompt_kernel(
        A_x, A_wqkv, A_w_phi, A_wo, B_x, B_w_r, B_w_gate, B_w_up, B_w_down, gate_w):
    anyspec = pl.BlockSpec(memory_space=pl.ANY)
    V = pltpu.VMEM
    DMA = pltpu.SemaphoreType.DMA
    out = pl.pallas_call(
        kernel,
        out_shape=jax.ShapeDtypeStruct((S, D), BF),
        in_specs=[anyspec] * 9,
        out_specs=anyspec,
        scratch_shapes=[
            V((S, D), BF), V((D, D), BF), V((D, D), BF), V((D, D), BF), V((D, D), BF),
            V((D, F), BF), V((D, F), BF), V((F, D), BF),
            V((D, DH), BF), V((8, 128), BF), V((8, 128), BF),
            V((S, D), BF), V((16, 64, 128), F32), V((16, 128, 128), F32),
            V((16, 64, 128), BF), V((16, 128, 128), F32), V((S, 128), F32),
            V((D, 128), F32), V((16, F), F32), V((F, 128), F32), V((8, D), F32), V((16, D), BF),
            V((7, HD, HD), BF), V((7, HD, HD), BF), V((7, HD, HD), BF), V((5, HD, HD), BF),
            V((NT, 5, HT, HD), BF),
            DMA((8,)), DMA((8,)), DMA((NT + 1,)), DMA((2,)), DMA((2,)), DMA((NT,)),
        ],
        compiler_params=pltpu.CompilerParams(vmem_limit_bytes=110 * 2**20, flags={"XLA_TPU_EVENLY_DISTRIBUTE_CRITICAL_NODES": True}),
    )(A_x.reshape(S, D), A_wqkv, A_w_phi.reshape(D, DH), A_wo,
      B_w_r.reshape(8, 128), B_w_gate, B_w_up, B_w_down, gate_w.reshape(8, 128))
    return out.reshape(1, S, D)
```

```python
import functools
import jax
import jax.numpy as jnp
import numpy as np
from jax import lax
from jax.experimental import pallas as pl
from jax.experimental.pallas import tpu as pltpu

S, D, H, DH, F = 2048, 1024, 32, 32, 3584
TM = 512
NT = S // TM
HT = TM // 2
HD = D // 2
GCUT = (0, 384, 1920, 3072, F)
DCUT = (0, 1792, F)
LOG2E = 1.4426950408889634
BF = jnp.bfloat16
F32 = jnp.float32
U32 = jnp.uint32
QUADS = ((0, HD), (HT, 0), (0, 0), (HT, HD))


def _nt(a, b):
    return lax.dot_general(a, b, (((1,), (1,)), ((), ())), preferred_element_type=F32)


def _nn(a, b):
    return jnp.dot(a, b, preferred_element_type=F32)


def _red8(x4, op):
    r = x4[:, 0]
    for k in range(1, 8):
        r = op(r, x4[:, k])
    return r


def _rot(r, op):
    r = op(r, pltpu.roll(r, 4, 1))
    return op(r, pltpu.roll(r, 2, 1))


def _pack(even, odd):
    return pltpu.bitcast(pltpu.pack_elementwise([even, odd], packed_dtype=BF), U32)


def _planes(x):
    w = pltpu.bitcast(x, U32)
    return [pltpu.unpack_elementwise(w, index=i, packed_dtype=BF, unpacked_dtype=F32) for i in range(2)]


def _unpack(x):
    return pltpu.bitcast(x, BF)


def _rcp(x):
    r = pl.reciprocal(x, approx=True)
    return r * (2.0 - x * r)


def _dual_softmax_parts(pT):
    n = pT.shape[0] // 64
    p4 = pT.reshape(n, 8, 8, pT.shape[1])
    mx = _rot(_red8(p4, jnp.maximum), jnp.maximum)
    mn = _rot(_red8(p4, jnp.minimum), jnp.minimum)
    ep = jnp.exp2(p4 - mx[:, None])
    en = jnp.exp2(mn[:, None] - p4)
    rp = _rcp(_rot(_red8(ep, jnp.add), jnp.add))
    rn = _rcp(_rot(_red8(en, jnp.add), jnp.add))
    return ep, en, rp, rn


def _rowdot(xf, w8):
    acc = xf[:, 0:128] * w8[0:1]
    for k in range(1, 8):
        acc = acc + xf[:, k * 128:(k + 1) * 128] * w8[k:k + 1]
    return jnp.sum(acc, axis=1, keepdims=True)


def _lhs_combos(a11, a12, a21, a22):
    return (a11 + a22, a21 + a22, a11, a22, a11 + a12, a21 - a11, a12 - a22)


def _rhs_combos(b11, b12, b21, b22):
    return (b11 + b22, b11, b12 - b22, b21 - b11, b22, b11 + b12, b21 + b22)


def _assemble(m):
    c11 = m[0] + m[3] - m[4] + m[6]
    c12 = m[2] + m[4]
    c21 = m[1] + m[3]
    c22 = m[0] - m[1] + m[2] + m[5]
    return jnp.concatenate([jnp.concatenate([c11, c12], axis=1), jnp.concatenate([c21, c22], axis=1)], axis=0)


def kernel(xa_h, wqkv_h, wphi_h, wo_h, wr_h, wg_h, wu_h, wd_h, gw_h, out_h,
           xa, wq, wk, wv, wo, wg, wu, wd, wphi, wr, gw, bdt,
           ob, kvacc, zacc, kvt, zb, gb, xsb, gu, hb, yacc, pb, wk7, wv7, wq7, wo7, xc7, fence,
           sem, ksem, xsem, gsem, usem, dsem, osem, fsem):
    def cp(src, dst, k):
        return pltpu.make_async_copy(src, dst, sem.at[k])

    def xcp(j, r0, n):
        return pltpu.make_async_copy(xa_h.at[pl.ds(r0, n), :], xa.at[pl.ds(r0, n), :], xsem.at[j])

    def gucp(i):
        cs = pl.ds(GCUT[i], GCUT[i + 1] - GCUT[i])
        return (pltpu.make_async_copy(wg_h.at[:, cs], wg.at[:, cs], gsem.at[i]),
                pltpu.make_async_copy(wu_h.at[:, cs], wu.at[:, cs], usem.at[i]))

    def dcp(i):
        rs = pl.ds(DCUT[i], DCUT[i + 1] - DCUT[i])
        return pltpu.make_async_copy(wd_h.at[rs, :], wd.at[rs, :], dsem.at[i])

    def kcp(g):
        return [pltpu.make_async_copy(wqkv_h.at[:, pl.ds(D + c * 128, 128)], wk.at[:, pl.ds(c * 128, 128)], ksem.at[c])
                for c in (g, g + 4)]

    def ocp(t):
        return pltpu.make_async_copy(ob.at[pl.ds(t * TM, TM), :], out_h.at[pl.ds(t * TM, TM), :], osem.at[t])

    def qcp(q):
        rs, cs = pl.ds((NT - 1) * TM + QUADS[q][0], HT), pl.ds(QUADS[q][1], HD)
        return pltpu.make_async_copy(ob.at[rs, cs], out_h.at[rs, cs], osem.at[NT - 1 + q])

    def fcp(i):
        return pltpu.make_async_copy(wr_h, fence.at[i], fsem.at[i])

    def start(*cs):
        for c in cs:
            c.start()

    def wait(*cs):
        for c in cs:
            c.wait()

    c_wphi = cp(wphi_h, wphi, 0)
    c_wv = cp(wqkv_h.at[:, pl.ds(2 * D, D)], wv, 1)
    c_wq = cp(wqkv_h.at[:, pl.ds(0, D)], wq, 2)
    c_wr = cp(wr_h, wr, 3)
    c_gw = cp(gw_h, gw, 4)
    c_wo = cp(wo_h, wo, 5)
    c_x = [xcp(0, 0, HT), xcp(1, HT, HT)] + [xcp(1 + t, t * TM, TM) for t in range(1, NT)]

    def fold7(w_ref, dst, g):
        ta = _nt(bdt[:, g * 128:(g + 1) * 128], w_ref[:, g * 128:(g + 1) * 128]) * LOG2E
        tb = _nt(bdt[:, (g + 4) * 128:(g + 5) * 128], w_ref[:, (g + 4) * 128:(g + 5) * 128]) * LOG2E
        for j, c in enumerate(_lhs_combos(ta[:, :HD], ta[:, HD:], tb[:, :HD], tb[:, HD:])):
            for p in range(2):
                dst[j, g * 64 + p * DH:g * 64 + (p + 1) * DH, :] = _pack(c[p * 64:p * 64 + DH], c[p * 64 + DH:(p + 1) * 64])

    def prep_wv():
        for g in range(4):
            ta = _planes(wv[:, g * 128:(g + 1) * 128].T)
            tb = _planes(wv[:, (g + 4) * 128:(g + 5) * 128].T)
            cs = [_lhs_combos(u[:, :HD], u[:, HD:], v[:, :HD], v[:, HD:]) for u, v in zip(ta, tb)]
            for j in range(7):
                wv7[j, g * 64:(g + 1) * 64, :] = _pack(cs[0][j], cs[1][j])

    def rhs7(src, r0, nr, dst, swap, never=None):
        prev = None
        for q in range(nr // 16):
            ra = slice(r0 + q * 16, r0 + (q + 1) * 16)
            rb = slice(r0 + nr + q * 16, r0 + nr + (q + 1) * 16)
            rd = slice(q * 8, (q + 1) * 8)
            for c in range(HD // 128):
                ca = slice(c * 128, (c + 1) * 128)
                cb = slice(HD + c * 128, HD + (c + 1) * 128)
                r11, r22 = src[ra, ca], src[rb, cb]
                dst[1, rd, ca] = pltpu.bitcast(r11, U32)
                dst[4, rd, ca] = pltpu.bitcast(r22, U32)
                b11, b12, b21, b22 = _planes(r11), _planes(src[rb, ca]), _planes(src[ra, cb]), _planes(r22)
                if swap:
                    b12, b21 = b21, b12
                for s, u, v, op in ((0, b11, b22, jnp.add), (2, b12, b22, jnp.subtract), (3, b21, b11, jnp.subtract),
                                    (5, b11, b12, jnp.add), (6, b21, b22, jnp.add)):
                    u0 = u[0] if never is None or prev is None else jnp.where(never, prev, u[0])
                    u1 = u[1] if never is None or prev is None else jnp.where(never, prev, u[1])
                    prev = op(u0, v[0])
                    dst[s, rd, ca] = _pack(prev, op(u1, v[1]))

    def prep_x(t, never=None):
        rhs7(xa, t * TM, HT, xc7.at[t], False, never)

    def prep_wo(never=None):
        rhs7(wo, 0, HD, wo7, True, never)

    def x_operand(t, j):
        return _unpack(xc7[t, j])

    def wo_operand(j):
        return _unpack(wo7[j])

    def proj_t(w7, t):
        return _assemble([_nt(_unpack(w7[j]), x_operand(t, j)) for j in range(7)])

    def prods(w7, t, js):
        return {j: _nt(_unpack(w7[j]), x_operand(t, j)) for j in js}

    def phi_k(t, pT):
        ep, en, rp, rn = _dual_softmax_parts(pT)
        php = (ep * rp[:, None]).reshape(16, 64, TM)
        phn = (en * rn[:, None]).reshape(16, 64, TM)
        ph = jnp.concatenate([php, phn], axis=1)
        zz = ph[:, :, 0:128]
        for c in range(1, TM // 128):
            zz = zz + ph[:, :, c * 128:(c + 1) * 128]
        zacc[...] = zz if t == 0 else zacc[...] + zz
        return ph.astype(BF)

    def kv_accumulate(t, vT, phb):
        vT = vT.astype(BF)
        for j in range(16):
            u = _nt(vT[j * 64:(j + 1) * 64], phb[j])
            kvacc[j] = u if t == 0 else kvacc[j] + u

    def kv_update(t):
        kv_accumulate(t, proj_t(wv7, t), phi_k(t, proj_t(wk7, t)))

    def gate(t):
        xf = xa[t * TM:(t + 1) * TM, :].astype(F32)
        gb[t * TM:(t + 1) * TM, :] = jnp.broadcast_to(jax.nn.sigmoid(_rowdot(xf, gw[...].astype(F32))), (TM, 128))

    def router(t, bv, bi, with_gate=True):
        xf = xa[t * TM:(t + 1) * TM, :].astype(F32)
        if with_gate:
            gate(t)
        r = _rowdot(xf, wr[...].astype(F32)).astype(BF).astype(F32)
        r = jnp.broadcast_to(jnp.where(r != r, -jnp.inf, r), (TM, 128))
        row = lax.broadcasted_iota(jnp.int32, (8, 128), 0) + t * TM
        for k in range(TM // 8):
            rk = r[k * 8:(k + 1) * 8]
            better = rk > bv
            bv = jnp.where(better, rk, bv)
            bi = jnp.where(better, row + k * 8, bi)
        return bv, bi

    def gate_up(lo, hi, never=None):
        acc = None
        for c0 in range(GCUT[lo], GCUT[hi], 128):
            for m, w_ref in enumerate((wg, wu)):
                acc = jnp.zeros((8, 128), F32) if acc is None or never is None else jnp.where(never, acc, 0.0)
                for k in range(D // 16):
                    t = w_ref[k * 16:(k + 1) * 16, c0:c0 + 128].astype(F32) * xsb[k * 16:(k + 1) * 16, :]
                    acc = acc + t[0:8]
                    acc = acc + t[8:16]
                gu[m * 8:(m + 1) * 8, c0:c0 + 128] = acc

    def hidden():
        gg = jnp.sum(gu[0:8, :], axis=0, keepdims=True)
        uu = jnp.sum(gu[8:16, :], axis=0, keepdims=True)
        hb[...] = jnp.broadcast_to(gg * jax.nn.sigmoid(gg) * uu, (128, F)).T

    def down(i, never):
        acc = None
        for c in range(D // 128):
            acc = jnp.zeros((8, 128), F32) if acc is None else jnp.where(never, acc, 0.0)
            for k in range(DCUT[i] // 16, DCUT[i + 1] // 16):
                t = wd[k * 16:(k + 1) * 16, c * 128:(c + 1) * 128].astype(F32) * hb[k * 16:(k + 1) * 16, :]
                acc = acc + t[0:8]
                acc = acc + t[8:16]
            cs = slice(c * 128, (c + 1) * 128)
            yacc[:, cs] = acc if i == 0 else yacc[:, cs] + acc

    def finalize_kv():
        r3 = lax.broadcasted_iota(jnp.int32, (16, 64, 128), 1)
        c3 = lax.broadcasted_iota(jnp.int32, (16, 64, 128), 2)
        kvt[...] = pltpu.bitcast(jnp.where((r3 >> 5) == (c3 & 1), kvacc[...], 0.0).reshape(D, 128).astype(BF), U32)
        zb[...] = jnp.broadcast_to(jnp.sum(zacc[...], axis=2, keepdims=True), zb.shape)

    def attend(t, y, idx):
        ep, en, rp, rn = _dual_softmax_parts(proj_t(wq7, t))
        z4 = zb[...].reshape(16, 2, 8, 8, 128)
        zp = jnp.concatenate([z4[:, 0]] * (TM // 128), axis=-1)
        zn = jnp.concatenate([z4[:, 1]] * (TM // 128), axis=-1)
        den = _rot(_red8(ep * zp, jnp.add) * rp + _red8(en * zn, jnp.add) * rn, jnp.add) + 1e-6
        rd = _rcp(den)
        php = (ep * (rp * rd)[:, None]).reshape(16, 64, TM)
        phn = (en * (rn * rd)[:, None]).reshape(16, 64, TM)
        phb = jnp.concatenate([php, phn], axis=1).astype(BF)
        oT = jnp.concatenate([_nn(_unpack(kvt[j * 32:(j + 1) * 32, :]), phb[j]) for j in range(16)], axis=0)
        oc = _lhs_combos(oT[:HD, :HT], oT[HD:, :HT], oT[:HD, HT:], oT[HD:, HT:])
        r0 = t * TM
        a = _assemble([_nn(oc[j].astype(BF).T, wo_operand(j)) for j in range(7)])
        g = jnp.concatenate([gb[r0:r0 + TM, :]] * (D // 128), axis=1)
        b = xa[r0:r0 + TM, :].astype(F32)
        if y is not None:
            b = jnp.where(lax.broadcasted_iota(jnp.int32, (TM, D), 0) == idx - r0, b + y, b)
        res = (g * a + (1.0 - g) * b).astype(BF)
        if t < NT - 1:
            ob[r0:r0 + TM, :] = res
            ocp(t).start()
        else:
            for q, (rq, cq) in enumerate(QUADS):
                ob[r0 + rq:r0 + rq + HT, cq:cq + HD] = res[rq:rq + HT, cq:cq + HD]
                qcp(q).start()

    start(c_wphi, *kcp(0), *kcp(1), c_wr, c_gw, *[fcp(i) for i in range(5)])
    jj = lax.broadcasted_iota(jnp.int32, (128, DH), 0)
    ff = lax.broadcasted_iota(jnp.int32, (128, DH), 1)
    et = jnp.where((jj & (DH - 1)) == ff, 1.0, 0.0).astype(BF)
    j2 = lax.broadcasted_iota(jnp.int32, (128, 128), 0)
    c2 = lax.broadcasted_iota(jnp.int32, (128, 128), 1)
    keep = (c2 >> 5) == (j2 >> 5)
    wait(c_wphi)
    bd = _nt(et, wphi[...])
    for g in range(8):
        bdt[:, g * 128:(g + 1) * 128] = jnp.where(keep, bd[:, g * 128:(g + 1) * 128], 0.0).astype(BF)

    never0 = jnp.max(jnp.where(bd[0:8, 0:128] > 0.0, 1, 0)) < 0
    nxt = [kcp(2), kcp(3), [c_x[0]], [c_x[1]]]
    for g in range(4):
        wait(kcp(g)[0])
        start(*nxt[g])
        wait(kcp(g)[1])
        fold7(wk, wk7, g)
    wait(c_x[0])
    start(c_wv)
    wait(c_x[1])
    wait(c_wr, c_gw)
    prep_x(0)
    mk = prods(wk7, 0, (1, 4, 2, 3, 0))
    bv = jnp.full((8, 128), -jnp.inf, F32)
    bi = lax.broadcasted_iota(jnp.int32, (8, 128), 0)
    bv, bi = router(0, bv, bi)
    wait(c_wv)
    start(c_x[2], c_x[3], c_x[4], *gucp(0))
    wait(fcp(0))
    prep_wv()
    mk.update(prods(wk7, 0, (6, 5)))
    kv_accumulate(0, proj_t(wv7, 0), phi_k(0, _assemble(mk)))
    wait(c_x[2], c_x[3])
    start(*gucp(1))
    wait(c_x[4])
    prep_x(1)
    kv_update(1)
    prep_x(2, never0)
    for t in range(1, NT):
        bv, bi = router(t, bv, bi)
    rmax = jnp.max(bv, axis=0, keepdims=True)
    idx = jnp.min(jnp.where(bv == rmax, bi, S))
    rsel = jax.nn.sigmoid(rmax)
    base = pl.multiple_of((idx >> 4) << 4, 16)
    rows = lax.broadcasted_iota(jnp.int32, (16, D), 0)
    blk = xa[pl.ds(base, 16), :].astype(F32)
    xs = jnp.sum(jnp.where(rows == idx - base, blk, 0.0), axis=0, keepdims=True)
    xsb[...] = jnp.broadcast_to(xs, (128, D)).T
    never = idx < 0
    wait(*gucp(0), *gucp(1))
    start(c_wo, *gucp(2))
    wait(fcp(1))
    kv_update(2)
    prep_x(3, never)
    gate_up(0, 2, never)
    wait(c_wo, *gucp(2))
    start(c_wq, *gucp(3))
    wait(fcp(2))
    kv_update(3)
    prep_wo(never)
    gate_up(2, 3, never)
    wait(c_wq, *gucp(3))
    start(dcp(0), dcp(1))
    wait(fcp(3))
    for g in range(4):
        fold7(wq, wq7, g)
    gate_up(3, 4)
    wait(fcp(4))
    finalize_kv()
    hidden()
    attend(0, None, None)
    wait(dcp(0), dcp(1))
    attend(1, None, None)
    down(0, never)
    wait(ocp(0))
    attend(2, None, None)
    down(1, never)
    wait(ocp(1))
    y = jnp.sum(yacc[...], axis=0, keepdims=True) * jnp.concatenate([rsel] * 8, axis=1)
    attend(3, y, idx)
    wait(ocp(2))

    @pl.when(idx < (NT - 1) * TM)
    def _():
        gsel = jnp.concatenate([gb[pl.ds(base, 16), :]] * (D // 128), axis=1)
        old = ob[pl.ds(base, 16), :].astype(F32)
        pb[...] = jnp.where(rows == idx - base, old + (1.0 - gsel) * y, old).astype(BF)
        c_patch = cp(pb, out_h.at[pl.ds(base, 16), :], 7)
        c_patch.start()
        c_patch.wait()

    wait(*[qcp(q) for q in range(4)])


@jax.jit
def pallas_gated_mix__linear_kernel_hedgehog__moe_arch_mod__prompt_kernel(
        A_x, A_wqkv, A_w_phi, A_wo, B_x, B_w_r, B_w_gate, B_w_up, B_w_down, gate_w):
    anyspec = pl.BlockSpec(memory_space=pl.ANY)
    V = pltpu.VMEM
    DMA = pltpu.SemaphoreType.DMA
    out = pl.pallas_call(
        kernel,
        out_shape=jax.ShapeDtypeStruct((S, D), BF),
        in_specs=[anyspec] * 9,
        out_specs=anyspec,
        scratch_shapes=[
            V((S, D), BF), V((D, D), BF), V((D, D), BF), V((D, D), BF), V((D, D), BF),
            V((D, F), BF), V((D, F), BF), V((F, D), BF),
            V((D, DH), BF), V((8, 128), BF), V((8, 128), BF), V((128, D), BF),
            V((S, D), BF), V((16, 64, 128), F32), V((16, 128, 128), F32),
            V((D // 2, 128), U32), V((16, 128, 128), F32), V((S, 128), F32),
            V((D, 128), F32), V((16, F), F32), V((F, 128), F32), V((8, D), F32), V((16, D), BF),
            V((7, HD // 2, HD), U32), V((7, HD // 2, HD), U32), V((7, HD // 2, HD), U32), V((7, HD // 2, HD), U32),
            V((NT, 7, HT // 2, HD), U32), V((5, 8, 128), BF),
            DMA((8,)), DMA((8,)), DMA((NT + 1,)), DMA((4,)), DMA((4,)), DMA((2,)), DMA((NT + 3,)), DMA((5,)),
        ],
        compiler_params=pltpu.CompilerParams(vmem_limit_bytes=110 * 2**20, flags={"XLA_TPU_EVENLY_DISTRIBUTE_CRITICAL_NODES": True}),
    )(A_x.reshape(S, D), A_wqkv, A_w_phi.reshape(D, DH), A_wo,
      B_w_r.reshape(8, 128), B_w_gate, B_w_up, B_w_down, gate_w.reshape(8, 128))
    return out.reshape(1, S, D)
```

```python
import functools
import jax
import jax.numpy as jnp
import numpy as np
from jax import lax
from jax.experimental import pallas as pl
from jax.experimental.pallas import tpu as pltpu

S, D, H, DH, F = 2048, 1024, 32, 32, 3584
TM = 512
NT = S // TM
HT = TM // 2
HD = D // 2
GDMA = (0, 1024, 1792, 2304, F)
UDMA = (0, 1792, F)
GCUT = (0, 1792, F)
DCUT = (0, 1792, F)
LOG2E = 1.4426950408889634
BF = jnp.bfloat16
F32 = jnp.float32
U32 = jnp.uint32
PIECES = ((0, HD, HD), (HT, 0, HD), (HT, HD, 256), (HT, HD + 256, 256), (0, 0, 128), (0, 128, 128), (0, 256, 128), (0, 384, 128))
PORD = (2, 4, 1, 3, 0, 6, 5)
OORD = (2, 4, 5, 1, 3, 0, 6)


def _nt(a, b):
    return lax.dot_general(a, b, (((1,), (1,)), ((), ())), preferred_element_type=F32)


def _nn(a, b):
    return jnp.dot(a, b, preferred_element_type=F32)


def _red8(x4, op):
    r = x4[:, 0]
    for k in range(1, 8):
        r = op(r, x4[:, k])
    return r


def _rot(r, op):
    r = op(r, pltpu.roll(r, 4, 1))
    return op(r, pltpu.roll(r, 2, 1))


def _pack(even, odd):
    return pltpu.bitcast(pltpu.pack_elementwise([even, odd], packed_dtype=BF), U32)


def _planes(x):
    w = pltpu.bitcast(x, U32)
    return [pltpu.unpack_elementwise(w, index=i, packed_dtype=BF, unpacked_dtype=F32) for i in range(2)]


def _unpack(x):
    return pltpu.bitcast(x, BF)


def _rcp(x):
    r = pl.reciprocal(x, approx=True)
    return r * (2.0 - x * r)


def _dual_softmax_parts(pT):
    n = pT.shape[0] // 64
    p4 = pT.reshape(n, 8, 8, pT.shape[1])
    mx = _rot(_red8(p4, jnp.maximum), jnp.maximum)
    mn = _rot(_red8(p4, jnp.minimum), jnp.minimum)
    ep = jnp.exp2(p4 - mx[:, None])
    en = jnp.exp2(mn[:, None] - p4)
    rp = _rcp(_rot(_red8(ep, jnp.add), jnp.add))
    rn = _rcp(_rot(_red8(en, jnp.add), jnp.add))
    return ep, en, rp, rn


def _rowdot(xf, w8):
    acc = xf[:, 0:128] * w8[0:1]
    for k in range(1, 8):
        acc = acc + xf[:, k * 128:(k + 1) * 128] * w8[k:k + 1]
    return jnp.sum(acc, axis=1, keepdims=True)


def _lhs_combos(a11, a12, a21, a22):
    return (a11 + a22, a21 + a22, a11, a22, a11 + a12, a21 - a11, a12 - a22)


def _rhs_combos(b11, b12, b21, b22):
    return (b11 + b22, b11, b12 - b22, b21 - b11, b22, b11 + b12, b21 + b22)


def _assemble(m):
    c11 = m[0] + m[3] - m[4] + m[6]
    c12 = m[2] + m[4]
    c21 = m[1] + m[3]
    c22 = m[0] - m[1] + m[2] + m[5]
    return jnp.concatenate([jnp.concatenate([c11, c12], axis=1), jnp.concatenate([c21, c22], axis=1)], axis=0)


def kernel(xa_h, wqkv_h, wphi_h, wo_h, wr_h, wg_h, wu_h, wd_h, gw_h, out_h,
           xa, wq, wk, wv, wo, wg, wu, wd, wphi, wr, gw, bdt,
           ob, kvacc, zacc, kvt, zb, gb, xsb, gu, hb, yacc, pb, wk7, wv7, wq7, wo7, xc7, fence,
           sem, ksem, xsem, gsem, usem, dsem, osem, fsem):
    def cp(src, dst, k):
        return pltpu.make_async_copy(src, dst, sem.at[k])

    def xcp(j, r0, n):
        return pltpu.make_async_copy(xa_h.at[pl.ds(r0, n), :], xa.at[pl.ds(r0, n), :], xsem.at[j])

    def gcp(i):
        cs = pl.ds(GDMA[i], GDMA[i + 1] - GDMA[i])
        return pltpu.make_async_copy(wg_h.at[:, cs], wg.at[:, cs], gsem.at[i])

    def ucp(i):
        cs = pl.ds(UDMA[i], UDMA[i + 1] - UDMA[i])
        return pltpu.make_async_copy(wu_h.at[:, cs], wu.at[:, cs], usem.at[i])

    def dcp(i):
        rs = pl.ds(DCUT[i], DCUT[i + 1] - DCUT[i])
        return pltpu.make_async_copy(wd_h.at[rs, :], wd.at[rs, :], dsem.at[i])

    def kcp(g):
        return [pltpu.make_async_copy(wqkv_h.at[:, pl.ds(D + c * 128, 128)], wk.at[:, pl.ds(c * 128, 128)], ksem.at[g])
                for c in (g, g + 4)]

    def ocp(t):
        return pltpu.make_async_copy(ob.at[pl.ds(t * TM, TM), :], out_h.at[pl.ds(t * TM, TM), :], osem.at[t])

    def qcp(q):
        rs, cs = pl.ds((NT - 1) * TM + PIECES[q][0], HT), pl.ds(*PIECES[q][1:])
        return pltpu.make_async_copy(ob.at[rs, cs], out_h.at[rs, cs], osem.at[NT - 1])

    def fcp(i):
        return pltpu.make_async_copy(wr_h, fence.at[i], fsem.at[i])

    def start(*cs):
        for c in cs:
            c.start()

    def wait(*cs):
        for c in cs:
            c.wait()

    c_wphi = cp(wphi_h, wphi, 0)
    c_wv = cp(wqkv_h.at[:, pl.ds(2 * D, D)], wv, 1)
    c_wq = cp(wqkv_h.at[:, pl.ds(0, D)], wq, 2)
    c_wr = cp(wr_h, wr, 3)
    c_gw = cp(gw_h, gw, 4)
    c_wo = cp(wo_h, wo, 5)
    c_x = [xcp(0, 0, HT), xcp(1, HT, HT)] + [xcp(1 + t, t * TM, TM) for t in range(1, NT)]

    def fold7(w_ref, dst, g):
        ta = _nt(bdt[:, g * 128:(g + 1) * 128], w_ref[:, g * 128:(g + 1) * 128]) * LOG2E
        tb = _nt(bdt[:, (g + 4) * 128:(g + 5) * 128], w_ref[:, (g + 4) * 128:(g + 5) * 128]) * LOG2E
        for j, c in enumerate(_lhs_combos(ta[:, :HD], ta[:, HD:], tb[:, :HD], tb[:, HD:])):
            for p in range(2):
                dst[j, g * 64 + p * DH:g * 64 + (p + 1) * DH, :] = _pack(c[p * 64:p * 64 + DH], c[p * 64 + DH:(p + 1) * 64])

    def prep_wv():
        for g in range(4):
            ta = _planes(wv[:, g * 128:(g + 1) * 128].T)
            tb = _planes(wv[:, (g + 4) * 128:(g + 5) * 128].T)
            cs = [_lhs_combos(u[:, :HD], u[:, HD:], v[:, :HD], v[:, HD:]) for u, v in zip(ta, tb)]
            for j in range(7):
                wv7[j, g * 64:(g + 1) * 64, :] = _pack(cs[0][j], cs[1][j])

    def rhs7(src, r0, nr, dst, swap, never=None):
        prev = None
        for q in range(nr // 16):
            ra = slice(r0 + q * 16, r0 + (q + 1) * 16)
            rb = slice(r0 + nr + q * 16, r0 + nr + (q + 1) * 16)
            rd = slice(q * 8, (q + 1) * 8)
            for c in range(HD // 128):
                ca = slice(c * 128, (c + 1) * 128)
                cb = slice(HD + c * 128, HD + (c + 1) * 128)
                r11, r22 = src[ra, ca], src[rb, cb]
                dst[1, rd, ca] = pltpu.bitcast(r11, U32)
                dst[4, rd, ca] = pltpu.bitcast(r22, U32)
                b11, b12, b21, b22 = _planes(r11), _planes(src[rb, ca]), _planes(src[ra, cb]), _planes(r22)
                if swap:
                    b12, b21 = b21, b12
                for s, u, v, op in ((0, b11, b22, jnp.add), (2, b12, b22, jnp.subtract), (3, b21, b11, jnp.subtract),
                                    (5, b11, b12, jnp.add), (6, b21, b22, jnp.add)):
                    u0 = u[0] if never is None or prev is None else jnp.where(never, prev, u[0])
                    u1 = u[1] if never is None or prev is None else jnp.where(never, prev, u[1])
                    prev = op(u0, v[0])
                    dst[s, rd, ca] = _pack(prev, op(u1, v[1]))

    def prep_x(t, never=None):
        rhs7(xa, t * TM, HT, xc7.at[t], False, never)

    def prep_wo(never=None):
        rhs7(wo, 0, HD, wo7, True, never)

    def x_operand(t, j):
        return _unpack(xc7[t, j])

    def wo_operand(j):
        return _unpack(wo7[j])

    def ordered(dot, lhs, rhs, order, never, prev=None):
        m = {}
        for j in order:
            a = lhs(j)
            if prev is not None:
                tie = jnp.concatenate([prev[0:16, 0:128]] * (HD // 128), axis=1).astype(BF)
                a = jnp.concatenate([jnp.where(never, tie, a[0:16]), a[16:]], axis=0)
            prev = m[j] = dot(a, rhs(j))
        return m, prev

    def proj_o(w7, t, order, never, prev=None):
        m, prev = ordered(_nt, lambda j: _unpack(w7[j]), lambda j: x_operand(t, j), order, never, prev)
        return _assemble(m), prev

    def proj_t(w7, t):
        return _assemble([_nt(_unpack(w7[j]), x_operand(t, j)) for j in range(7)])

    def prods(w7, t, js):
        return {j: _nt(_unpack(w7[j]), x_operand(t, j)) for j in js}

    def phi_k(t, pT):
        ep, en, rp, rn = _dual_softmax_parts(pT)
        php = (ep * rp[:, None]).reshape(16, 64, TM)
        phn = (en * rn[:, None]).reshape(16, 64, TM)
        ph = jnp.concatenate([php, phn], axis=1)
        zz = ph[:, :, 0:128]
        for c in range(1, TM // 128):
            zz = zz + ph[:, :, c * 128:(c + 1) * 128]
        zacc[...] = zz if t == 0 else zacc[...] + zz
        return ph.astype(BF)

    def kv_accumulate(t, vT, phb):
        vT = vT.astype(BF)
        for j in range(16):
            u = _nt(vT[j * 64:(j + 1) * 64], phb[j])
            kvacc[j] = u if t == 0 else kvacc[j] + u

    def kv_update(t):
        kv_accumulate(t, proj_t(wv7, t), phi_k(t, proj_t(wk7, t)))

    def kv_update_o(t, never, ko=PORD, vo=PORD):
        pT, prev = proj_o(wk7, t, ko, never)
        vT, _ = proj_o(wv7, t, vo, never, prev)
        kv_accumulate(t, vT, phi_k(t, pT))

    def gate(t):
        xf = xa[t * TM:(t + 1) * TM, :].astype(F32)
        gb[t * TM:(t + 1) * TM, :] = jnp.broadcast_to(jax.nn.sigmoid(_rowdot(xf, gw[...].astype(F32))), (TM, 128))

    def router(t, bv, bi, with_gate=True):
        xf = xa[t * TM:(t + 1) * TM, :].astype(F32)
        if with_gate:
            gate(t)
        r = _rowdot(xf, wr[...].astype(F32)).astype(BF).astype(F32)
        r = jnp.broadcast_to(jnp.where(r != r, -jnp.inf, r), (TM, 128))
        row = lax.broadcasted_iota(jnp.int32, (8, 128), 0) + t * TM
        for k in range(TM // 8):
            rk = r[k * 8:(k + 1) * 8]
            better = rk > bv
            bv = jnp.where(better, rk, bv)
            bi = jnp.where(better, row + k * 8, bi)
        return bv, bi

    def gate_up(lo, hi, never=None):
        acc = None
        for c0 in range(GCUT[lo], GCUT[hi], 128):
            for m, w_ref in enumerate((wg, wu)):
                acc = jnp.zeros((8, 128), F32) if acc is None or never is None else jnp.where(never, acc, 0.0)
                for k in range(D // 16):
                    t = w_ref[k * 16:(k + 1) * 16, c0:c0 + 128].astype(F32) * xsb[k * 16:(k + 1) * 16, :]
                    acc = acc + t[0:8]
                    acc = acc + t[8:16]
                gu[m * 8:(m + 1) * 8, c0:c0 + 128] = acc

    def hidden():
        gg = jnp.sum(gu[0:8, :], axis=0, keepdims=True)
        uu = jnp.sum(gu[8:16, :], axis=0, keepdims=True)
        hb[...] = jnp.broadcast_to(gg * jax.nn.sigmoid(gg) * uu, (128, F)).T

    def down(i, never):
        acc = None
        for c in range(D // 128):
            acc = jnp.zeros((8, 128), F32) if acc is None else jnp.where(never, acc, 0.0)
            for k in range(DCUT[i] // 16, DCUT[i + 1] // 16):
                t = wd[k * 16:(k + 1) * 16, c * 128:(c + 1) * 128].astype(F32) * hb[k * 16:(k + 1) * 16, :]
                acc = acc + t[0:8]
                acc = acc + t[8:16]
            cs = slice(c * 128, (c + 1) * 128)
            yacc[:, cs] = acc if i == 0 else yacc[:, cs] + acc

    def finalize_kv():
        r3 = lax.broadcasted_iota(jnp.int32, (16, 64, 128), 1)
        c3 = lax.broadcasted_iota(jnp.int32, (16, 64, 128), 2)
        kvt[...] = pltpu.bitcast(jnp.where((r3 >> 5) == (c3 & 1), kvacc[...], 0.0).reshape(D, 128).astype(BF), U32)
        zb[...] = jnp.broadcast_to(jnp.sum(zacc[...], axis=2, keepdims=True), zb.shape)

    def attend(t, y, idx, never=None, qo=None, oo=None):
        ep, en, rp, rn = _dual_softmax_parts(proj_t(wq7, t) if qo is None else proj_o(wq7, t, qo, never)[0])
        z4 = zb[...].reshape(16, 2, 8, 8, 128)
        zp = jnp.concatenate([z4[:, 0]] * (TM // 128), axis=-1)
        zn = jnp.concatenate([z4[:, 1]] * (TM // 128), axis=-1)
        den = _rot(_red8(ep * zp, jnp.add) * rp + _red8(en * zn, jnp.add) * rn, jnp.add) + 1e-6
        rd = _rcp(den)
        php = (ep * (rp * rd)[:, None]).reshape(16, 64, TM)
        phn = (en * (rn * rd)[:, None]).reshape(16, 64, TM)
        phb = jnp.concatenate([php, phn], axis=1).astype(BF)
        oT = jnp.concatenate([_nn(_unpack(kvt[j * 32:(j + 1) * 32, :]), phb[j]) for j in range(16)], axis=0)
        oc = _lhs_combos(oT[:HD, :HT], oT[HD:, :HT], oT[:HD, HT:], oT[HD:, HT:])
        r0 = t * TM
        if oo is None:
            a = _assemble([_nn(oc[j].astype(BF).T, wo_operand(j)) for j in range(7)])
        else:
            a = _assemble(ordered(_nn, lambda j: oc[j].astype(BF).T, wo_operand, oo, never)[0])
        g = jnp.concatenate([gb[r0:r0 + TM, :]] * (D // 128), axis=1)
        b = xa[r0:r0 + TM, :].astype(F32)
        if y is not None:
            b = jnp.where(lax.broadcasted_iota(jnp.int32, (TM, D), 0) == idx - r0, b + y, b)
        res = (g * a + (1.0 - g) * b).astype(BF)
        if t < NT - 1:
            ob[r0:r0 + TM, :] = res
            ocp(t).start()
        else:
            for q, (rq, cq, wq_) in enumerate(PIECES):
                ob[r0 + rq:r0 + rq + HT, cq:cq + wq_] = res[rq:rq + HT, cq:cq + wq_]
                qcp(q).start()

    start(c_wphi, *kcp(0), *kcp(1), c_wr, c_gw, *[fcp(i) for i in range(4)])
    jj = lax.broadcasted_iota(jnp.int32, (128, DH), 0)
    ff = lax.broadcasted_iota(jnp.int32, (128, DH), 1)
    et = jnp.where((jj & (DH - 1)) == ff, 1.0, 0.0).astype(BF)
    j2 = lax.broadcasted_iota(jnp.int32, (128, 128), 0)
    c2 = lax.broadcasted_iota(jnp.int32, (128, 128), 1)
    keep = (c2 >> 5) == (j2 >> 5)
    wait(c_wphi)
    bd = _nt(et, wphi[...])
    for g in range(8):
        bdt[:, g * 128:(g + 1) * 128] = jnp.where(keep, bd[:, g * 128:(g + 1) * 128], 0.0).astype(BF)

    never0 = jnp.max(jnp.where(bd[0:8, 0:128] > 0.0, 1, 0)) < 0
    z0 = jnp.where(never0, 1, 0)
    for r in (wk7, wv7, wq7, wo7):
        r[z0, 0:8, 0:128] = jnp.zeros((8, 128), U32)
    xc7[z0, 0, 0:8, 0:128] = jnp.zeros((8, 128), U32)
    z8 = pl.multiple_of(z0 * 8, 8)
    for r in (gb, xsb, hb):
        r[pl.ds(z8, 8), :] = jnp.zeros((8, 128), F32)
    for r in (kvacc, zacc, zb):
        r[z0, 0:8, :] = jnp.zeros((8, 128), F32)
    kvt[pl.ds(z8, 8), :] = jnp.zeros((8, 128), U32)
    gu[pl.ds(z8, 8), 0:128] = jnp.zeros((8, 128), F32)
    nxt = [kcp(2), kcp(3), [c_x[0]], [c_x[1]]]
    for g in range(4):
        wait(kcp(g)[0])
        start(*nxt[g])
        wait(kcp(g)[1])
        fold7(wk, wk7, g)
    wait(c_x[0])
    start(c_wv)
    wait(c_x[1])
    wait(c_wr, c_gw)
    prep_x(0)
    mk = prods(wk7, 0, (1, 4, 2, 3, 0))
    bv = jnp.full((8, 128), -jnp.inf, F32)
    bi = lax.broadcasted_iota(jnp.int32, (8, 128), 0)
    bv, bi = router(0, bv, bi)
    wait(c_wv)
    start(c_x[2], c_x[3], c_x[4], gcp(0))
    wait(fcp(0))
    prep_wv()
    mk.update(prods(wk7, 0, (6, 5)))
    kv_accumulate(0, proj_t(wv7, 0), phi_k(0, _assemble(mk)))
    wait(c_x[2], c_x[3])
    start(gcp(1), ucp(0), gcp(2))
    wait(c_x[4])
    prep_x(1)
    kv_update_o(1, never0, (1, 4, 2, 3, 0, 6, 5))
    prep_x(2, never0)
    for t in range(1, NT):
        bv, bi = router(t, bv, bi)
    rmax = jnp.max(bv, axis=0, keepdims=True)
    idx = jnp.min(jnp.where(bv == rmax, bi, S))
    rsel = jax.nn.sigmoid(rmax)
    base = pl.multiple_of((idx >> 4) << 4, 16)
    rows = lax.broadcasted_iota(jnp.int32, (16, D), 0)
    blk = xa[pl.ds(base, 16), :].astype(F32)
    xs = jnp.sum(jnp.where(rows == idx - base, blk, 0.0), axis=0, keepdims=True)
    xsb[...] = jnp.broadcast_to(xs, (128, D)).T
    never = idx < 0
    wait(gcp(0), gcp(1), ucp(0))
    start(gcp(3), ucp(1))
    wait(fcp(1))
    kv_update_o(2, never)
    prep_x(3, never)
    gate_up(0, 1, never)
    wait(gcp(2), gcp(3), ucp(1))
    start(c_wq, c_wo)
    wait(fcp(2))
    kv_update_o(3, never)
    gate_up(1, 2, never)
    wait(c_wq, c_wo)
    start(dcp(0), dcp(1))
    wait(fcp(3))
    for g in range(4):
        fold7(wq, wq7, g)
    finalize_kv()
    hidden()
    prep_wo()
    attend(0, None, None, never, PORD, OORD)
    wait(dcp(0), dcp(1))
    attend(1, None, None, never, None, OORD)
    down(0, never)
    wait(ocp(0))
    attend(2, None, None, never, None, OORD)
    down(1, never)
    wait(ocp(1))
    y = jnp.sum(yacc[...], axis=0, keepdims=True) * jnp.concatenate([rsel] * 8, axis=1)
    attend(3, y, idx, never, None, OORD)
    wait(ocp(2))

    @pl.when(idx < (NT - 1) * TM)
    def _():
        gsel = jnp.concatenate([gb[pl.ds(base, 16), :]] * (D // 128), axis=1)
        old = ob[pl.ds(base, 16), :].astype(F32)
        pb[...] = jnp.where(rows == idx - base, old + (1.0 - gsel) * y, old).astype(BF)
        c_patch = cp(pb, out_h.at[pl.ds(base, 16), :], 7)
        c_patch.start()
        c_patch.wait()

    wait(*[qcp(q) for q in range(len(PIECES))])


@jax.jit
def pallas_gated_mix__linear_kernel_hedgehog__moe_arch_mod__prompt_kernel(
        A_x, A_wqkv, A_w_phi, A_wo, B_x, B_w_r, B_w_gate, B_w_up, B_w_down, gate_w):
    anyspec = pl.BlockSpec(memory_space=pl.ANY)
    V = pltpu.VMEM
    DMA = pltpu.SemaphoreType.DMA
    out = pl.pallas_call(
        kernel,
        out_shape=jax.ShapeDtypeStruct((S, D), BF),
        in_specs=[anyspec] * 9,
        out_specs=anyspec,
        scratch_shapes=[
            V((S, D), BF), V((D, D), BF), V((D, D), BF), V((D, D), BF), V((D, D), BF),
            V((D, F), BF), V((D, F), BF), V((F, D), BF),
            V((D, DH), BF), V((8, 128), BF), V((8, 128), BF), V((128, D), BF),
            V((S, D), BF), V((16, 64, 128), F32), V((16, 128, 128), F32),
            V((D // 2, 128), U32), V((16, 128, 128), F32), V((S, 128), F32),
            V((D, 128), F32), V((16, F), F32), V((F, 128), F32), V((8, D), F32), V((16, D), BF),
            V((7, HD // 2, HD), U32), V((7, HD // 2, HD), U32), V((7, HD // 2, HD), U32), V((7, HD // 2, HD), U32),
            V((NT, 7, HT // 2, HD), U32), V((4, 8, 128), BF),
            DMA((8,)), DMA((4,)), DMA((NT + 1,)), DMA((4,)), DMA((2,)), DMA((2,)), DMA((NT,)), DMA((4,)),
        ],
        compiler_params=pltpu.CompilerParams(vmem_limit_bytes=110 * 2**20, flags={"XLA_TPU_EVENLY_DISTRIBUTE_CRITICAL_NODES": True}),
    )(A_x.reshape(S, D), A_wqkv, A_w_phi.reshape(D, DH), A_wo,
      B_w_r.reshape(8, 128), B_w_gate, B_w_up, B_w_down, gate_w.reshape(8, 128))
    return out.reshape(1, S, D)
```

```python
import functools
import jax
import jax.numpy as jnp
import numpy as np
from jax import lax
from jax.experimental import pallas as pl
from jax.experimental.pallas import tpu as pltpu

S, D, H, DH, F = 2048, 1024, 32, 32, 3584
TM = 512
NT = S // TM
HT = TM // 2
HD = D // 2
GDMA = (0, 1024, 1792, 2304, F)
UDMA = (0, 1792, F)
GCUT = (0, 1792, F)
DCUT = (0, 1792, F)
LOG2E = 1.4426950408889634
BF = jnp.bfloat16
F32 = jnp.float32
U32 = jnp.uint32
PIECES = ((0, HD, HD), (HT, 0, HD), (HT, HD, 256), (HT, HD + 256, 256), (0, 0, 128), (0, 128, 128), (0, 256, 128), (0, 384, 128))
PORD = (2, 4, 1, 3, 0, 6, 5)
OORD = (2, 4, 5, 1, 3, 0, 6)
QORD = (0, 3, 4, 6, 2, 1, 5)


def _nt(a, b):
    return lax.dot_general(a, b, (((1,), (1,)), ((), ())), preferred_element_type=F32)


def _nn(a, b):
    return jnp.dot(a, b, preferred_element_type=F32)


def _red8(x4, op):
    r = x4[:, 0]
    for k in range(1, 8):
        r = op(r, x4[:, k])
    return r


def _rot(r, op):
    r = op(r, pltpu.roll(r, 4, 1))
    return op(r, pltpu.roll(r, 2, 1))


def _pack(even, odd):
    return pltpu.bitcast(pltpu.pack_elementwise([even, odd], packed_dtype=BF), U32)


def _planes(x):
    w = pltpu.bitcast(x, U32)
    return [pltpu.unpack_elementwise(w, index=i, packed_dtype=BF, unpacked_dtype=F32) for i in range(2)]


def _unpack(x):
    return pltpu.bitcast(x, BF)


def _rcp(x):
    r = pl.reciprocal(x, approx=True)
    return r * (2.0 - x * r)


def _dual_softmax_parts(pT):
    n = pT.shape[0] // 64
    p4 = pT.reshape(n, 8, 8, pT.shape[1])
    mx = _rot(_red8(p4, jnp.maximum), jnp.maximum)
    mn = _rot(_red8(p4, jnp.minimum), jnp.minimum)
    ep = jnp.exp2(p4 - mx[:, None])
    en = jnp.exp2(mn[:, None] - p4)
    rp = _rcp(_rot(_red8(ep, jnp.add), jnp.add))
    rn = _rcp(_rot(_red8(en, jnp.add), jnp.add))
    return ep, en, rp, rn


def _rowdot(xf, w8):
    acc = xf[:, 0:128] * w8[0:1]
    for k in range(1, 8):
        acc = acc + xf[:, k * 128:(k + 1) * 128] * w8[k:k + 1]
    return jnp.sum(acc, axis=1, keepdims=True)


def _lhs_combos(a11, a12, a21, a22):
    return (a11 + a22, a21 + a22, a11, a22, a11 + a12, a21 - a11, a12 - a22)


def _rhs_combos(b11, b12, b21, b22):
    return (b11 + b22, b11, b12 - b22, b21 - b11, b22, b11 + b12, b21 + b22)


def _assemble(m):
    c11 = m[0] + m[3] - m[4] + m[6]
    c12 = m[2] + m[4]
    c21 = m[1] + m[3]
    c22 = m[0] - m[1] + m[2] + m[5]
    return jnp.concatenate([jnp.concatenate([c11, c12], axis=1), jnp.concatenate([c21, c22], axis=1)], axis=0)


def _assemble_logits(m):
    c11 = m[0] + m[3] - m[4] + m[6]
    c12 = m[2] + m[4]
    c21 = m[1] + m[3]
    c22 = m[0] - m[1] + m[2] + m[5]
    slot = lax.broadcasted_iota(jnp.int32, (8, 2 * c11.shape[1]), 0) >> 1
    rows = []
    for half in (jnp.concatenate([c11, c12], axis=1), jnp.concatenate([c21, c22], axis=1)):
        first = [jnp.zeros(slot.shape, F32), jnp.zeros(slot.shape, F32)]
        rest = []
        for p in range(1, 8):
            r0 = 64 * p - 16
            v = [half[r0 + 8 * k:r0 + 8 * k + 8] for k in range(8)]
            lent = slot == p % 4
            first[p // 4] = jnp.where(lent, v[p // 4], first[p // 4])
            v[p // 4] = jnp.where(lent, 0.0, v[p // 4])
            rest += v
        rows += first + [half[0:48]] + rest
    return jnp.concatenate(rows, axis=0)


def kernel(xa_h, wqkv_h, wphi_h, wo_h, wr_h, wg_h, wu_h, wd_h, gw_h, out_h,
           xa, wq, wk, wv, wo, wg, wu, wd, wphi, wr, gw, bdt,
           ob, kvacc, zacc, kvt, zb, gb, xsb, gu, hb, yacc, pb, wk7, wv7, wq7, wo7, xc7, fence,
           sem, ksem, xsem, gsem, usem, dsem, osem, fsem):
    def cp(src, dst, k):
        return pltpu.make_async_copy(src, dst, sem.at[k])

    def xcp(j, r0, n):
        return pltpu.make_async_copy(xa_h.at[pl.ds(r0, n), :], xa.at[pl.ds(r0, n), :], xsem.at[j])

    def gcp(i):
        cs = pl.ds(GDMA[i], GDMA[i + 1] - GDMA[i])
        return pltpu.make_async_copy(wg_h.at[:, cs], wg.at[:, cs], gsem.at[i])

    def ucp(i):
        cs = pl.ds(UDMA[i], UDMA[i + 1] - UDMA[i])
        return pltpu.make_async_copy(wu_h.at[:, cs], wu.at[:, cs], usem.at[i])

    def dcp(i):
        rs = pl.ds(DCUT[i], DCUT[i + 1] - DCUT[i])
        return pltpu.make_async_copy(wd_h.at[rs, :], wd.at[rs, :], dsem.at[i])

    def kcp(g):
        return [pltpu.make_async_copy(wqkv_h.at[:, pl.ds(D + c * 128, 128)], wk.at[:, pl.ds(c * 128, 128)], ksem.at[g])
                for c in (g, g + 4)]

    def ocp(t):
        return pltpu.make_async_copy(ob.at[pl.ds(t * TM, TM), :], out_h.at[pl.ds(t * TM, TM), :], osem.at[t])

    def qcp(q):
        rs, cs = pl.ds((NT - 1) * TM + PIECES[q][0], HT), pl.ds(*PIECES[q][1:])
        return pltpu.make_async_copy(ob.at[rs, cs], out_h.at[rs, cs], osem.at[NT - 1])

    def fcp(i):
        return pltpu.make_async_copy(wr_h, fence.at[i], fsem.at[i])

    def start(*cs):
        for c in cs:
            c.start()

    def wait(*cs):
        for c in cs:
            c.wait()

    c_wphi = cp(wphi_h, wphi, 0)
    c_wv = cp(wqkv_h.at[:, pl.ds(2 * D, D)], wv, 1)
    c_wq = cp(wqkv_h.at[:, pl.ds(0, D)], wq, 2)
    c_wr = cp(wr_h, wr, 3)
    c_gw = cp(gw_h, gw, 4)
    c_wo = cp(wo_h, wo, 5)
    c_x = [xcp(0, 0, HT), xcp(1, HT, HT)] + [xcp(1 + t, t * TM, TM) for t in range(1, NT)]

    def fold7(w_ref, dst, g, lent):
        t = [_nt(bdt[:, c * 128:(c + 1) * 128], w_ref[:, c * 128:(c + 1) * 128]) * LOG2E for c in (g, g + 4)]
        for q in range(2):
            p = 2 * g + q
            heads = [[x[r0:r0 + DH] - x[r0 + p:r0 + p + 1] for x in t] for r0 in (q * 64, q * 64 + DH)]
            if p == 0:
                lent = [[x[0:8] for x in h] for h in heads]
                heads = [[x[8:] for x in h] for h in heads]
                rs = slice(0, DH - 8)
            else:
                row = lax.broadcasted_iota(jnp.int32, (8, D), 0) == p
                heads = [[jnp.concatenate([jnp.where(row, y, x[0:8]), x[8:]], axis=0) for x, y in zip(h, l)]
                         for h, l in zip(heads, lent)]
                rs = slice(p * DH - 8, (p + 1) * DH - 8)
            cs = [_lhs_combos(u[:, :HD], u[:, HD:], v[:, :HD], v[:, HD:]) for u, v in heads]
            for j in range(7):
                dst[j, rs, :] = _pack(cs[0][j], cs[1][j])
        return lent

    def prep_wv():
        for g in range(4):
            ta = _planes(wv[:, g * 128:(g + 1) * 128].T)
            tb = _planes(wv[:, (g + 4) * 128:(g + 5) * 128].T)
            cs = [_lhs_combos(u[:, :HD], u[:, HD:], v[:, :HD], v[:, HD:]) for u, v in zip(ta, tb)]
            for j in range(7):
                wv7[j, g * 64:(g + 1) * 64, :] = _pack(cs[0][j], cs[1][j])

    def rhs7(src, r0, nr, dst, swap, never=None):
        prev = None
        for q in range(nr // 16):
            ra = slice(r0 + q * 16, r0 + (q + 1) * 16)
            rb = slice(r0 + nr + q * 16, r0 + nr + (q + 1) * 16)
            rd = slice(q * 8, (q + 1) * 8)
            for c in range(HD // 128):
                ca = slice(c * 128, (c + 1) * 128)
                cb = slice(HD + c * 128, HD + (c + 1) * 128)
                r11, r22 = src[ra, ca], src[rb, cb]
                dst[1, rd, ca] = pltpu.bitcast(r11, U32)
                dst[4, rd, ca] = pltpu.bitcast(r22, U32)
                b11, b12, b21, b22 = _planes(r11), _planes(src[rb, ca]), _planes(src[ra, cb]), _planes(r22)
                if swap:
                    b12, b21 = b21, b12
                for s, u, v, op in ((0, b11, b22, jnp.add), (2, b12, b22, jnp.subtract), (3, b21, b11, jnp.subtract),
                                    (5, b11, b12, jnp.add), (6, b21, b22, jnp.add)):
                    u0 = u[0] if never is None or prev is None else jnp.where(never, prev, u[0])
                    u1 = u[1] if never is None or prev is None else jnp.where(never, prev, u[1])
                    prev = op(u0, v[0])
                    dst[s, rd, ca] = _pack(prev, op(u1, v[1]))

    def prep_x(t, never=None):
        rhs7(xa, t * TM, HT, xc7.at[t], False, never)

    def prep_wo(never=None):
        rhs7(wo, 0, HD, wo7, True, never)

    def x_operand(t, j):
        return _unpack(xc7[t, j])

    def wo_operand(j):
        return _unpack(wo7[j])

    def ordered(dot, lhs, rhs, order, never, prev=None):
        m = {}
        for j in order:
            a = lhs(j)
            if prev is not None:
                tie = jnp.concatenate([prev[0:16, 0:128]] * (HD // 128), axis=1).astype(BF)
                a = jnp.concatenate([jnp.where(never, tie, a[0:16]), a[16:]], axis=0)
            prev = m[j] = dot(a, rhs(j))
        return m, prev

    def proj_o(w7, t, order, never, prev=None):
        m, prev = ordered(_nt, lambda j: _unpack(w7[j]), lambda j: x_operand(t, j), order, never, prev)
        return (_assemble if w7 is wv7 else _assemble_logits)(m), prev

    def proj_t(w7, t):
        return (_assemble if w7 is wv7 else _assemble_logits)([_nt(_unpack(w7[j]), x_operand(t, j)) for j in range(7)])

    def prods(w7, t, js):
        return {j: _nt(_unpack(w7[j]), x_operand(t, j)) for j in js}

    def phi_k(t, pT):
        ep, en, rp, rn = _dual_softmax_parts(pT)
        php = (ep * rp[:, None]).reshape(16, 64, TM)
        phn = (en * rn[:, None]).reshape(16, 64, TM)
        ph = jnp.concatenate([php, phn], axis=1)
        zz = ph[:, :, 0:128]
        for c in range(1, TM // 128):
            zz = zz + ph[:, :, c * 128:(c + 1) * 128]
        zacc[...] = zz if t == 0 else zacc[...] + zz
        return ph.astype(BF)

    def kv_accumulate(t, vT, phb):
        vT = vT.astype(BF)
        for j in range(16):
            u = _nt(vT[j * 64:(j + 1) * 64], phb[j])
            kvacc[j] = u if t == 0 else kvacc[j] + u

    def kv_update(t):
        kv_accumulate(t, proj_t(wv7, t), phi_k(t, proj_t(wk7, t)))

    def kv_update_o(t, never, ko=PORD, vo=PORD):
        pT, prev = proj_o(wk7, t, ko, never)
        vT, _ = proj_o(wv7, t, vo, never, prev)
        kv_accumulate(t, vT, phi_k(t, pT))

    def kv_update_s(t, never, seq):
        w = {"k": wk7, "v": wv7}
        m, _ = ordered(_nt, lambda s_: _unpack(w[s_[0]][int(s_[1])]), lambda s_: x_operand(t, int(s_[1])), seq.split(), never)
        kv_accumulate(t, _assemble([m["v%d" % j] for j in range(7)]), phi_k(t, _assemble_logits([m["k%d" % j] for j in range(7)])))

    def gate(t):
        xf = xa[t * TM:(t + 1) * TM, :].astype(F32)
        gb[t * TM:(t + 1) * TM, :] = jnp.broadcast_to(jax.nn.sigmoid(_rowdot(xf, gw[...].astype(F32))), (TM, 128))

    def router(t, bv, bi, with_gate=True):
        xf = xa[t * TM:(t + 1) * TM, :].astype(F32)
        if with_gate:
            gate(t)
        r = _rowdot(xf, wr[...].astype(F32)).astype(BF).astype(F32)
        r = jnp.broadcast_to(jnp.where(r != r, -jnp.inf, r), (TM, 128))
        row = lax.broadcasted_iota(jnp.int32, (8, 128), 0) + t * TM
        for k in range(TM // 8):
            rk = r[k * 8:(k + 1) * 8]
            better = rk > bv
            bv = jnp.where(better, rk, bv)
            bi = jnp.where(better, row + k * 8, bi)
        return bv, bi

    def gate_up(lo, hi, never=None):
        acc = None
        for c0 in range(GCUT[lo], GCUT[hi], 128):
            for m, w_ref in enumerate((wg, wu)):
                acc = jnp.zeros((8, 128), F32) if acc is None or never is None else jnp.where(never, acc, 0.0)
                for k in range(D // 16):
                    t = w_ref[k * 16:(k + 1) * 16, c0:c0 + 128].astype(F32) * xsb[k * 16:(k + 1) * 16, :]
                    acc = acc + t[0:8]
                    acc = acc + t[8:16]
                gu[m * 8:(m + 1) * 8, c0:c0 + 128] = acc

    def hidden():
        gg = jnp.sum(gu[0:8, :], axis=0, keepdims=True)
        uu = jnp.sum(gu[8:16, :], axis=0, keepdims=True)
        hb[...] = jnp.broadcast_to(gg * jax.nn.sigmoid(gg) * uu, (128, F)).T

    def down(i, never):
        acc = None
        for c in range(D // 128):
            acc = jnp.zeros((8, 128), F32) if acc is None else jnp.where(never, acc, 0.0)
            for k in range(DCUT[i] // 16, DCUT[i + 1] // 16):
                t = wd[k * 16:(k + 1) * 16, c * 128:(c + 1) * 128].astype(F32) * hb[k * 16:(k + 1) * 16, :]
                acc = acc + t[0:8]
                acc = acc + t[8:16]
            cs = slice(c * 128, (c + 1) * 128)
            yacc[:, cs] = acc if i == 0 else yacc[:, cs] + acc

    def finalize_kv():
        r3 = lax.broadcasted_iota(jnp.int32, (16, 64, 128), 1)
        c3 = lax.broadcasted_iota(jnp.int32, (16, 64, 128), 2)
        kvt[...] = pltpu.bitcast(jnp.where((r3 >> 5) == (c3 & 1), kvacc[...], 0.0).reshape(D, 128).astype(BF), U32)
        zb[...] = jnp.broadcast_to(jnp.sum(zacc[...], axis=2, keepdims=True), zb.shape)

    def attend(t, y, idx, never=None, qo=None, oo=None):
        ep, en, rp, rn = _dual_softmax_parts(proj_t(wq7, t) if qo is None else proj_o(wq7, t, qo, never)[0])
        z4 = zb[...].reshape(16, 2, 8, 8, 128)
        zp = jnp.concatenate([z4[:, 0]] * (TM // 128), axis=-1)
        zn = jnp.concatenate([z4[:, 1]] * (TM // 128), axis=-1)
        den = _rot(_red8(ep * zp, jnp.add) * rp + _red8(en * zn, jnp.add) * rn, jnp.add) + 1e-6
        rd = _rcp(den)
        php = (ep * (rp * rd)[:, None]).reshape(16, 64, TM)
        phn = (en * (rn * rd)[:, None]).reshape(16, 64, TM)
        phb = jnp.concatenate([php, phn], axis=1).astype(BF)
        oT = jnp.concatenate([_nn(_unpack(kvt[j * 32:(j + 1) * 32, :]), phb[j]) for j in range(16)], axis=0)
        oc = _lhs_combos(oT[:HD, :HT], oT[HD:, :HT], oT[:HD, HT:], oT[HD:, HT:])
        r0 = t * TM
        if oo is None:
            a = _assemble([_nn(oc[j].astype(BF).T, wo_operand(j)) for j in range(7)])
        else:
            a = _assemble(ordered(_nn, lambda j: oc[j].astype(BF).T, wo_operand, oo, never)[0])
        g = jnp.concatenate([gb[r0:r0 + TM, :]] * (D // 128), axis=1)
        b = xa[r0:r0 + TM, :].astype(F32)
        if y is not None:
            b = jnp.where(lax.broadcasted_iota(jnp.int32, (TM, D), 0) == idx - r0, b + y, b)
        res = (g * a + (1.0 - g) * b).astype(BF)
        if t < NT - 1:
            ob[r0:r0 + TM, :] = res
            ocp(t).start()
        else:
            for q, (rq, cq, wq_) in enumerate(PIECES):
                ob[r0 + rq:r0 + rq + HT, cq:cq + wq_] = res[rq:rq + HT, cq:cq + wq_]
                qcp(q).start()

    start(c_wphi, *kcp(0), *kcp(1), c_wr, c_gw, *[fcp(i) for i in range(4)])
    jj = lax.broadcasted_iota(jnp.int32, (128, DH), 0)
    ff = lax.broadcasted_iota(jnp.int32, (128, DH), 1)
    et = jnp.where((jj & (DH - 1)) == ff, 1.0, 0.0).astype(BF)
    j2 = lax.broadcasted_iota(jnp.int32, (128, 128), 0)
    c2 = lax.broadcasted_iota(jnp.int32, (128, 128), 1)
    keep = (c2 >> 5) == (j2 >> 5)
    wait(c_wphi)
    bd = _nt(et, wphi[...])
    for g in range(8):
        bdt[:, g * 128:(g + 1) * 128] = jnp.where(keep, bd[:, g * 128:(g + 1) * 128], 0.0).astype(BF)

    never0 = jnp.max(jnp.where(bd[0:8, 0:128] > 0.0, 1, 0)) < 0
    z0 = jnp.where(never0, 1, 0)
    for r in (wk7, wv7, wq7, wo7):
        r[z0, 0:8, 0:128] = jnp.zeros((8, 128), U32)
    xc7[z0, 0, 0:8, 0:128] = jnp.zeros((8, 128), U32)
    z8 = pl.multiple_of(z0 * 8, 8)
    for r in (gb, xsb, hb):
        r[pl.ds(z8, 8), :] = jnp.zeros((8, 128), F32)
    for r in (kvacc, zacc, zb):
        r[z0, 0:8, :] = jnp.zeros((8, 128), F32)
    kvt[pl.ds(z8, 8), :] = jnp.zeros((8, 128), U32)
    gu[pl.ds(z8, 8), 0:128] = jnp.zeros((8, 128), F32)
    lent = None
    nxt = [kcp(2), kcp(3), [c_x[0]], [c_x[1]]]
    for g in range(4):
        wait(kcp(g)[0])
        start(*nxt[g])
        wait(kcp(g)[1])
        lent = fold7(wk, wk7, g, lent)
    wait(c_x[0])
    start(c_wv)
    wait(c_x[1])
    wait(c_wr, c_gw)
    prep_x(0)
    mk = prods(wk7, 0, (1, 4, 2, 3))
    bv = jnp.full((8, 128), -jnp.inf, F32)
    bi = lax.broadcasted_iota(jnp.int32, (8, 128), 0)
    bv, bi = router(0, bv, bi)
    wait(c_wv)
    start(c_x[2], c_x[3], c_x[4], gcp(0))
    wait(fcp(0))
    prep_wv()
    mk.update(prods(wk7, 0, (0, 6, 5)))
    kv_accumulate(0, proj_t(wv7, 0), phi_k(0, _assemble_logits(mk)))
    wait(c_x[2], c_x[3])
    start(gcp(1), ucp(0), gcp(2))
    wait(c_x[4])
    prep_x(1)
    kv_update_s(1, never0, 'k4 k1 k2 k3 v1 k0 k6 v4 k5 v2 v3 v0 v6 v5')
    prep_x(2, never0)
    for t in range(1, NT):
        bv, bi = router(t, bv, bi)
    rmax = jnp.max(bv, axis=0, keepdims=True)
    idx = jnp.min(jnp.where(bv == rmax, bi, S))
    rsel = jax.nn.sigmoid(rmax)
    base = pl.multiple_of((idx >> 4) << 4, 16)
    rows = lax.broadcasted_iota(jnp.int32, (16, D), 0)
    blk = xa[pl.ds(base, 16), :].astype(F32)
    xs = jnp.sum(jnp.where(rows == idx - base, blk, 0.0), axis=0, keepdims=True)
    xsb[...] = jnp.broadcast_to(xs, (128, D)).T
    never = idx < 0
    wait(gcp(0), gcp(1), ucp(0))
    start(gcp(3), ucp(1))
    wait(fcp(1))
    kv_update_o(2, never)
    prep_x(3, never)
    gate_up(0, 1, never)
    wait(gcp(2), gcp(3), ucp(1))
    start(c_wq, c_wo)
    wait(fcp(2))
    kv_update_o(3, never)
    gate_up(1, 2, never)
    wait(c_wq, c_wo)
    start(dcp(0), dcp(1))
    wait(fcp(3))
    for g in range(4):
        lent = fold7(wq, wq7, g, lent)
    finalize_kv()
    hidden()
    prep_wo()
    attend(0, None, None, never, PORD, OORD)
    wait(dcp(0), dcp(1))
    attend(1, None, None, never, QORD, OORD)
    down(0, never)
    wait(ocp(0))
    attend(2, None, None, never, QORD, OORD)
    down(1, never)
    wait(ocp(1))
    y = jnp.sum(yacc[...], axis=0, keepdims=True) * jnp.concatenate([rsel] * 8, axis=1)
    attend(3, y, idx, never, PORD, OORD)
    wait(ocp(2))

    @pl.when(idx < (NT - 1) * TM)
    def _():
        gsel = jnp.concatenate([gb[pl.ds(base, 16), :]] * (D // 128), axis=1)
        old = ob[pl.ds(base, 16), :].astype(F32)
        pb[...] = jnp.where(rows == idx - base, old + (1.0 - gsel) * y, old).astype(BF)
        c_patch = cp(pb, out_h.at[pl.ds(base, 16), :], 7)
        c_patch.start()
        c_patch.wait()

    wait(*[qcp(q) for q in range(len(PIECES))])


@jax.jit
def pallas_gated_mix__linear_kernel_hedgehog__moe_arch_mod__prompt_kernel(
        A_x, A_wqkv, A_w_phi, A_wo, B_x, B_w_r, B_w_gate, B_w_up, B_w_down, gate_w):
    anyspec = pl.BlockSpec(memory_space=pl.ANY)
    V = pltpu.VMEM
    DMA = pltpu.SemaphoreType.DMA
    out = pl.pallas_call(
        kernel,
        out_shape=jax.ShapeDtypeStruct((S, D), BF),
        in_specs=[anyspec] * 9,
        out_specs=anyspec,
        scratch_shapes=[
            V((S, D), BF), V((D, D), BF), V((D, D), BF), V((D, D), BF), V((D, D), BF),
            V((D, F), BF), V((D, F), BF), V((F, D), BF),
            V((D, DH), BF), V((8, 128), BF), V((8, 128), BF), V((128, D), BF),
            V((S, D), BF), V((16, 64, 128), F32), V((16, 128, 128), F32),
            V((D // 2, 128), U32), V((16, 128, 128), F32), V((S, 128), F32),
            V((D, 128), F32), V((16, F), F32), V((F, 128), F32), V((8, D), F32), V((16, D), BF),
            V((7, HD // 2 - 8, HD), U32), V((7, HD // 2, HD), U32), V((7, HD // 2 - 8, HD), U32), V((7, HD // 2, HD), U32),
            V((NT, 7, HT // 2, HD), U32), V((4, 8, 128), BF),
            DMA((8,)), DMA((4,)), DMA((NT + 1,)), DMA((4,)), DMA((2,)), DMA((2,)), DMA((NT,)), DMA((4,)),
        ],
        compiler_params=pltpu.CompilerParams(vmem_limit_bytes=110 * 2**20, flags={"XLA_TPU_EVENLY_DISTRIBUTE_CRITICAL_NODES": True}),
    )(A_x.reshape(S, D), A_wqkv, A_w_phi.reshape(D, DH), A_wo,
      B_w_r.reshape(8, 128), B_w_gate, B_w_up, B_w_down, gate_w.reshape(8, 128))
    return out.reshape(1, S, D)
```

```python
import jax
import jax.numpy as jnp
from jax import lax
from jax.experimental import pallas as pl
from jax.experimental.pallas import tpu as pltpu

S, D, H, DH, F = 2048, 1024, 32, 32, 3584
TM = 512
NT = S // TM
HT = TM // 2
HD = D // 2
GDMA = (0, 1024, 1792, 2304, F)
UDMA = (0, 1792, F)
FCUT = (0, 1792, F)
PIECES = ((0, HD, HD), (HT, 0, HD), (HT, HD, 256), (HT, HD + 256, 256),
          (0, 0, 128), (0, 128, 128), (0, 256, 128), (0, 384, 128))
PORD = (2, 4, 1, 3, 0, 6, 5)
QORD = (0, 3, 4, 6, 2, 1, 5)
OORD = (2, 4, 5, 1, 3, 0, 6)
LOG2E = 1.4426950408889634
BF = jnp.bfloat16
F32 = jnp.float32
U32 = jnp.uint32


def _nt(a, b):
    return lax.dot_general(a, b, (((1,), (1,)), ((), ())), preferred_element_type=F32)


def _nn(a, b):
    return jnp.dot(a, b, preferred_element_type=F32)


def _pack(even, odd):
    return pltpu.bitcast(pltpu.pack_elementwise([even, odd], packed_dtype=BF), U32)


def _planes(x):
    w = pltpu.bitcast(x, U32)
    return [pltpu.unpack_elementwise(w, index=i, packed_dtype=BF, unpacked_dtype=F32) for i in range(2)]


def _unpack(x):
    return pltpu.bitcast(x, BF)


def _rcp(x):
    r = pl.reciprocal(x, approx=True)
    return r * (2.0 - x * r)


def _red8(x4, op):
    r = x4[:, 0]
    for k in range(1, 8):
        r = op(r, x4[:, k])
    return r


def _rot(r, op):
    r = op(r, pltpu.roll(r, 4, 1))
    return op(r, pltpu.roll(r, 2, 1))


def _dual_softmax_parts(pT):
    p4 = pT.reshape(H // 2, 8, 8, pT.shape[1])
    mx = _rot(_red8(p4, jnp.maximum), jnp.maximum)
    mn = _rot(_red8(p4, jnp.minimum), jnp.minimum)
    ep = jnp.exp2(p4 - mx[:, None])
    en = jnp.exp2(mn[:, None] - p4)
    rp = _rcp(_rot(_red8(ep, jnp.add), jnp.add))
    rn = _rcp(_rot(_red8(en, jnp.add), jnp.add))
    return ep, en, rp, rn


def _rowdot(xf, w8):
    acc = xf[:, 0:128] * w8[0:1]
    for k in range(1, 8):
        acc = acc + xf[:, k * 128:(k + 1) * 128] * w8[k:k + 1]
    return jnp.sum(acc, axis=1, keepdims=True)


def _matvec(w_ref, v_ref, r0, r1, c0, acc):
    for r in range(r0, r1, 16):
        t = w_ref[r:r + 16, c0:c0 + 128].astype(F32) * v_ref[r:r + 16, :]
        acc = acc + t[0:8]
        acc = acc + t[8:16]
    return acc


def _lhs_combos(a11, a12, a21, a22):
    return (a11 + a22, a21 + a22, a11, a22, a11 + a12, a21 - a11, a12 - a22)


RHS_SUMS = ((0, 0, 3, jnp.add), (2, 1, 3, jnp.subtract), (3, 2, 0, jnp.subtract),
            (5, 0, 1, jnp.add), (6, 2, 3, jnp.add))


def _halves(m):
    c11 = m[0] + m[3] - m[4] + m[6]
    c12 = m[2] + m[4]
    c21 = m[1] + m[3]
    c22 = m[0] - m[1] + m[2] + m[5]
    return jnp.concatenate([c11, c12], axis=1), jnp.concatenate([c21, c22], axis=1)


def _assemble(m):
    return jnp.concatenate(_halves(m), axis=0)


def _assemble_logits(m):
    slot = lax.broadcasted_iota(jnp.int32, (8, TM), 0) >> 1
    rows = []
    for half in _halves(m):
        first = [jnp.zeros(slot.shape, F32), jnp.zeros(slot.shape, F32)]
        rest = []
        for p in range(1, 8):
            r0 = 64 * p - 16
            v = [half[r0 + 8 * k:r0 + 8 * k + 8] for k in range(8)]
            lent = slot == p % 4
            first[p // 4] = jnp.where(lent, v[p // 4], first[p // 4])
            v[p // 4] = jnp.where(lent, 0.0, v[p // 4])
            rest += v
        rows += first + [half[0:48]] + rest
    return jnp.concatenate(rows, axis=0)


def _ordered(dot, lhs, rhs, order, never, prev=None):
    m = {}
    for j in order:
        a = lhs(j)
        if prev is not None:
            tie = jnp.concatenate([prev[0:16, 0:128]] * (HD // 128), axis=1).astype(BF)
            a = jnp.concatenate([jnp.where(never, tie, a[0:16]), a[16:]], axis=0)
        prev = m[j] = dot(a, rhs(j))
    return m, prev


def kernel(xa_h, wqkv_h, wphi_h, wo_h, wr_h, wg_h, wu_h, wd_h, gw_h, out_h,
           xa, wq, wk, wv, wo, wg, wu, wd, wphi, wr, gw, bdt,
           ob, kvacc, zacc, kvt, zb, gb, xsb, gu, hb, yacc, pb, wk7, wv7, wq7, wo7, xc7, fence,
           sem, ksem, xsem, gsem, usem, dsem, osem, fsem):
    def cp(src, dst, k):
        return pltpu.make_async_copy(src, dst, sem.at[k])

    def wcp(part, dst, k):
        return cp(wqkv_h.at[:, pl.ds(part * D, D)], dst, k)

    def xcp(j):
        rs = pl.ds(j * HT, HT) if j < 2 else pl.ds((j - 1) * TM, TM)
        return pltpu.make_async_copy(xa_h.at[rs, :], xa.at[rs, :], xsem.at[j])

    def kcp(g, half):
        c0 = (g + 4 * half) * 128
        return pltpu.make_async_copy(wqkv_h.at[:, pl.ds(D + c0, 128)], wk.at[:, pl.ds(c0, 128)], ksem.at[g])

    def gcp(i):
        cs = pl.ds(GDMA[i], GDMA[i + 1] - GDMA[i])
        return pltpu.make_async_copy(wg_h.at[:, cs], wg.at[:, cs], gsem.at[i])

    def ucp(i):
        cs = pl.ds(UDMA[i], UDMA[i + 1] - UDMA[i])
        return pltpu.make_async_copy(wu_h.at[:, cs], wu.at[:, cs], usem.at[i])

    def dcp(i):
        rs = pl.ds(FCUT[i], FCUT[i + 1] - FCUT[i])
        return pltpu.make_async_copy(wd_h.at[rs, :], wd.at[rs, :], dsem.at[i])

    def ocp(t):
        rs = pl.ds(t * TM, TM)
        return pltpu.make_async_copy(ob.at[rs, :], out_h.at[rs, :], osem.at[t])

    def qcp(q):
        rs, cs = pl.ds((NT - 1) * TM + PIECES[q][0], HT), pl.ds(*PIECES[q][1:])
        return pltpu.make_async_copy(ob.at[rs, cs], out_h.at[rs, cs], osem.at[NT - 1])

    def fcp(i):
        return pltpu.make_async_copy(wr_h, fence.at[i], fsem.at[i])

    def start(*cs):
        for c in cs:
            c.start()

    def wait(*cs):
        for c in cs:
            c.wait()

    def fold7(w_ref, dst, g, lent):
        t = [_nt(bdt[:, c * 128:(c + 1) * 128], w_ref[:, c * 128:(c + 1) * 128]) * LOG2E for c in (g, g + 4)]
        for q in range(2):
            p = 2 * g + q
            heads = [[x[r0:r0 + DH] - x[r0 + p:r0 + p + 1] for x in t] for r0 in (q * 64, q * 64 + DH)]
            if p == 0:
                lent = [[x[0:8] for x in h] for h in heads]
                heads = [[x[8:] for x in h] for h in heads]
                rs = slice(0, DH - 8)
            else:
                row = lax.broadcasted_iota(jnp.int32, (8, D), 0) == p
                heads = [[jnp.concatenate([jnp.where(row, y, x[0:8]), x[8:]], axis=0) for x, y in zip(h, l)]
                         for h, l in zip(heads, lent)]
                rs = slice(p * DH - 8, (p + 1) * DH - 8)
            cs = [_lhs_combos(u[:, :HD], u[:, HD:], v[:, :HD], v[:, HD:]) for u, v in heads]
            for j in range(7):
                dst[j, rs, :] = _pack(cs[0][j], cs[1][j])
        return lent

    def prep_wv():
        for g in range(4):
            ta = _planes(wv[:, g * 128:(g + 1) * 128].T)
            tb = _planes(wv[:, (g + 4) * 128:(g + 5) * 128].T)
            cs = [_lhs_combos(u[:, :HD], u[:, HD:], v[:, :HD], v[:, HD:]) for u, v in zip(ta, tb)]
            for j in range(7):
                wv7[j, g * 64:(g + 1) * 64, :] = _pack(cs[0][j], cs[1][j])

    def rhs7(src, corners, nr, dst, never):
        prev = None
        for r in range(0, nr, 16):
            rd = slice(r // 2, r // 2 + 8)
            for c in range(0, HD, 128):
                cd = slice(c, c + 128)
                raw = [src[r0 + r:r0 + r + 16, c0 + c:c0 + c + 128] for r0, c0 in corners]
                dst[1, rd, cd] = pltpu.bitcast(raw[0], U32)
                dst[4, rd, cd] = pltpu.bitcast(raw[3], U32)
                b = [_planes(x) for x in raw]
                for j, u, v, op in RHS_SUMS:
                    bu = b[u] if never is None or prev is None else [jnp.where(never, prev, x) for x in b[u]]
                    prev = op(bu[0], b[v][0])
                    dst[j, rd, cd] = _pack(prev, op(bu[1], b[v][1]))

    def prep_x(t, never=None):
        r0 = t * TM
        rhs7(xa, ((r0, 0), (r0 + HT, 0), (r0, HD), (r0 + HT, HD)), HT, xc7.at[t], never)

    def prep_wo():
        rhs7(wo, ((0, 0), (0, HD), (HD, 0), (HD, HD)), HD, wo7, None)

    def products(w7, t, order, never, prev=None):
        return _ordered(_nt, lambda j: _unpack(w7[j]), lambda j: _unpack(xc7[t, j]), order, never, prev)

    def free_products(w7, t, js):
        return {j: _nt(_unpack(w7[j]), _unpack(xc7[t, j])) for j in js}

    def kv_accumulate(first, mk, mv):
        ep, en, rp, rn = _dual_softmax_parts(_assemble_logits(mk))
        php = (ep * rp[:, None]).reshape(H // 2, 64, TM)
        phn = (en * rn[:, None]).reshape(H // 2, 64, TM)
        ph = jnp.concatenate([php, phn], axis=1)
        zz = ph[:, :, 0:128]
        for c in range(1, TM // 128):
            zz = zz + ph[:, :, c * 128:(c + 1) * 128]
        zacc[...] = zz if first else zacc[...] + zz
        phb = ph.astype(BF)
        vT = _assemble(mv).astype(BF)
        for j in range(H // 2):
            u = _nt(vT[j * 64:(j + 1) * 64], phb[j])
            kvacc[j] = u if first else kvacc[j] + u

    def kv_update(t, never):
        mk, prev = products(wk7, t, PORD, never)
        kv_accumulate(False, mk, products(wv7, t, PORD, never, prev)[0])

    def finalize_kv():
        r3 = lax.broadcasted_iota(jnp.int32, kvacc.shape, 1)
        c3 = lax.broadcasted_iota(jnp.int32, kvacc.shape, 2)
        same_head = (r3 >> 5) == (c3 & 1)
        kvt[...] = pltpu.bitcast(jnp.where(same_head, kvacc[...], 0.0).reshape(D, 128).astype(BF), U32)
        zb[...] = jnp.broadcast_to(jnp.sum(zacc[...], axis=2, keepdims=True), zb.shape)

    def router(t, bv, bi):
        rs = slice(t * TM, (t + 1) * TM)
        xf = xa[rs, :].astype(F32)
        gb[rs, :] = jnp.broadcast_to(jax.nn.sigmoid(_rowdot(xf, gw[...].astype(F32))), (TM, 128))
        r = _rowdot(xf, wr[...].astype(F32)).astype(BF).astype(F32)
        r = jnp.broadcast_to(jnp.where(r != r, -jnp.inf, r), (TM, 128))
        row = lax.broadcasted_iota(jnp.int32, (8, 128), 0) + t * TM
        for k in range(TM // 8):
            rk = r[k * 8:(k + 1) * 8]
            better = rk > bv
            bv = jnp.where(better, rk, bv)
            bi = jnp.where(better, row + k * 8, bi)
        return bv, bi

    def gate_up(i, never):
        acc = None
        for c0 in range(FCUT[i], FCUT[i + 1], 128):
            for m, w_ref in enumerate((wg, wu)):
                acc = jnp.zeros((8, 128), F32) if acc is None else jnp.where(never, acc, 0.0)
                acc = _matvec(w_ref, xsb, 0, D, c0, acc)
                gu[m * 8:(m + 1) * 8, c0:c0 + 128] = acc

    def hidden():
        gg = jnp.sum(gu[0:8, :], axis=0, keepdims=True)
        uu = jnp.sum(gu[8:16, :], axis=0, keepdims=True)
        hb[...] = jnp.broadcast_to(gg * jax.nn.sigmoid(gg) * uu, (128, F)).T

    def down(i, never):
        acc = None
        for c0 in range(0, D, 128):
            cs = slice(c0, c0 + 128)
            acc = jnp.zeros((8, 128), F32) if acc is None else jnp.where(never, acc, 0.0)
            acc = _matvec(wd, hb, FCUT[i], FCUT[i + 1], c0, acc)
            yacc[:, cs] = acc if i == 0 else yacc[:, cs] + acc

    def attend(t, qorder, never, y=None, idx=None):
        r0 = t * TM
        ep, en, rp, rn = _dual_softmax_parts(_assemble_logits(products(wq7, t, qorder, never)[0]))
        z4 = zb[...].reshape(H // 2, 2, 8, 8, 128)
        zp = jnp.concatenate([z4[:, 0]] * (TM // 128), axis=-1)
        zn = jnp.concatenate([z4[:, 1]] * (TM // 128), axis=-1)
        den = _rot(_red8(ep * zp, jnp.add) * rp + _red8(en * zn, jnp.add) * rn, jnp.add) + 1e-6
        rd = _rcp(den)
        php = (ep * (rp * rd)[:, None]).reshape(H // 2, 64, TM)
        phn = (en * (rn * rd)[:, None]).reshape(H // 2, 64, TM)
        phb = jnp.concatenate([php, phn], axis=1).astype(BF)
        oT = jnp.concatenate([_nn(_unpack(kvt[j * 32:(j + 1) * 32, :]), phb[j]) for j in range(H // 2)], axis=0)
        oc = _lhs_combos(oT[:HD, :HT], oT[HD:, :HT], oT[:HD, HT:], oT[HD:, HT:])
        a = _assemble(_ordered(_nn, lambda j: oc[j].astype(BF).T, lambda j: _unpack(wo7[j]), OORD, never)[0])
        g = jnp.concatenate([gb[r0:r0 + TM, :]] * (D // 128), axis=1)
        b = xa[r0:r0 + TM, :].astype(F32)
        if y is not None:
            b = jnp.where(lax.broadcasted_iota(jnp.int32, (TM, D), 0) == idx - r0, b + y, b)
        res = (g * a + (1.0 - g) * b).astype(BF)
        if t < NT - 1:
            ob[r0:r0 + TM, :] = res
            start(ocp(t))
        else:
            for q, (rq, cq, wq_) in enumerate(PIECES):
                ob[r0 + rq:r0 + rq + HT, cq:cq + wq_] = res[rq:rq + HT, cq:cq + wq_]
                start(qcp(q))

    start(cp(wphi_h, wphi, 0), kcp(0, 0), kcp(0, 1), kcp(1, 0), kcp(1, 1), cp(wr_h, wr, 3), cp(gw_h, gw, 4),
          *[fcp(i) for i in range(4)])
    jj = lax.broadcasted_iota(jnp.int32, (128, DH), 0)
    ff = lax.broadcasted_iota(jnp.int32, (128, DH), 1)
    pick = jnp.where((jj & (DH - 1)) == ff, 1.0, 0.0).astype(BF)
    j2 = lax.broadcasted_iota(jnp.int32, (128, 128), 0)
    c2 = lax.broadcasted_iota(jnp.int32, (128, 128), 1)
    keep = (c2 >> 5) == (j2 >> 5)
    wait(cp(wphi_h, wphi, 0))
    bd = _nt(pick, wphi[...])
    for g in range(8):
        bdt[:, g * 128:(g + 1) * 128] = jnp.where(keep, bd[:, g * 128:(g + 1) * 128], 0.0).astype(BF)
    never = jnp.max(jnp.where(bd[0:8, 0:128] > 0.0, 1, 0)) < 0
    z0 = jnp.where(never, 1, 0)
    z8 = pl.ds(pl.multiple_of(z0 * 8, 8), 8)
    for r in (wk7, wv7, wq7, wo7):
        r[z0, 0:8, 0:128] = jnp.zeros((8, 128), U32)
    xc7[z0, 0, 0:8, 0:128] = jnp.zeros((8, 128), U32)
    for r in (gb, xsb, hb):
        r[z8, :] = jnp.zeros((8, 128), F32)
    for r in (kvacc, zacc, zb):
        r[z0, 0:8, :] = jnp.zeros((8, 128), F32)
    kvt[z8, :] = jnp.zeros((8, 128), U32)
    gu[z8, 0:128] = jnp.zeros((8, 128), F32)

    lent = None
    for g in range(4):
        wait(kcp(g, 0))
        start(*((kcp(g + 2, 0), kcp(g + 2, 1)) if g < 2 else (xcp(g - 2),)))
        wait(kcp(g, 1))
        lent = fold7(wk, wk7, g, lent)
    wait(xcp(0))
    start(wcp(2, wv, 1))
    wait(xcp(1))
    wait(cp(wr_h, wr, 3), cp(gw_h, gw, 4))
    prep_x(0)
    mk = free_products(wk7, 0, (1, 4, 2, 3))
    bv = jnp.full((8, 128), -jnp.inf, F32)
    bi = lax.broadcasted_iota(jnp.int32, (8, 128), 0)
    bv, bi = router(0, bv, bi)
    wait(wcp(2, wv, 1))
    start(xcp(2), xcp(3), xcp(4), gcp(0))
    wait(fcp(0))
    prep_wv()
    mk.update(free_products(wk7, 0, (0, 6, 5)))
    kv_accumulate(True, mk, free_products(wv7, 0, range(7)))
    wait(xcp(2), xcp(3))
    start(gcp(1), ucp(0), gcp(2))
    wait(xcp(4))
    prep_x(1)
    order = ((0, 4), (0, 1), (0, 2), (0, 3), (1, 1), (0, 0), (0, 6), (1, 4), (0, 5), (1, 2), (1, 3), (1, 0), (1, 6), (1, 5))
    m, _ = _ordered(_nt, lambda s: _unpack((wk7, wv7)[s[0]][s[1]]), lambda s: _unpack(xc7[1, s[1]]), order, never)
    kv_accumulate(False, [m[0, j] for j in range(7)], [m[1, j] for j in range(7)])
    prep_x(2, never)
    for t in range(1, NT):
        bv, bi = router(t, bv, bi)
    rmax = jnp.max(bv, axis=0, keepdims=True)
    idx = jnp.min(jnp.where(bv == rmax, bi, S))
    rsel = jax.nn.sigmoid(rmax)
    blk = pl.ds(pl.multiple_of((idx >> 4) << 4, 16), 16)
    routed = lax.broadcasted_iota(jnp.int32, (16, D), 0) == (idx & 15)
    xs = jnp.sum(jnp.where(routed, xa[blk, :].astype(F32), 0.0), axis=0, keepdims=True)
    xsb[...] = jnp.broadcast_to(xs, (128, D)).T
    wait(gcp(0), gcp(1), ucp(0))
    start(gcp(3), ucp(1))
    wait(fcp(1))
    kv_update(2, never)
    prep_x(3, never)
    gate_up(0, never)
    wait(gcp(2), gcp(3), ucp(1))
    start(wcp(0, wq, 2), cp(wo_h, wo, 5))
    wait(fcp(2))
    kv_update(3, never)
    gate_up(1, never)
    wait(wcp(0, wq, 2), cp(wo_h, wo, 5))
    start(dcp(0), dcp(1))
    wait(fcp(3))
    for g in range(4):
        lent = fold7(wq, wq7, g, lent)
    finalize_kv()
    hidden()
    prep_wo()
    attend(0, PORD, never)
    wait(dcp(0), dcp(1))
    attend(1, QORD, never)
    down(0, never)
    wait(ocp(0))
    attend(2, QORD, never)
    down(1, never)
    wait(ocp(1))
    y = jnp.sum(yacc[...], axis=0, keepdims=True) * jnp.concatenate([rsel] * (D // 128), axis=1)
    attend(3, PORD, never, y, idx)
    wait(ocp(2))

    @pl.when(idx < (NT - 1) * TM)
    def _():
        gsel = jnp.concatenate([gb[blk, :]] * (D // 128), axis=1)
        old = ob[blk, :].astype(F32)
        pb[...] = jnp.where(routed, old + (1.0 - gsel) * y, old).astype(BF)
        patch = cp(pb, out_h.at[blk, :], 7)
        patch.start()
        patch.wait()

    wait(*[qcp(q) for q in range(len(PIECES))])


@jax.jit
def pallas_gated_mix__linear_kernel_hedgehog__moe_arch_mod__prompt_kernel(
        A_x, A_wqkv, A_w_phi, A_wo, B_x, B_w_r, B_w_gate, B_w_up, B_w_down, gate_w):
    del B_x
    anyspec = pl.BlockSpec(memory_space=pl.ANY)
    V = pltpu.VMEM
    DMA = pltpu.SemaphoreType.DMA
    out = pl.pallas_call(
        kernel,
        out_shape=jax.ShapeDtypeStruct((S, D), BF),
        in_specs=[anyspec] * 9,
        out_specs=anyspec,
        scratch_shapes=[
            V((S, D), BF), V((D, D), BF), V((D, D), BF), V((D, D), BF), V((D, D), BF),
            V((D, F), BF), V((D, F), BF), V((F, D), BF),
            V((D, DH), BF), V((8, 128), BF), V((8, 128), BF), V((128, D), BF),
            V((S, D), BF), V((H // 2, 64, 128), F32), V((H // 2, 128, 128), F32),
            V((D // 2, 128), U32), V((H // 2, 128, 128), F32), V((S, 128), F32),
            V((D, 128), F32), V((16, F), F32), V((F, 128), F32), V((8, D), F32), V((16, D), BF),
            V((7, HD // 2 - 8, HD), U32), V((7, HD // 2, HD), U32), V((7, HD // 2 - 8, HD), U32),
            V((7, HD // 2, HD), U32), V((NT, 7, HT // 2, HD), U32), V((4, 8, 128), BF),
            DMA((8,)), DMA((4,)), DMA((NT + 1,)), DMA((4,)), DMA((2,)), DMA((2,)), DMA((NT,)), DMA((4,)),
        ],
        compiler_params=pltpu.CompilerParams(
            vmem_limit_bytes=110 * 2**20, flags={"XLA_TPU_EVENLY_DISTRIBUTE_CRITICAL_NODES": True}),
    )(A_x.reshape(S, D), A_wqkv, A_w_phi.reshape(D, DH), A_wo,
      B_w_r.reshape(8, 128), B_w_gate, B_w_up, B_w_down, gate_w.reshape(8, 128))
    return out.reshape(1, S, D)
```

```python
import jax
import jax.numpy as jnp
from jax import lax
from jax.experimental import pallas as pl
from jax.experimental.pallas import tpu as pltpu

S, D, H, DH, F = 2048, 1024, 32, 32, 3584
TM = 512
NT = S // TM
HT = TM // 2
HD = D // 2
GDMA = (0, 1024, 1792, 2304, F)
UDMA = (0, 1792, F)
FCUT = (0, 1792, F)
PIECES = ((0, HD, HD), (HT, 0, HD), (HT, HD, 256), (HT, HD + 256, 256),
          (0, 0, 128), (0, 128, 128), (0, 256, 128), (0, 384, 128))
PORD = (2, 4, 1, 3, 0, 6, 5)
QORD = (0, 3, 4, 6, 2, 1, 5)
OORD = (2, 4, 5, 1, 3, 0, 6)
LOG2E = 1.4426950408889634
BF = jnp.bfloat16
F32 = jnp.float32
U32 = jnp.uint32


def _nt(a, b):
    return lax.dot_general(a, b, (((1,), (1,)), ((), ())), preferred_element_type=F32)


def _nn(a, b):
    return jnp.dot(a, b, preferred_element_type=F32)


def _store_packed(ref, rows, c0, x):
    for c in range(0, x.shape[1], 128):
        ref[rows, c0 + c:c0 + c + 128] = pltpu.bitcast(x[:, c:c + 128].astype(BF), U32)


def _unpack(x):
    return pltpu.bitcast(x, BF)


def _rcp(x):
    r = pl.reciprocal(x, approx=True)
    return r * (2.0 - x * r)


def _red8(x4, op):
    r = x4[:, 0]
    for k in range(1, 8):
        r = op(r, x4[:, k])
    return r


def _rot(r, op):
    r = op(r, pltpu.roll(r, 4, r.ndim - 2))
    return op(r, pltpu.roll(r, 2, r.ndim - 2))


def _dual_softmax_parts(pT):
    p4 = pT.reshape(H // 2, 8, 8, pT.shape[1])
    mx = _rot(_red8(p4, jnp.maximum), jnp.maximum)
    mn = _rot(_red8(p4, jnp.minimum), jnp.minimum)
    ep = jnp.exp2(p4 - mx[:, None])
    en = jnp.exp2(mn[:, None] - p4)
    rp = _rcp(_rot(_red8(ep, jnp.add), jnp.add))
    rn = _rcp(_rot(_red8(en, jnp.add), jnp.add))
    return ep, en, rp, rn


def _rowdot(xf, w8):
    acc = xf[:, 0:128] * w8[0:1]
    for k in range(1, 8):
        acc = acc + xf[:, k * 128:(k + 1) * 128] * w8[k:k + 1]
    return jnp.sum(acc, axis=1, keepdims=True)


def _matvec(w_ref, v_ref, r0, r1, c0, acc):
    for r in range(r0, r1, 16):
        t = w_ref[r:r + 16, c0:c0 + 128].astype(F32) * v_ref[r:r + 16, :]
        acc = acc + t[0:8]
        acc = acc + t[8:16]
    return acc


def _lhs_combos(a11, a12, a21, a22):
    return (a11 + a22, a21 + a22, a11, a22, a11 + a12, a21 - a11, a12 - a22)


RHS_SUMS = ((0, 0, 3, jnp.add), (2, 1, 3, jnp.subtract), (3, 2, 0, jnp.subtract),
            (5, 0, 1, jnp.add), (6, 2, 3, jnp.add))


def _halves(m):
    c11 = m[0] + m[3] - m[4] + m[6]
    c12 = m[2] + m[4]
    c21 = m[1] + m[3]
    c22 = m[0] - m[1] + m[2] + m[5]
    return jnp.concatenate([c11, c12], axis=1), jnp.concatenate([c21, c22], axis=1)


def _assemble(m):
    return jnp.concatenate(_halves(m), axis=0)


def _assemble_logits(m):
    slot = lax.broadcasted_iota(jnp.int32, (8, TM), 0) >> 1
    rows = []
    for half in _halves(m):
        first = [jnp.zeros(slot.shape, F32), jnp.zeros(slot.shape, F32)]
        rest = []
        for p in range(1, 8):
            r0 = 64 * p - 16
            v = [half[r0 + 8 * k:r0 + 8 * k + 8] for k in range(8)]
            lent = slot == p % 4
            first[p // 4] = jnp.where(lent, v[p // 4], first[p // 4])
            v[p // 4] = jnp.where(lent, 0.0, v[p // 4])
            rest += v
        rows += first + [half[0:48]] + rest
    return jnp.concatenate(rows, axis=0)


def _ordered(dot, lhs, rhs, order, never, prev=None):
    m = {}
    for j in order:
        a = lhs(j)
        if prev is not None:
            tie = jnp.concatenate([prev[0:16, 0:128]] * (HD // 128), axis=1).astype(BF)
            a = jnp.concatenate([jnp.where(never, tie, a[0:16]), a[16:]], axis=0)
        prev = m[j] = dot(a, rhs(j))
    return m, prev


def kernel(xa_h, wqkv_h, wphi_h, wo_h, wr_h, wg_h, wu_h, wd_h, gw_h, out_h,
           xa, wq, wk, wv, wo, wg, wu, wd, wphi, wr, gw, bdt,
           ob, kvacc, zacc, kvt, zb, gb, xsb, gu, hb, yacc, pb, wk7, wv7, wq7, wo7, xc7, fence,
           sem, ksem, xsem, gsem, usem, dsem, osem, fsem):
    def cp(src, dst, k):
        return pltpu.make_async_copy(src, dst, sem.at[k])

    def wcp(part, dst, k):
        return cp(wqkv_h.at[:, pl.ds(part * D, D)], dst, k)

    def xcp(j):
        rs = pl.ds(j * HT, HT) if j < 2 else pl.ds((j - 1) * TM, TM)
        return pltpu.make_async_copy(xa_h.at[rs, :], xa.at[rs, :], xsem.at[j])

    def kcp(g, half):
        c0 = (g + 4 * half) * 128
        return pltpu.make_async_copy(wqkv_h.at[:, pl.ds(D + c0, 128)], wk.at[:, pl.ds(c0, 128)], ksem.at[g])

    def gcp(i):
        cs = pl.ds(GDMA[i], GDMA[i + 1] - GDMA[i])
        return pltpu.make_async_copy(wg_h.at[:, cs], wg.at[:, cs], gsem.at[i])

    def ucp(i):
        cs = pl.ds(UDMA[i], UDMA[i + 1] - UDMA[i])
        return pltpu.make_async_copy(wu_h.at[:, cs], wu.at[:, cs], usem.at[i])

    def dcp(i):
        rs = pl.ds(FCUT[i], FCUT[i + 1] - FCUT[i])
        return pltpu.make_async_copy(wd_h.at[rs, :], wd.at[rs, :], dsem.at[i])

    def ocp(t):
        rs = pl.ds(t * TM, TM)
        return pltpu.make_async_copy(ob.at[rs, :], out_h.at[rs, :], osem.at[t])

    def qcp(q):
        rs, cs = pl.ds((NT - 1) * TM + PIECES[q][0], HT), pl.ds(*PIECES[q][1:])
        return pltpu.make_async_copy(ob.at[rs, cs], out_h.at[rs, cs], osem.at[NT - 1])

    def fcp(i):
        return pltpu.make_async_copy(wr_h, fence.at[i], fsem.at[i])

    def start(*cs):
        for c in cs:
            c.start()

    def wait(*cs):
        for c in cs:
            c.wait()

    def fold7(w_ref, dst, g, lent):
        slot = lax.broadcasted_iota(jnp.int32, (8, D), 0) >> 1
        t = [_nt(bdt[:, c * 128:(c + 1) * 128], w_ref[:, c * 128:(c + 1) * 128]) * LOG2E for c in (g, g + 4)]
        for q in range(2):
            p = 2 * g + q
            own = slot == p % 4
            pair = []
            for x in t:
                v = [x[q * 64 + 8 * k:q * 64 + 8 * k + 8] for k in range(8)]
                shift = _rot(jnp.where(own, v[p // 4], 0.0), jnp.add)
                pair.append([u - shift for u in v])
            if p == 0:
                lent = [v[:2] for v in pair]
                pair = [v[2:] for v in pair]
                rows = slice(0, DH - 8)
            else:
                for v, l in zip(pair, lent):
                    v[p // 4] = jnp.where(own, l[p // 4], v[p // 4])
                rows = slice(p * DH - 8, (p + 1) * DH - 8)
            u, w = [jnp.concatenate(v, axis=0) for v in pair]
            for j, c in enumerate(_lhs_combos(u[:, :HD], u[:, HD:], w[:, :HD], w[:, HD:])):
                _store_packed(dst.at[j], rows, 0, c)
        return lent

    def prep_wv():
        for g in range(4):
            u = wv[:, g * 128:(g + 1) * 128].T.astype(F32)
            w = wv[:, (g + 4) * 128:(g + 5) * 128].T.astype(F32)
            for j, c in enumerate(_lhs_combos(u[:, :HD], u[:, HD:], w[:, :HD], w[:, HD:])):
                _store_packed(wv7.at[j], slice(g * 64, (g + 1) * 64), 0, c)

    def rhs7(src, corners, nr, dst, never):
        prev = None
        for r in range(0, nr, 16):
            rd = slice(r // 2, r // 2 + 8)
            for c in range(0, HD, 128):
                raw = [src[r0 + r:r0 + r + 16, c0 + c:c0 + c + 128] for r0, c0 in corners]
                dst[1, rd, c:c + 128] = pltpu.bitcast(raw[0], U32)
                dst[4, rd, c:c + 128] = pltpu.bitcast(raw[3], U32)
                b = [x.astype(F32) for x in raw]
                for j, u, v, op in RHS_SUMS:
                    bu = b[u] if never is None or prev is None else jnp.where(never, prev, b[u])
                    prev = op(bu, b[v])
                    _store_packed(dst.at[j], rd, c, prev)

    def prep_x(t, never=None):
        r0 = t * TM
        rhs7(xa, ((r0, 0), (r0 + HT, 0), (r0, HD), (r0 + HT, HD)), HT, xc7.at[t], never)

    def prep_wo():
        rhs7(wo, ((0, 0), (0, HD), (HD, 0), (HD, HD)), HD, wo7, None)

    def products(w7, t, order, never, prev=None):
        return _ordered(_nt, lambda j: _unpack(w7[j]), lambda j: _unpack(xc7[t, j]), order, never, prev)

    def free_products(w7, t, js):
        return {j: _nt(_unpack(w7[j]), _unpack(xc7[t, j])) for j in js}

    def kv_accumulate(first, mk, mv):
        ep, en, rp, rn = _dual_softmax_parts(_assemble_logits(mk))
        php = (ep * rp[:, None]).reshape(H // 2, 64, TM)
        phn = (en * rn[:, None]).reshape(H // 2, 64, TM)
        ph = jnp.concatenate([php, phn], axis=1)
        zz = ph[:, :, 0:128]
        for c in range(1, TM // 128):
            zz = zz + ph[:, :, c * 128:(c + 1) * 128]
        zacc[...] = zz if first else zacc[...] + zz
        phb = ph.astype(BF)
        vT = _assemble(mv).astype(BF)
        for j in range(H // 2):
            u = _nt(vT[j * 64:(j + 1) * 64], phb[j])
            kvacc[j] = u if first else kvacc[j] + u

    def kv_update(t, never):
        mk, prev = products(wk7, t, PORD, never)
        kv_accumulate(False, mk, products(wv7, t, PORD, never, prev)[0])

    def finalize_kv():
        r3 = lax.broadcasted_iota(jnp.int32, kvacc.shape, 1)
        c3 = lax.broadcasted_iota(jnp.int32, kvacc.shape, 2)
        same_head = (r3 >> 5) == (c3 & 1)
        kvt[...] = pltpu.bitcast(jnp.where(same_head, kvacc[...], 0.0).reshape(D, 128).astype(BF), U32)
        zb[...] = jnp.broadcast_to(jnp.sum(zacc[...], axis=2, keepdims=True), zb.shape)

    def router(t, bv, bi):
        rs = slice(t * TM, (t + 1) * TM)
        xf = xa[rs, :].astype(F32)
        gb[rs, :] = jnp.broadcast_to(jax.nn.sigmoid(_rowdot(xf, gw[...].astype(F32))), (TM, 128))
        r = _rowdot(xf, wr[...].astype(F32)).astype(BF).astype(F32)
        r = jnp.broadcast_to(jnp.where(r != r, -jnp.inf, r), (TM, 128))
        row = lax.broadcasted_iota(jnp.int32, (8, 128), 0) + t * TM
        for k in range(TM // 8):
            rk = r[k * 8:(k + 1) * 8]
            better = rk > bv
            bv = jnp.where(better, rk, bv)
            bi = jnp.where(better, row + k * 8, bi)
        return bv, bi

    def gate_up(i, never):
        acc = None
        for c0 in range(FCUT[i], FCUT[i + 1], 128):
            for m, w_ref in enumerate((wg, wu)):
                acc = jnp.zeros((8, 128), F32) if acc is None else jnp.where(never, acc, 0.0)
                acc = _matvec(w_ref, xsb, 0, D, c0, acc)
                gu[m * 8:(m + 1) * 8, c0:c0 + 128] = acc

    def hidden():
        gg = jnp.sum(gu[0:8, :], axis=0, keepdims=True)
        uu = jnp.sum(gu[8:16, :], axis=0, keepdims=True)
        hb[...] = jnp.broadcast_to(gg * jax.nn.sigmoid(gg) * uu, (128, F)).T

    def down(i, never):
        acc = None
        for c0 in range(0, D, 128):
            cs = slice(c0, c0 + 128)
            acc = jnp.zeros((8, 128), F32) if acc is None else jnp.where(never, acc, 0.0)
            acc = _matvec(wd, hb, FCUT[i], FCUT[i + 1], c0, acc)
            yacc[:, cs] = acc if i == 0 else yacc[:, cs] + acc

    def attend(t, qorder, never, y=None, idx=None):
        r0 = t * TM
        ep, en, rp, rn = _dual_softmax_parts(_assemble_logits(products(wq7, t, qorder, never)[0]))
        z4 = zb[...].reshape(H // 2, 2, 8, 8, 128)
        zp = jnp.concatenate([z4[:, 0]] * (TM // 128), axis=-1)
        zn = jnp.concatenate([z4[:, 1]] * (TM // 128), axis=-1)
        den = _rot(_red8(ep * zp, jnp.add) * rp + _red8(en * zn, jnp.add) * rn, jnp.add) + 1e-6
        rd = _rcp(den)
        php = (ep * (rp * rd)[:, None]).reshape(H // 2, 64, TM)
        phn = (en * (rn * rd)[:, None]).reshape(H // 2, 64, TM)
        phb = jnp.concatenate([php, phn], axis=1).astype(BF)
        oT = jnp.concatenate([_nn(_unpack(kvt[j * 32:(j + 1) * 32, :]), phb[j]) for j in range(H // 2)], axis=0)
        oc = _lhs_combos(oT[:HD, :HT], oT[HD:, :HT], oT[:HD, HT:], oT[HD:, HT:])
        a = _assemble(_ordered(_nn, lambda j: oc[j].astype(BF).T, lambda j: _unpack(wo7[j]), OORD, never)[0])
        g = jnp.concatenate([gb[r0:r0 + TM, :]] * (D // 128), axis=1)
        b = xa[r0:r0 + TM, :].astype(F32)
        if y is not None:
            b = jnp.where(lax.broadcasted_iota(jnp.int32, (TM, D), 0) == idx - r0, b + y, b)
        res = (g * a + (1.0 - g) * b).astype(BF)
        if t < NT - 1:
            ob[r0:r0 + TM, :] = res
            start(ocp(t))
        else:
            for q, (rq, cq, wq_) in enumerate(PIECES):
                ob[r0 + rq:r0 + rq + HT, cq:cq + wq_] = res[rq:rq + HT, cq:cq + wq_]
                start(qcp(q))

    start(cp(wphi_h, wphi, 0), kcp(0, 0), kcp(0, 1), kcp(1, 0), kcp(1, 1), cp(wr_h, wr, 3), cp(gw_h, gw, 4),
          *[fcp(i) for i in range(4)])
    jj = lax.broadcasted_iota(jnp.int32, (128, DH), 0)
    ff = lax.broadcasted_iota(jnp.int32, (128, DH), 1)
    pick = jnp.where(((jj & 63) >> 1) == ff, 1.0, 0.0).astype(BF)
    j2 = lax.broadcasted_iota(jnp.int32, (128, 128), 0)
    c2 = lax.broadcasted_iota(jnp.int32, (128, 128), 1)
    keep = (c2 >> 5) == (j2 >> 6) * 2 + (j2 & 1)
    wait(cp(wphi_h, wphi, 0))
    bd = _nt(pick, wphi[...])
    for g in range(8):
        bdt[:, g * 128:(g + 1) * 128] = jnp.where(keep, bd[:, g * 128:(g + 1) * 128], 0.0).astype(BF)
    never = jnp.max(jnp.where(bd[0:8, 0:128] > 0.0, 1, 0)) < 0
    z0 = jnp.where(never, 1, 0)
    z8 = pl.ds(pl.multiple_of(z0 * 8, 8), 8)
    for r in (wk7, wv7, wq7, wo7):
        r[z0, 0:8, 0:128] = jnp.zeros((8, 128), U32)
    xc7[z0, 0, 0:8, 0:128] = jnp.zeros((8, 128), U32)
    for r in (gb, xsb, hb):
        r[z8, :] = jnp.zeros((8, 128), F32)
    for r in (kvacc, zacc, zb):
        r[z0, 0:8, :] = jnp.zeros((8, 128), F32)
    kvt[z8, :] = jnp.zeros((8, 128), U32)
    gu[z8, 0:128] = jnp.zeros((8, 128), F32)

    lent = None
    for g in range(4):
        wait(kcp(g, 0))
        start(*((kcp(g + 2, 0), kcp(g + 2, 1)) if g < 2 else (xcp(g - 2),)))
        wait(kcp(g, 1))
        lent = fold7(wk, wk7, g, lent)
    wait(xcp(0))
    start(wcp(2, wv, 1))
    wait(xcp(1))
    wait(cp(wr_h, wr, 3), cp(gw_h, gw, 4))
    prep_x(0)
    mk = free_products(wk7, 0, (1, 4, 2, 3))
    bv = jnp.full((8, 128), -jnp.inf, F32)
    bi = lax.broadcasted_iota(jnp.int32, (8, 128), 0)
    bv, bi = router(0, bv, bi)
    wait(wcp(2, wv, 1))
    start(xcp(2), xcp(3), xcp(4), gcp(0))
    wait(fcp(0))
    prep_wv()
    mk.update(free_products(wk7, 0, (0, 6, 5)))
    kv_accumulate(True, mk, free_products(wv7, 0, range(7)))
    wait(xcp(2), xcp(3))
    start(gcp(1), ucp(0), gcp(2))
    wait(xcp(4))
    prep_x(1)
    order = ((0, 4), (0, 1), (0, 2), (0, 3), (1, 1), (0, 0), (0, 6), (1, 4), (0, 5), (1, 2), (1, 3), (1, 0), (1, 6), (1, 5))
    m, _ = _ordered(_nt, lambda s: _unpack((wk7, wv7)[s[0]][s[1]]), lambda s: _unpack(xc7[1, s[1]]), order, never)
    kv_accumulate(False, [m[0, j] for j in range(7)], [m[1, j] for j in range(7)])
    prep_x(2, never)
    for t in range(1, NT):
        bv, bi = router(t, bv, bi)
    rmax = jnp.max(bv, axis=0, keepdims=True)
    idx = jnp.min(jnp.where(bv == rmax, bi, S))
    rsel = jax.nn.sigmoid(rmax)
    blk = pl.ds(pl.multiple_of((idx >> 4) << 4, 16), 16)
    routed = lax.broadcasted_iota(jnp.int32, (16, D), 0) == (idx & 15)
    xs = jnp.sum(jnp.where(routed, xa[blk, :].astype(F32), 0.0), axis=0, keepdims=True)
    xsb[...] = jnp.broadcast_to(xs, (128, D)).T
    wait(gcp(0), gcp(1), ucp(0))
    start(gcp(3), ucp(1))
    wait(fcp(1))
    kv_update(2, never)
    prep_x(3, never)
    gate_up(0, never)
    wait(gcp(2), gcp(3), ucp(1))
    start(wcp(0, wq, 2), cp(wo_h, wo, 5))
    wait(fcp(2))
    kv_update(3, never)
    gate_up(1, never)
    wait(wcp(0, wq, 2), cp(wo_h, wo, 5))
    start(dcp(0), dcp(1))
    wait(fcp(3))
    for g in range(4):
        lent = fold7(wq, wq7, g, lent)
    finalize_kv()
    hidden()
    prep_wo()
    attend(0, PORD, never)
    wait(dcp(0), dcp(1))
    attend(1, QORD, never)
    down(0, never)
    wait(ocp(0))
    attend(2, QORD, never)
    down(1, never)
    wait(ocp(1))
    y = jnp.sum(yacc[...], axis=0, keepdims=True) * jnp.concatenate([rsel] * (D // 128), axis=1)
    attend(3, PORD, never, y, idx)
    wait(ocp(2))

    @pl.when(idx < (NT - 1) * TM)
    def _():
        gsel = jnp.concatenate([gb[blk, :]] * (D // 128), axis=1)
        old = ob[blk, :].astype(F32)
        pb[...] = jnp.where(routed, old + (1.0 - gsel) * y, old).astype(BF)
        patch = cp(pb, out_h.at[blk, :], 7)
        patch.start()
        patch.wait()

    wait(*[qcp(q) for q in range(len(PIECES))])


@jax.jit
def pallas_gated_mix__linear_kernel_hedgehog__moe_arch_mod__prompt_kernel(
        A_x, A_wqkv, A_w_phi, A_wo, B_x, B_w_r, B_w_gate, B_w_up, B_w_down, gate_w):
    del B_x
    anyspec = pl.BlockSpec(memory_space=pl.ANY)
    V = pltpu.VMEM
    DMA = pltpu.SemaphoreType.DMA
    out = pl.pallas_call(
        kernel,
        out_shape=jax.ShapeDtypeStruct((S, D), BF),
        in_specs=[anyspec] * 9,
        out_specs=anyspec,
        scratch_shapes=[
            V((S, D), BF), V((D, D), BF), V((D, D), BF), V((D, D), BF), V((D, D), BF),
            V((D, F), BF), V((D, F), BF), V((F, D), BF),
            V((D, DH), BF), V((8, 128), BF), V((8, 128), BF), V((128, D), BF),
            V((S, D), BF), V((H // 2, 64, 128), F32), V((H // 2, 128, 128), F32),
            V((D // 2, 128), U32), V((H // 2, 128, 128), F32), V((S, 128), F32),
            V((D, 128), F32), V((16, F), F32), V((F, 128), F32), V((8, D), F32), V((16, D), BF),
            V((7, HD // 2 - 8, HD), U32), V((7, HD // 2, HD), U32), V((7, HD // 2 - 8, HD), U32),
            V((7, HD // 2, HD), U32), V((NT, 7, HT // 2, HD), U32), V((4, 8, 128), BF),
            DMA((8,)), DMA((4,)), DMA((NT + 1,)), DMA((4,)), DMA((2,)), DMA((2,)), DMA((NT,)), DMA((4,)),
        ],
        compiler_params=pltpu.CompilerParams(
            vmem_limit_bytes=110 * 2**20, flags={"XLA_TPU_EVENLY_DISTRIBUTE_CRITICAL_NODES": True}),
    )(A_x.reshape(S, D), A_wqkv, A_w_phi.reshape(D, DH), A_wo,
      B_w_r.reshape(8, 128), B_w_gate, B_w_up, B_w_down, gate_w.reshape(8, 128))
    return out.reshape(1, S, D)
```

```python
import jax
import jax.numpy as jnp
from jax import lax
from jax.experimental import pallas as pl
from jax.experimental.pallas import tpu as pltpu

S, D, H, DH, F = 2048, 1024, 32, 32, 3584
TM = 512
NT = S // TM
HT = TM // 2
HD = D // 2
GDMA = (0, 1024, 1792, 2304, F)
UDMA = (0, 1792, F)
FCUT = (0, 1792, F)
PIECES = ((0, HD, HD), (HT, 0, HD), (HT, HD, 256), (HT, HD + 256, 256),
          (0, 0, 128), (0, 128, 128), (0, 256, 128), (0, 384, 128))
PORD = (2, 4, 1, 3, 0, 6, 5)
QORD = (1, 3, 4, 2, 0, 6, 5)
OORD = (2, 4, 5, 1, 3, 0, 6)
LOG2E = 1.4426950408889634
BF = jnp.bfloat16
F32 = jnp.float32
U32 = jnp.uint32


def _nt(a, b):
    return lax.dot_general(a, b, (((1,), (1,)), ((), ())), preferred_element_type=F32)


def _nn(a, b):
    return jnp.dot(a, b, preferred_element_type=F32)


def _store_packed(ref, rows, c0, x):
    for c in range(0, x.shape[1], 128):
        ref[rows, c0 + c:c0 + c + 128] = pltpu.bitcast(x[:, c:c + 128].astype(BF), U32)


def _unpack(x):
    return pltpu.bitcast(x, BF)


def _rcp(x):
    r = pl.reciprocal(x, approx=True)
    return r * (2.0 - x * r)


def _red8(x4, op):
    r = x4[:, 0]
    for k in range(1, 8):
        r = op(r, x4[:, k])
    return r


def _rot(r, op):
    r = op(r, pltpu.roll(r, 4, r.ndim - 2))
    return op(r, pltpu.roll(r, 2, r.ndim - 2))


def _dual_softmax_parts(pT):
    p4 = pT.reshape(H // 2, 8, 8, pT.shape[1])
    mx = _rot(_red8(p4, jnp.maximum), jnp.maximum)
    mn = _rot(_red8(p4, jnp.minimum), jnp.minimum)
    ep = jnp.exp2(p4 - mx[:, None])
    en = jnp.exp2(mn[:, None] - p4)
    rp = _rcp(_rot(_red8(ep, jnp.add), jnp.add))
    rn = _rcp(_rot(_red8(en, jnp.add), jnp.add))
    return ep, en, rp, rn


def _rowdot(xf, w8):
    acc = xf[:, 0:128] * w8[0:1]
    for k in range(1, 8):
        acc = acc + xf[:, k * 128:(k + 1) * 128] * w8[k:k + 1]
    return jnp.sum(acc, axis=1, keepdims=True)


def _matvec(w_ref, v_ref, r0, r1, c0, acc):
    for r in range(r0, r1, 16):
        t = w_ref[r:r + 16, c0:c0 + 128].astype(F32) * v_ref[r:r + 16, :]
        acc = acc + t[0:8]
        acc = acc + t[8:16]
    return acc


def _lhs_combos(a11, a12, a21, a22):
    return (a11 + a22, a21 + a22, a11, a22, a11 + a12, a21 - a11, a12 - a22)


RHS_SUMS = ((0, 0, 3, jnp.add), (2, 1, 3, jnp.subtract), (3, 2, 0, jnp.subtract),
            (5, 0, 1, jnp.add), (6, 2, 3, jnp.add))


def _halves(m):
    c11 = m[0] + m[3] - m[4] + m[6]
    c12 = m[2] + m[4]
    c21 = m[1] + m[3]
    c22 = m[0] - m[1] + m[2] + m[5]
    return jnp.concatenate([c11, c12], axis=1), jnp.concatenate([c21, c22], axis=1)


def _assemble(m):
    return jnp.concatenate(_halves(m), axis=0)


def _assemble_logits(m):
    slot = lax.broadcasted_iota(jnp.int32, (8, TM), 0) >> 1
    rows = []
    for half in _halves(m):
        first = [jnp.zeros(slot.shape, F32), jnp.zeros(slot.shape, F32)]
        rest = []
        for p in range(1, 8):
            r0 = 64 * p - 16
            v = [half[r0 + 8 * k:r0 + 8 * k + 8] for k in range(8)]
            lent = slot == p % 4
            first[p // 4] = jnp.where(lent, v[p // 4], first[p // 4])
            v[p // 4] = jnp.where(lent, 0.0, v[p // 4])
            rest += v
        rows += first + [half[0:48]] + rest
    return jnp.concatenate(rows, axis=0)


def _ordered(dot, lhs, rhs, order, never, prev=None):
    m = {}
    for j in order:
        a = lhs(j)
        if prev is not None:
            tie = jnp.concatenate([prev[0:16, 0:128]] * (HD // 128), axis=1).astype(BF)
            a = jnp.concatenate([jnp.where(never, tie, a[0:16]), a[16:]], axis=0)
        prev = m[j] = dot(a, rhs(j))
    return m, prev


def _ordered_tn(lhs, rhs, order, never):
    m = {}
    prev = None
    for j in order:
        a = lhs(j)
        if prev is not None:
            tie = jnp.concatenate([prev[0:16, 0:128]] * (HD // 16), axis=0).astype(BF)
            a = jnp.concatenate([jnp.where(never, tie, a[:, 0:128]), a[:, 128:]], axis=1)
        prev = m[j] = lax.dot_general(a, rhs(j), (((0,), (0,)), ((), ())), preferred_element_type=F32)
    return m


def kernel(xa_h, wqkv_h, wphi_h, wo_h, wr_h, wg_h, wu_h, wd_h, gw_h, out_h,
           xa, wq, wk, wv, wo, wg, wu, wd, wphi, wr, gw, bdt,
           ob, kvacc, zacc, kvt, zb, gb, xsb, gu, hb, yacc, pb, wk7, wv7, wq7, wo7, xc7, fence,
           sem, ksem, xsem, gsem, usem, dsem, osem, fsem):
    def cp(src, dst, k):
        return pltpu.make_async_copy(src, dst, sem.at[k])

    def wcp(part, dst, k):
        return cp(wqkv_h.at[:, pl.ds(part * D, D)], dst, k)

    def xcp(j):
        rs = pl.ds(j * HT, HT) if j < 2 else pl.ds((j - 1) * TM, TM)
        return pltpu.make_async_copy(xa_h.at[rs, :], xa.at[rs, :], xsem.at[j])

    def kcp(g, half):
        c0 = (g + 4 * half) * 128
        return pltpu.make_async_copy(wqkv_h.at[:, pl.ds(D + c0, 128)], wk.at[:, pl.ds(c0, 128)], ksem.at[g])

    def gcp(i):
        cs = pl.ds(GDMA[i], GDMA[i + 1] - GDMA[i])
        return pltpu.make_async_copy(wg_h.at[:, cs], wg.at[:, cs], gsem.at[i])

    def ucp(i):
        cs = pl.ds(UDMA[i], UDMA[i + 1] - UDMA[i])
        return pltpu.make_async_copy(wu_h.at[:, cs], wu.at[:, cs], usem.at[i])

    def dcp(i):
        rs = pl.ds(FCUT[i], FCUT[i + 1] - FCUT[i])
        return pltpu.make_async_copy(wd_h.at[rs, :], wd.at[rs, :], dsem.at[i])

    def ocp(t):
        rs = pl.ds(t * TM, TM)
        return pltpu.make_async_copy(ob.at[rs, :], out_h.at[rs, :], osem.at[t])

    def qcp(q):
        rs, cs = pl.ds((NT - 1) * TM + PIECES[q][0], HT), pl.ds(*PIECES[q][1:])
        return pltpu.make_async_copy(ob.at[rs, cs], out_h.at[rs, cs], osem.at[NT - 1])

    def fcp(i):
        return pltpu.make_async_copy(wr_h, fence.at[i], fsem.at[i])

    def start(*cs):
        for c in cs:
            c.start()

    def wait(*cs):
        for c in cs:
            c.wait()

    def fold7(w_ref, dst, g, lent):
        slot = lax.broadcasted_iota(jnp.int32, (8, D), 0) >> 1
        t = [_nt(bdt[:, c * 128:(c + 1) * 128], w_ref[:, c * 128:(c + 1) * 128]) * LOG2E for c in (g, g + 4)]
        for q in range(2):
            p = 2 * g + q
            own = slot == p % 4
            pair = []
            for x in t:
                v = [x[q * 64 + 8 * k:q * 64 + 8 * k + 8] for k in range(8)]
                shift = _rot(jnp.where(own, v[p // 4], 0.0), jnp.add)
                pair.append([u - shift for u in v])
            if p == 0:
                lent = [v[:2] for v in pair]
                pair = [v[2:] for v in pair]
                rows = slice(0, DH - 8)
            else:
                for v, l in zip(pair, lent):
                    v[p // 4] = jnp.where(own, l[p // 4], v[p // 4])
                rows = slice(p * DH - 8, (p + 1) * DH - 8)
            u, w = [jnp.concatenate(v, axis=0) for v in pair]
            for j, c in enumerate(_lhs_combos(u[:, :HD], u[:, HD:], w[:, :HD], w[:, HD:])):
                _store_packed(dst.at[j], rows, 0, c)
        return lent

    def prep_wv():
        for g in range(4):
            u = wv[:, g * 128:(g + 1) * 128].T.astype(F32)
            w = wv[:, (g + 4) * 128:(g + 5) * 128].T.astype(F32)
            for j, c in enumerate(_lhs_combos(u[:, :HD], u[:, HD:], w[:, :HD], w[:, HD:])):
                _store_packed(wv7.at[j], slice(g * 64, (g + 1) * 64), 0, c)

    def rhs7(src, corners, nr, dst, never):
        prev = None
        for r in range(0, nr, 16):
            rd = slice(r // 2, r // 2 + 8)
            for c in range(0, HD, 128):
                raw = [src[r0 + r:r0 + r + 16, c0 + c:c0 + c + 128] for r0, c0 in corners]
                dst[1, rd, c:c + 128] = pltpu.bitcast(raw[0], U32)
                dst[4, rd, c:c + 128] = pltpu.bitcast(raw[3], U32)
                b = [x.astype(F32) for x in raw]
                for j, u, v, op in RHS_SUMS:
                    bu = b[u] if never is None or prev is None else jnp.where(never, prev, b[u])
                    prev = op(bu, b[v])
                    _store_packed(dst.at[j], rd, c, prev)

    def prep_x(t, never=None):
        r0 = t * TM
        rhs7(xa, ((r0, 0), (r0 + HT, 0), (r0, HD), (r0 + HT, HD)), HT, xc7.at[t], never)

    def prep_wo():
        rhs7(wo, ((0, 0), (0, HD), (HD, 0), (HD, HD)), HD, wo7, None)

    def products(w7, t, order, never, prev=None):
        return _ordered(_nt, lambda j: _unpack(w7[j]), lambda j: _unpack(xc7[t, j]), order, never, prev)

    def free_products(w7, t, js):
        return {j: _nt(_unpack(w7[j]), _unpack(xc7[t, j])) for j in js}

    def kv_accumulate(first, mk, mv):
        ep, en, rp, rn = _dual_softmax_parts(_assemble_logits(mk))
        php = (ep * rp[:, None]).reshape(H // 2, 64, TM)
        phn = (en * rn[:, None]).reshape(H // 2, 64, TM)
        ph = jnp.concatenate([php, phn], axis=1)
        zz = ph[:, :, 0:128]
        for c in range(1, TM // 128):
            zz = zz + ph[:, :, c * 128:(c + 1) * 128]
        zacc[...] = zz if first else zacc[...] + zz
        phb = ph.astype(BF)
        vT = _assemble(mv).astype(BF)
        for j in range(H // 2):
            u = _nt(vT[j * 64:(j + 1) * 64], phb[j])
            kvacc[j] = u if first else kvacc[j] + u

    def kv_update(t, never):
        mk, prev = products(wk7, t, PORD, never)
        kv_accumulate(False, mk, products(wv7, t, PORD, never, prev)[0])

    def finalize_kv():
        r3 = lax.broadcasted_iota(jnp.int32, kvacc.shape, 1)
        c3 = lax.broadcasted_iota(jnp.int32, kvacc.shape, 2)
        same_head = (r3 >> 5) == (c3 & 1)
        kvt[...] = pltpu.bitcast(jnp.where(same_head, kvacc[...], 0.0).reshape(D, 128).astype(BF), U32)
        zb[...] = jnp.broadcast_to(jnp.sum(zacc[...], axis=2, keepdims=True), zb.shape)

    def router(t, bv, bi):
        rs = slice(t * TM, (t + 1) * TM)
        xf = xa[rs, :].astype(F32)
        gb[rs, :] = jnp.broadcast_to(jax.nn.sigmoid(_rowdot(xf, gw[...].astype(F32))), (TM, 128))
        r = _rowdot(xf, wr[...].astype(F32)).astype(BF).astype(F32)
        r = jnp.broadcast_to(jnp.where(r != r, -jnp.inf, r), (TM, 128))
        row = lax.broadcasted_iota(jnp.int32, (8, 128), 0) + t * TM
        for k in range(TM // 8):
            rk = r[k * 8:(k + 1) * 8]
            better = rk > bv
            bv = jnp.where(better, rk, bv)
            bi = jnp.where(better, row + k * 8, bi)
        return bv, bi

    def gate_up(i, never):
        acc = None
        for c0 in range(FCUT[i], FCUT[i + 1], 128):
            for m, w_ref in enumerate((wg, wu)):
                acc = jnp.zeros((8, 128), F32) if acc is None else jnp.where(never, acc, 0.0)
                acc = _matvec(w_ref, xsb, 0, D, c0, acc)
                gu[m * 8:(m + 1) * 8, c0:c0 + 128] = acc

    def hidden():
        gg = jnp.sum(gu[0:8, :], axis=0, keepdims=True)
        uu = jnp.sum(gu[8:16, :], axis=0, keepdims=True)
        hb[...] = jnp.broadcast_to(gg * jax.nn.sigmoid(gg) * uu, (128, F)).T

    def down(i, never):
        acc = None
        for c0 in range(0, D, 128):
            cs = slice(c0, c0 + 128)
            acc = jnp.zeros((8, 128), F32) if acc is None else jnp.where(never, acc, 0.0)
            acc = _matvec(wd, hb, FCUT[i], FCUT[i + 1], c0, acc)
            yacc[:, cs] = acc if i == 0 else yacc[:, cs] + acc

    def attend(t, never, y=None, idx=None):
        r0 = t * TM
        ep, en, rp, rn = _dual_softmax_parts(_assemble_logits(products(wq7, t, QORD, never)[0]))
        z4 = zb[...].reshape(H // 2, 2, 8, 8, 128)
        zp = jnp.concatenate([z4[:, 0]] * (TM // 128), axis=-1)
        zn = jnp.concatenate([z4[:, 1]] * (TM // 128), axis=-1)
        den = _rot(_red8(ep * zp, jnp.add) * rp + _red8(en * zn, jnp.add) * rn, jnp.add) + 1e-6
        rd = _rcp(den)
        php = (ep * (rp * rd)[:, None]).reshape(H // 2, 64, TM)
        phn = (en * (rn * rd)[:, None]).reshape(H // 2, 64, TM)
        phb = jnp.concatenate([php, phn], axis=1).astype(BF)
        oT = jnp.concatenate([_nn(_unpack(kvt[j * 32:(j + 1) * 32, :]), phb[j]) for j in range(H // 2)], axis=0)
        oc = _lhs_combos(oT[:HD, :HT], oT[HD:, :HT], oT[:HD, HT:], oT[HD:, HT:])
        a = _assemble(_ordered_tn(lambda j: oc[j].astype(BF), lambda j: _unpack(wo7[j]), OORD, never))
        g = jnp.concatenate([gb[r0:r0 + TM, :]] * (D // 128), axis=1)
        b = xa[r0:r0 + TM, :].astype(F32)
        if y is not None:
            b = jnp.where(lax.broadcasted_iota(jnp.int32, (TM, D), 0) == idx - r0, b + y, b)
        res = (g * a + (1.0 - g) * b).astype(BF)
        if t < NT - 1:
            ob[r0:r0 + TM, :] = res
            start(ocp(t))
        else:
            for q, (rq, cq, wq_) in enumerate(PIECES):
                ob[r0 + rq:r0 + rq + HT, cq:cq + wq_] = res[rq:rq + HT, cq:cq + wq_]
                start(qcp(q))

    start(cp(wphi_h, wphi, 0), kcp(0, 0), kcp(0, 1), kcp(1, 0), kcp(1, 1), cp(wr_h, wr, 3), cp(gw_h, gw, 4),
          *[fcp(i) for i in range(4)])
    jj = lax.broadcasted_iota(jnp.int32, (128, DH), 0)
    ff = lax.broadcasted_iota(jnp.int32, (128, DH), 1)
    pick = jnp.where(((jj & 63) >> 1) == ff, 1.0, 0.0).astype(BF)
    j2 = lax.broadcasted_iota(jnp.int32, (128, 128), 0)
    c2 = lax.broadcasted_iota(jnp.int32, (128, 128), 1)
    keep = (c2 >> 5) == (j2 >> 6) * 2 + (j2 & 1)
    wait(cp(wphi_h, wphi, 0))
    bd = _nt(pick, wphi[...])
    for g in range(8):
        bdt[:, g * 128:(g + 1) * 128] = jnp.where(keep, bd[:, g * 128:(g + 1) * 128], 0.0).astype(BF)
    never = jnp.max(jnp.where(bd[0:8, 0:128] > 0.0, 1, 0)) < 0
    z0 = jnp.where(never, 1, 0)
    z8 = pl.ds(pl.multiple_of(z0 * 8, 8), 8)
    for r in (wk7, wv7, wq7, wo7):
        r[z0, 0:8, 0:128] = jnp.zeros((8, 128), U32)
    xc7[z0, 0, 0:8, 0:128] = jnp.zeros((8, 128), U32)
    for r in (gb, xsb, hb):
        r[z8, :] = jnp.zeros((8, 128), F32)
    for r in (kvacc, zacc, zb):
        r[z0, 0:8, :] = jnp.zeros((8, 128), F32)
    kvt[z8, :] = jnp.zeros((8, 128), U32)
    gu[z8, 0:128] = jnp.zeros((8, 128), F32)

    lent = None
    for g in range(4):
        wait(kcp(g, 0))
        start(*((kcp(g + 2, 0), kcp(g + 2, 1)) if g < 2 else (xcp(g - 2),)))
        wait(kcp(g, 1))
        lent = fold7(wk, wk7, g, lent)
    wait(xcp(0))
    start(wcp(2, wv, 1))
    wait(xcp(1))
    wait(cp(wr_h, wr, 3), cp(gw_h, gw, 4))
    prep_x(0)
    mk = free_products(wk7, 0, (1, 4, 2, 3))
    bv = jnp.full((8, 128), -jnp.inf, F32)
    bi = lax.broadcasted_iota(jnp.int32, (8, 128), 0)
    bv, bi = router(0, bv, bi)
    wait(wcp(2, wv, 1))
    start(xcp(2), xcp(3), xcp(4), gcp(0))
    wait(fcp(0))
    prep_wv()
    mk.update(free_products(wk7, 0, (0, 6, 5)))
    kv_accumulate(True, mk, free_products(wv7, 0, range(7)))
    wait(xcp(2), xcp(3))
    start(gcp(1), ucp(0), gcp(2))
    wait(xcp(4))
    prep_x(1)
    order = ((0, 4), (0, 1), (0, 2), (0, 3), (1, 1), (0, 0), (0, 6), (1, 4), (0, 5), (1, 2), (1, 3), (1, 0), (1, 6), (1, 5))
    m, _ = _ordered(_nt, lambda s: _unpack((wk7, wv7)[s[0]][s[1]]), lambda s: _unpack(xc7[1, s[1]]), order, never)
    kv_accumulate(False, [m[0, j] for j in range(7)], [m[1, j] for j in range(7)])
    prep_x(2, never)
    for t in range(1, NT):
        bv, bi = router(t, bv, bi)
    rmax = jnp.max(bv, axis=0, keepdims=True)
    idx = jnp.min(jnp.where(bv == rmax, bi, S))
    rsel = jax.nn.sigmoid(rmax)
    blk = pl.ds(pl.multiple_of((idx >> 4) << 4, 16), 16)
    routed = lax.broadcasted_iota(jnp.int32, (16, D), 0) == (idx & 15)
    xs = jnp.sum(jnp.where(routed, xa[blk, :].astype(F32), 0.0), axis=0, keepdims=True)
    xsb[...] = jnp.broadcast_to(xs, (128, D)).T
    wait(gcp(0), gcp(1), ucp(0))
    start(gcp(3), ucp(1))
    wait(fcp(1))
    kv_update(2, never)
    prep_x(3, never)
    gate_up(0, never)
    wait(gcp(2), gcp(3), ucp(1))
    start(wcp(0, wq, 2), cp(wo_h, wo, 5))
    wait(fcp(2))
    kv_update(3, never)
    gate_up(1, never)
    wait(wcp(0, wq, 2), cp(wo_h, wo, 5))
    start(dcp(0), dcp(1))
    wait(fcp(3))
    for g in range(4):
        lent = fold7(wq, wq7, g, lent)
    finalize_kv()
    hidden()
    prep_wo()
    attend(0, never)
    wait(dcp(0), dcp(1))
    attend(1, never)
    down(0, never)
    wait(ocp(0))
    attend(2, never)
    down(1, never)
    wait(ocp(1))
    y = jnp.sum(yacc[...], axis=0, keepdims=True) * jnp.concatenate([rsel] * (D // 128), axis=1)
    attend(3, never, y, idx)
    wait(ocp(2))

    @pl.when(idx < (NT - 1) * TM)
    def _():
        gsel = jnp.concatenate([gb[blk, :]] * (D // 128), axis=1)
        old = ob[blk, :].astype(F32)
        pb[...] = jnp.where(routed, old + (1.0 - gsel) * y, old).astype(BF)
        patch = cp(pb, out_h.at[blk, :], 7)
        patch.start()
        patch.wait()

    wait(*[qcp(q) for q in range(len(PIECES))])


@jax.jit
def pallas_gated_mix__linear_kernel_hedgehog__moe_arch_mod__prompt_kernel(
        A_x, A_wqkv, A_w_phi, A_wo, B_x, B_w_r, B_w_gate, B_w_up, B_w_down, gate_w):
    del B_x
    anyspec = pl.BlockSpec(memory_space=pl.ANY)
    V = pltpu.VMEM
    DMA = pltpu.SemaphoreType.DMA
    out = pl.pallas_call(
        kernel,
        out_shape=jax.ShapeDtypeStruct((S, D), BF),
        in_specs=[anyspec] * 9,
        out_specs=anyspec,
        scratch_shapes=[
            V((S, D), BF), V((D, D), BF), V((D, D), BF), V((D, D), BF), V((D, D), BF),
            V((D, F), BF), V((D, F), BF), V((F, D), BF),
            V((D, DH), BF), V((8, 128), BF), V((8, 128), BF), V((128, D), BF),
            V((S, D), BF), V((H // 2, 64, 128), F32), V((H // 2, 128, 128), F32),
            V((D // 2, 128), U32), V((H // 2, 128, 128), F32), V((S, 128), F32),
            V((D, 128), F32), V((16, F), F32), V((F, 128), F32), V((8, D), F32), V((16, D), BF),
            V((7, HD // 2 - 8, HD), U32), V((7, HD // 2, HD), U32), V((7, HD // 2 - 8, HD), U32),
            V((7, HD // 2, HD), U32), V((NT, 7, HT // 2, HD), U32), V((4, 8, 128), BF),
            DMA((8,)), DMA((4,)), DMA((NT + 1,)), DMA((4,)), DMA((2,)), DMA((2,)), DMA((NT,)), DMA((4,)),
        ],
        compiler_params=pltpu.CompilerParams(
            vmem_limit_bytes=110 * 2**20, flags={"XLA_TPU_EVENLY_DISTRIBUTE_CRITICAL_NODES": True}),
    )(A_x.reshape(S, D), A_wqkv, A_w_phi.reshape(D, DH), A_wo,
      B_w_r.reshape(8, 128), B_w_gate, B_w_up, B_w_down, gate_w.reshape(8, 128))
    return out.reshape(1, S, D)
```

```python
import jax
import jax.numpy as jnp
from jax import lax
from jax.experimental import pallas as pl
from jax.experimental.pallas import tpu as pltpu

S, D, H, DH, F = 2048, 1024, 32, 32, 3584
TM = 512
NT = S // TM
HT = TM // 2
HD = D // 2
GDMA = (0, 1024, 1792, 2304, F)
UDMA = (0, 1792, F)
FCUT = (0, 1792, F)
PIECES = ((0, HD, HD), (HT, 0, HD), (HT, HD, 256), (HT, HD + 256, 256),
          (0, 0, 128), (0, 128, 128), (0, 256, 128), (0, 384, 128))
PORD = (2, 4, 1, 3, 0, 6, 5)
QORD = (1, 3, 4, 2, 0, 6, 5)
OORD = (2, 4, 5, 1, 3, 0, 6)
LOG2E = 1.4426950408889634
BF = jnp.bfloat16
F32 = jnp.float32
U32 = jnp.uint32


def _nt(a, b):
    return lax.dot_general(a, b, (((1,), (1,)), ((), ())), preferred_element_type=F32)


def _nn(a, b):
    return jnp.dot(a, b, preferred_element_type=F32)


def _store_packed(ref, rows, c0, x):
    for c in range(0, x.shape[1], 128):
        ref[rows, c0 + c:c0 + c + 128] = pltpu.bitcast(x[:, c:c + 128].astype(BF), U32)


def _unpack(x):
    return pltpu.bitcast(x, BF)


def _rcp(x):
    r = pl.reciprocal(x, approx=True)
    return r * (2.0 - x * r)


def _red8(x4, op):
    r = x4[:, 0]
    for k in range(1, 8):
        r = op(r, x4[:, k])
    return r


def _rot(r, op):
    r = op(r, pltpu.roll(r, 4, r.ndim - 2))
    return op(r, pltpu.roll(r, 2, r.ndim - 2))


def _dual_softmax_parts(pT):
    p4 = pT.reshape(H // 2, 8, 8, pT.shape[1])
    mx = _rot(_red8(p4, jnp.maximum), jnp.maximum)
    mn = _rot(_red8(p4, jnp.minimum), jnp.minimum)
    ep = jnp.exp2(p4 - mx[:, None])
    en = jnp.exp2(mn[:, None] - p4)
    rp = _rcp(_rot(_red8(ep, jnp.add), jnp.add))
    rn = _rcp(_rot(_red8(en, jnp.add), jnp.add))
    return ep, en, rp, rn


def _rowdot(xf, w8):
    acc = xf[:, 0:128] * w8[0:1]
    for k in range(1, 8):
        acc = acc + xf[:, k * 128:(k + 1) * 128] * w8[k:k + 1]
    return jnp.sum(acc, axis=1, keepdims=True)


def _matvec(w_ref, v_ref, r0, r1, c0, acc):
    for r in range(r0, r1, 16):
        t = w_ref[r:r + 16, c0:c0 + 128].astype(F32) * v_ref[r:r + 16, :]
        acc = acc + t[0:8]
        acc = acc + t[8:16]
    return acc


def _lhs_combos(a11, a12, a21, a22):
    return (a11 + a22, a21 + a22, a11, a22, a11 + a12, a21 - a11, a12 - a22)


RHS_SUMS = ((0, 0, 3, jnp.add), (2, 1, 3, jnp.subtract), (3, 2, 0, jnp.subtract),
            (5, 0, 1, jnp.add), (6, 2, 3, jnp.add))


def _halves(m):
    c11 = m[0] + m[3] - m[4] + m[6]
    c12 = m[2] + m[4]
    c21 = m[1] + m[3]
    c22 = m[0] - m[1] + m[2] + m[5]
    return jnp.concatenate([c11, c12], axis=1), jnp.concatenate([c21, c22], axis=1)


def _assemble(m):
    return jnp.concatenate(_halves(m), axis=0)


def _assemble_logits(m):
    slot = lax.broadcasted_iota(jnp.int32, (8, TM), 0) >> 1
    rows = []
    for half in _halves(m):
        first = [jnp.zeros(slot.shape, F32), jnp.zeros(slot.shape, F32)]
        rest = []
        for p in range(1, 8):
            r0 = 64 * p - 16
            v = [half[r0 + 8 * k:r0 + 8 * k + 8] for k in range(8)]
            lent = slot == p % 4
            first[p // 4] = jnp.where(lent, v[p // 4], first[p // 4])
            v[p // 4] = jnp.where(lent, 0.0, v[p // 4])
            rest += v
        rows += first + [half[0:48]] + rest
    return jnp.concatenate(rows, axis=0)


def _ordered(dot, lhs, rhs, order, never, prev=None):
    m = {}
    for j in order:
        a = lhs(j)
        if prev is not None:
            tie = jnp.concatenate([prev[0:16, 0:128]] * (HD // 128), axis=1).astype(BF)
            a = jnp.concatenate([jnp.where(never, tie, a[0:16]), a[16:]], axis=0)
        prev = m[j] = dot(a, rhs(j))
    return m, prev


def _ordered_tn(lhs, rhs, order, never):
    m = {}
    prev = None
    for j in order:
        a = lhs(j)
        if prev is not None:
            tie = jnp.concatenate([prev[0:16, 0:128]] * (HD // 16), axis=0).astype(BF)
            a = jnp.concatenate([jnp.where(never, tie, a[:, 0:128]), a[:, 128:]], axis=1)
        prev = m[j] = lax.dot_general(a, rhs(j), (((0,), (0,)), ((), ())), preferred_element_type=F32)
    return m


def kernel(xa_h, wqkv_h, wphi_h, wo_h, wr_h, wg_h, wu_h, wd_h, gw_h, out_h,
           xa, wq, wk, wv, wo, wg, wu, wd, wphi, wr, gw, bdt,
           ob, kvacc, zacc, kvt, zb, gb, xsb, gu, hb, yacc, pb, wk7, wv7, wq7, wo7, xc7, fence,
           sem, ksem, xsem, gsem, usem, dsem, osem, fsem):
    def cp(src, dst, k):
        return pltpu.make_async_copy(src, dst, sem.at[k])

    def wcp(part, dst, k):
        return cp(wqkv_h.at[:, pl.ds(part * D, D)], dst, k)

    def xcp(j):
        rs = pl.ds(j * HT, HT) if j < 2 else pl.ds((j - 1) * TM, TM)
        return pltpu.make_async_copy(xa_h.at[rs, :], xa.at[rs, :], xsem.at[j])

    def kcp(i):
        return pltpu.make_async_copy(wqkv_h.at[:, pl.ds(D + i * 256, 256)], wk.at[:, pl.ds(i * 256, 256)], ksem.at[i])

    def gcp(i):
        cs = pl.ds(GDMA[i], GDMA[i + 1] - GDMA[i])
        return pltpu.make_async_copy(wg_h.at[:, cs], wg.at[:, cs], gsem.at[i])

    def ucp(i):
        cs = pl.ds(UDMA[i], UDMA[i + 1] - UDMA[i])
        return pltpu.make_async_copy(wu_h.at[:, cs], wu.at[:, cs], usem.at[i])

    def dcp(i):
        rs = pl.ds(FCUT[i], FCUT[i + 1] - FCUT[i])
        return pltpu.make_async_copy(wd_h.at[rs, :], wd.at[rs, :], dsem.at[i])

    def ocp(t):
        rs = pl.ds(t * TM, TM)
        return pltpu.make_async_copy(ob.at[rs, :], out_h.at[rs, :], osem.at[t])

    def qcp(q):
        rs, cs = pl.ds((NT - 1) * TM + PIECES[q][0], HT), pl.ds(*PIECES[q][1:])
        return pltpu.make_async_copy(ob.at[rs, cs], out_h.at[rs, cs], osem.at[NT - 1])

    def fcp(i):
        return pltpu.make_async_copy(wr_h, fence.at[i], fsem.at[i])

    def start(*cs):
        for c in cs:
            c.start()

    def wait(*cs):
        for c in cs:
            c.wait()

    def fold(w_ref, c, lent):
        slot = lax.broadcasted_iota(jnp.int32, (8, D), 0) >> 1
        x = _nt(bdt[:, c * 128:(c + 1) * 128], w_ref[:, c * 128:(c + 1) * 128]) * LOG2E
        pairs = []
        for q in range(2):
            p = 2 * (c % 4) + q
            own = slot == p % 4
            v = [x[q * 64 + 8 * k:q * 64 + 8 * k + 8] for k in range(8)]
            shift = _rot(jnp.where(own, v[p // 4], 0.0), jnp.add)
            v = [u - shift for u in v]
            if p == 0:
                lent, v = v[:2], v[2:]
            else:
                v[p // 4] = jnp.where(own, lent[p // 4], v[p // 4])
            pairs.append(jnp.concatenate(v, axis=0))
        return pairs, lent

    def store_lhs(dst, p, top, bottom, js):
        rows = slice(max(p * DH - 8, 0), (p + 1) * DH - 8)
        combos = _lhs_combos(top[:, :HD], top[:, HD:], bottom[:, :HD], bottom[:, HD:])
        for j in js:
            _store_packed(dst.at[j], rows, 0, combos[j])

    def prep_wv():
        for g in range(4):
            u = wv[:, g * 128:(g + 1) * 128].T.astype(F32)
            w = wv[:, (g + 4) * 128:(g + 5) * 128].T.astype(F32)
            for j, c in enumerate(_lhs_combos(u[:, :HD], u[:, HD:], w[:, :HD], w[:, HD:])):
                _store_packed(wv7.at[j], slice(g * 64, (g + 1) * 64), 0, c)

    def rhs7(src, corners, nr, dst, never, js=range(7)):
        prev = None
        for r in range(0, nr, 16):
            rd = slice(r // 2, r // 2 + 8)
            for c in range(0, HD, 128):
                raw = {}
                for j, u, v, op in ((1, 0, 0, None), (4, 3, 3, None)) + RHS_SUMS:
                    if j not in js:
                        continue
                    for i in (u, v):
                        if i not in raw:
                            r0, c0 = corners[i]
                            raw[i] = src[r0 + r:r0 + r + 16, c0 + c:c0 + c + 128]
                    if op is None:
                        dst[j, rd, c:c + 128] = pltpu.bitcast(raw[u], U32)
                        continue
                    bu = raw[u].astype(F32)
                    if never is not None and prev is not None:
                        bu = jnp.where(never, prev, bu)
                    prev = op(bu, raw[v].astype(F32))
                    _store_packed(dst.at[j], rd, c, prev)

    def prep_x(t, never=None, js=range(7)):
        r0 = t * TM
        rhs7(xa, ((r0, 0), (r0 + HT, 0), (r0, HD), (r0 + HT, HD)), HT, xc7.at[t], never, js)

    def prep_wo():
        rhs7(wo, ((0, 0), (0, HD), (HD, 0), (HD, HD)), HD, wo7, None)

    def products(w7, t, order, never, prev=None):
        return _ordered(_nt, lambda j: _unpack(w7[j]), lambda j: _unpack(xc7[t, j]), order, never, prev)

    def free_products(w7, t, js):
        return {j: _nt(_unpack(w7[j]), _unpack(xc7[t, j])) for j in js}

    def kv_accumulate(first, mk, mv):
        ep, en, rp, rn = _dual_softmax_parts(_assemble_logits(mk))
        php = (ep * rp[:, None]).reshape(H // 2, 64, TM)
        phn = (en * rn[:, None]).reshape(H // 2, 64, TM)
        ph = jnp.concatenate([php, phn], axis=1)
        zz = ph[:, :, 0:128]
        for c in range(1, TM // 128):
            zz = zz + ph[:, :, c * 128:(c + 1) * 128]
        zacc[...] = zz if first else zacc[...] + zz
        phb = ph.astype(BF)
        vT = _assemble(mv).astype(BF)
        for j in range(H // 2):
            u = _nt(vT[j * 64:(j + 1) * 64], phb[j])
            kvacc[j] = u if first else kvacc[j] + u

    def kv_update(t, never):
        mk, prev = products(wk7, t, PORD, never)
        kv_accumulate(False, mk, products(wv7, t, PORD, never, prev)[0])

    def finalize_kv():
        r3 = lax.broadcasted_iota(jnp.int32, kvacc.shape, 1)
        c3 = lax.broadcasted_iota(jnp.int32, kvacc.shape, 2)
        same_head = (r3 >> 5) == (c3 & 1)
        kvt[...] = pltpu.bitcast(jnp.where(same_head, kvacc[...], 0.0).reshape(D, 128).astype(BF), U32)
        zb[...] = jnp.broadcast_to(jnp.sum(zacc[...], axis=2, keepdims=True), zb.shape)

    def router(t, bv, bi):
        rs = slice(t * TM, (t + 1) * TM)
        xf = xa[rs, :].astype(F32)
        gb[rs, :] = jnp.broadcast_to(jax.nn.sigmoid(_rowdot(xf, gw[...].astype(F32))), (TM, 128))
        r = _rowdot(xf, wr[...].astype(F32)).astype(BF).astype(F32)
        r = jnp.broadcast_to(jnp.where(r != r, -jnp.inf, r), (TM, 128))
        row = lax.broadcasted_iota(jnp.int32, (8, 128), 0) + t * TM
        for k in range(TM // 8):
            rk = r[k * 8:(k + 1) * 8]
            better = rk > bv
            bv = jnp.where(better, rk, bv)
            bi = jnp.where(better, row + k * 8, bi)
        return bv, bi

    def gate_up(i, never):
        acc = None
        for c0 in range(FCUT[i], FCUT[i + 1], 128):
            for m, w_ref in enumerate((wg, wu)):
                acc = jnp.zeros((8, 128), F32) if acc is None else jnp.where(never, acc, 0.0)
                acc = _matvec(w_ref, xsb, 0, D, c0, acc)
                gu[m * 8:(m + 1) * 8, c0:c0 + 128] = acc

    def hidden():
        gg = jnp.sum(gu[0:8, :], axis=0, keepdims=True)
        uu = jnp.sum(gu[8:16, :], axis=0, keepdims=True)
        hb[...] = jnp.broadcast_to(gg * jax.nn.sigmoid(gg) * uu, (128, F)).T

    def down(i, never):
        acc = None
        for c0 in range(0, D, 128):
            cs = slice(c0, c0 + 128)
            acc = jnp.zeros((8, 128), F32) if acc is None else jnp.where(never, acc, 0.0)
            acc = _matvec(wd, hb, FCUT[i], FCUT[i + 1], c0, acc)
            yacc[:, cs] = acc if i == 0 else yacc[:, cs] + acc

    def attend(t, never, y=None, idx=None):
        r0 = t * TM
        ep, en, rp, rn = _dual_softmax_parts(_assemble_logits(products(wq7, t, QORD, never)[0]))
        z4 = zb[...].reshape(H // 2, 2, 8, 8, 128)
        zp = jnp.concatenate([z4[:, 0]] * (TM // 128), axis=-1)
        zn = jnp.concatenate([z4[:, 1]] * (TM // 128), axis=-1)
        den = _rot(_red8(ep * zp, jnp.add) * rp + _red8(en * zn, jnp.add) * rn, jnp.add) + 1e-6
        rd = _rcp(den)
        php = (ep * (rp * rd)[:, None]).reshape(H // 2, 64, TM)
        phn = (en * (rn * rd)[:, None]).reshape(H // 2, 64, TM)
        phb = jnp.concatenate([php, phn], axis=1).astype(BF)
        oT = jnp.concatenate([_nn(_unpack(kvt[j * 32:(j + 1) * 32, :]), phb[j]) for j in range(H // 2)], axis=0)
        oc = _lhs_combos(oT[:HD, :HT], oT[HD:, :HT], oT[:HD, HT:], oT[HD:, HT:])
        a = _assemble(_ordered_tn(lambda j: oc[j].astype(BF), lambda j: _unpack(wo7[j]), OORD, never))
        g = jnp.concatenate([gb[r0:r0 + TM, :]] * (D // 128), axis=1)
        b = xa[r0:r0 + TM, :].astype(F32)
        if y is not None:
            b = jnp.where(lax.broadcasted_iota(jnp.int32, (TM, D), 0) == idx - r0, b + y, b)
        res = (g * a + (1.0 - g) * b).astype(BF)
        if t < NT - 1:
            ob[r0:r0 + TM, :] = res
            start(ocp(t))
        else:
            for q, (rq, cq, wq_) in enumerate(PIECES):
                ob[r0 + rq:r0 + rq + HT, cq:cq + wq_] = res[rq:rq + HT, cq:cq + wq_]
                start(qcp(q))

    start(cp(wphi_h, wphi, 0), kcp(2), xcp(0), cp(wr_h, wr, 3), cp(gw_h, gw, 4), *[fcp(i) for i in range(6)])
    jj = lax.broadcasted_iota(jnp.int32, (128, DH), 0)
    ff = lax.broadcasted_iota(jnp.int32, (128, DH), 1)
    pick = jnp.where(((jj & 63) >> 1) == ff, 1.0, 0.0).astype(BF)
    j2 = lax.broadcasted_iota(jnp.int32, (128, 128), 0)
    c2 = lax.broadcasted_iota(jnp.int32, (128, 128), 1)
    keep = (c2 >> 5) == (j2 >> 6) * 2 + (j2 & 1)
    wait(cp(wphi_h, wphi, 0))
    start(kcp(3))
    wait(cp(wr_h, wr, 3))
    bd = _nt(pick, wphi[...])
    for g in range(8):
        bdt[:, g * 128:(g + 1) * 128] = jnp.where(keep, bd[:, g * 128:(g + 1) * 128], 0.0).astype(BF)
    never = jnp.max(jnp.where(bd[0:8, 0:128] > 0.0, 1, 0)) < 0
    z0 = jnp.where(never, 1, 0)
    z8 = pl.ds(pl.multiple_of(z0 * 8, 8), 8)
    for r in (wk7, wv7, wq7, wo7):
        r[z0, 0:8, 0:128] = jnp.zeros((8, 128), U32)
    xc7[z0, 0, 0:8, 0:128] = jnp.zeros((8, 128), U32)
    for r in (gb, xsb, hb):
        r[z8, :] = jnp.zeros((8, 128), F32)
    for r in (kvacc, zacc, zb):
        r[z0, 0:8, :] = jnp.zeros((8, 128), F32)
    kvt[z8, :] = jnp.zeros((8, 128), U32)
    gu[z8, 0:128] = jnp.zeros((8, 128), F32)

    bottom, lent = [], None
    for i in range(2):
        wait(kcp(2 + i))
        start(kcp(i))
        wait(fcp(4 + i))
        for c in (4 + 2 * i, 5 + 2 * i):
            pairs, lent = fold(wk, c, lent)
            for w in pairs:
                store_lhs(wk7, len(bottom), w, w, (1, 3))
                bottom.append(w)
    wait(xcp(0))
    start(xcp(1), wcp(2, wv, 1))
    wait(cp(gw_h, gw, 4))
    prep_x(0, js=(1, 3))
    mk = free_products(wk7, 0, (1, 3))
    wait(kcp(0), kcp(1))
    for c in range(4):
        pairs, lent = fold(wk, c, lent)
        for q, u in enumerate(pairs):
            store_lhs(wk7, 2 * c + q, u, bottom[2 * c + q], (0, 2, 4, 5, 6))
    wait(xcp(1))
    prep_x(0, js=(0, 2, 4, 5, 6))
    mk.update(free_products(wk7, 0, (4, 2, 0)))
    bv = jnp.full((8, 128), -jnp.inf, F32)
    bi = lax.broadcasted_iota(jnp.int32, (8, 128), 0)
    bv, bi = router(0, bv, bi)
    wait(wcp(2, wv, 1))
    start(xcp(2), xcp(3), xcp(4), gcp(0))
    wait(fcp(0))
    prep_wv()
    mk.update(free_products(wk7, 0, (6, 5)))
    kv_accumulate(True, mk, free_products(wv7, 0, range(7)))
    wait(xcp(2), xcp(3))
    start(gcp(1), ucp(0), gcp(2))
    wait(xcp(4))
    prep_x(1)
    order = ((0, 4), (0, 1), (0, 2), (0, 3), (1, 1), (0, 0), (0, 6), (1, 4), (0, 5), (1, 2), (1, 3), (1, 0), (1, 6), (1, 5))
    m, _ = _ordered(_nt, lambda s: _unpack((wk7, wv7)[s[0]][s[1]]), lambda s: _unpack(xc7[1, s[1]]), order, never)
    kv_accumulate(False, [m[0, j] for j in range(7)], [m[1, j] for j in range(7)])
    prep_x(2, never)
    for t in range(1, NT):
        bv, bi = router(t, bv, bi)
    rmax = jnp.max(bv, axis=0, keepdims=True)
    idx = jnp.min(jnp.where(bv == rmax, bi, S))
    rsel = jax.nn.sigmoid(rmax)
    blk = pl.ds(pl.multiple_of((idx >> 4) << 4, 16), 16)
    routed = lax.broadcasted_iota(jnp.int32, (16, D), 0) == (idx & 15)
    xs = jnp.sum(jnp.where(routed, xa[blk, :].astype(F32), 0.0), axis=0, keepdims=True)
    xsb[...] = jnp.broadcast_to(xs, (128, D)).T
    wait(gcp(0), gcp(1), ucp(0))
    start(gcp(3), ucp(1))
    wait(fcp(1))
    kv_update(2, never)
    prep_x(3, never)
    gate_up(0, never)
    wait(gcp(2), gcp(3), ucp(1))
    start(wcp(0, wq, 2), cp(wo_h, wo, 5))
    wait(fcp(2))
    kv_update(3, never)
    gate_up(1, never)
    wait(wcp(0, wq, 2), cp(wo_h, wo, 5))
    start(dcp(0), dcp(1))
    wait(fcp(3))
    lent_top = lent_bottom = None
    for c in range(4):
        top, lent_top = fold(wq, c, lent_top)
        bottom, lent_bottom = fold(wq, c + 4, lent_bottom)
        for q in range(2):
            store_lhs(wq7, 2 * c + q, top[q], bottom[q], range(7))
    finalize_kv()
    hidden()
    prep_wo()
    attend(0, never)
    wait(dcp(0), dcp(1))
    attend(1, never)
    down(0, never)
    wait(ocp(0))
    attend(2, never)
    down(1, never)
    wait(ocp(1))
    y = jnp.sum(yacc[...], axis=0, keepdims=True) * jnp.concatenate([rsel] * (D // 128), axis=1)
    attend(3, never, y, idx)
    wait(ocp(2))

    @pl.when(idx < (NT - 1) * TM)
    def _():
        gsel = jnp.concatenate([gb[blk, :]] * (D // 128), axis=1)
        old = ob[blk, :].astype(F32)
        pb[...] = jnp.where(routed, old + (1.0 - gsel) * y, old).astype(BF)
        patch = cp(pb, out_h.at[blk, :], 7)
        patch.start()
        patch.wait()

    wait(*[qcp(q) for q in range(len(PIECES))])


@jax.jit
def pallas_gated_mix__linear_kernel_hedgehog__moe_arch_mod__prompt_kernel(
        A_x, A_wqkv, A_w_phi, A_wo, B_x, B_w_r, B_w_gate, B_w_up, B_w_down, gate_w):
    del B_x
    anyspec = pl.BlockSpec(memory_space=pl.ANY)
    V = pltpu.VMEM
    DMA = pltpu.SemaphoreType.DMA
    out = pl.pallas_call(
        kernel,
        out_shape=jax.ShapeDtypeStruct((S, D), BF),
        in_specs=[anyspec] * 9,
        out_specs=anyspec,
        scratch_shapes=[
            V((S, D), BF), V((D, D), BF), V((D, D), BF), V((D, D), BF), V((D, D), BF),
            V((D, F), BF), V((D, F), BF), V((F, D), BF),
            V((D, DH), BF), V((8, 128), BF), V((8, 128), BF), V((128, D), BF),
            V((S, D), BF), V((H // 2, 64, 128), F32), V((H // 2, 128, 128), F32),
            V((D // 2, 128), U32), V((H // 2, 128, 128), F32), V((S, 128), F32),
            V((D, 128), F32), V((16, F), F32), V((F, 128), F32), V((8, D), F32), V((16, D), BF),
            V((7, HD // 2 - 8, HD), U32), V((7, HD // 2, HD), U32), V((7, HD // 2 - 8, HD), U32),
            V((7, HD // 2, HD), U32), V((NT, 7, HT // 2, HD), U32), V((6, 8, 128), BF),
            DMA((8,)), DMA((4,)), DMA((NT + 1,)), DMA((4,)), DMA((2,)), DMA((2,)), DMA((NT,)), DMA((6,)),
        ],
        compiler_params=pltpu.CompilerParams(
            vmem_limit_bytes=110 * 2**20, flags={"XLA_TPU_EVENLY_DISTRIBUTE_CRITICAL_NODES": True}),
    )(A_x.reshape(S, D), A_wqkv, A_w_phi.reshape(D, DH), A_wo,
      B_w_r.reshape(8, 128), B_w_gate, B_w_up, B_w_down, gate_w.reshape(8, 128))
    return out.reshape(1, S, D)
```
